```python
import jax
import jax.numpy as jnp

def _softmax(x, axis=-1):
    return jax.nn.softmax(x, axis=axis)

def _gelu(x):
    return jax.nn.gelu(x, approximate=True)

def _silu(x):
    return jax.nn.silu(x)

def _sigmoid(x):
    return jax.nn.sigmoid(x)

def _layernorm(x, axis=-1, eps=1e-05):
    m = jnp.mean(x, axis=axis, keepdims=True)
    v = jnp.var(x, axis=axis, keepdims=True)
    return (x - m) / jnp.sqrt(v + eps)

def _scatter_add(tgt, idx, src, axis=0):
    return tgt.at[idx].add(src)

def _segment_sum(src, seg, n):
    return jax.ops.segment_sum(src, seg, n)

class _Rng:

    def __init__(self, key):
        self._k = key

    def _next(self):
        self._k, sub = jax.random.split(self._k)
        return sub

    def normal(self, shape):
        return jax.random.normal(self._next(), shape, dtype=jnp.bfloat16)

    def randint(self, lo, hi, shape):
        return jax.random.randint(self._next(), shape, lo, hi, dtype=jnp.int32)

    def uniform(self, shape, lo=0.0, hi=1.0):
        return jax.random.uniform(self._next(), shape, jnp.bfloat16, lo, hi)

    def permutation(self, n):
        return jax.random.permutation(self._next(), n)
kernel_name = 'gated_mix__memory_aug_recurrent_mem_tr__sliding_local_dilated__prompt'

def setup_inputs():
    _rng = _Rng(jax.random.key(int.from_bytes(__import__("os").urandom(4), "little")))
    _w = lambda a: (lambda t: t.astype(jnp.bfloat16) if jnp.issubdtype(t.dtype, jnp.floating) else t)(jnp.asarray(a))

    def _A_setup():
        B, S, Dm = (1, 2048, 640)
        H, Dh = (32, 192)
        M, seg = (8, 32)
        seg = min(seg, S)
        S = S // seg * seg
        return {'x': _w((lambda *s: _rng.normal(s) * 0.05)(B, S, Dm)), 'mem0': _w((lambda *s: _rng.normal(s) * 0.05)(B, M, Dm)), 'Wq': _w((lambda *s: _rng.normal(s) * 0.05)(Dm, H, Dh) * Dm ** (-0.5)), 'Wk': _w((lambda *s: _rng.normal(s) * 0.05)(Dm, H, Dh) * Dm ** (-0.5)), 'Wv': _w((lambda *s: _rng.normal(s) * 0.05)(Dm, H, Dh) * Dm ** (-0.5)), 'Wo': _w((lambda *s: _rng.normal(s) * 0.05)(H, Dh, Dm) * (H * Dh) ** (-0.5)), 'seg_len': seg}
    _A_in = _A_setup()

    def _B_setup():
        B, S, D = (1, 2048, 640)
        return {'x': _w((lambda *s: _rng.normal(s) * 0.05)(B, S, D)), 'wqkv': _w((lambda *s: _rng.normal(s) * 0.05)(D, 3 * D)), 'wo': _w((lambda *s: _rng.normal(s) * 0.05)(D, D))}
    _B_in = _B_setup()
    return {'A_x': _A_in['x'], 'A_mem0': _A_in['mem0'], 'A_Wq': _A_in['Wq'], 'A_Wk': _A_in['Wk'], 'A_Wv': _A_in['Wv'], 'A_Wo': _A_in['Wo'], 'A_seg_len': _A_in['seg_len'], 'B_x': _B_in['x'], 'B_wqkv': _B_in['wqkv'], 'B_wo': _B_in['wo'], 'gate_w': _w((lambda *s: _rng.normal(s) * 0.05)(640))}

def reference(A_x, A_mem0, A_Wq, A_Wk, A_Wv, A_Wo, A_seg_len, B_x, B_wqkv, B_wo, gate_w):

    def _A_ref(x, mem0, Wq, Wk, Wv, Wo, seg_len):
        B, S, Dm = x.shape
        H, Dh = (Wq.shape[1], Wq.shape[2])
        M = mem0.shape[1]
        scale = Dh ** (-0.5)
        n_seg = S // seg_len
        L = M + seg_len
        idx = jnp.arange(L)
        mask = (idx[:, None] < M) | (idx[:, None] >= idx[None, :])
        mem = mem0
        outs = []
        for s in range(n_seg):
            xs = x[:, s * seg_len:(s + 1) * seg_len, :].copy()
            h = jnp.concatenate([mem, xs], axis=1)
            q = jnp.einsum('btd,dhe->bhte', h, Wq)
            k = jnp.einsum('btd,dhe->bhte', h, Wk)
            v = jnp.einsum('btd,dhe->bhte', h, Wv)
            scores = jnp.einsum('bhqe,bhke->bhqk', q, k) * scale
            scores = jnp.where(mask[None, None], scores, -1000000000.0)
            p = _softmax(scores, axis=-1)
            o = jnp.einsum('bhqk,bhke->bhqe', p, v)
            o = jnp.einsum('bhte,hed->btd', o, Wo)
            mem = o[:, :M, :].copy()
            outs.append(o[:, M:, :])
        return jnp.concatenate(outs, axis=1)

    def _B_ref(x, wqkv, wo):
        B, S, D = x.shape
        H = 32
        Dh = D // H
        W, dil = (8, 2)
        qkv = (lambda x, *d: x.transpose(*d))((x @ wqkv).reshape(B, S, 3, H, Dh), 2, 0, 3, 1, 4)
        q, k, v = (qkv[0], qkv[1], qkv[2])
        scale = Dh ** (-0.5)
        pos = jnp.arange(S)
        off = jnp.arange(W) * dil
        idx = pos[:, None] - off[None, :]
        mask = idx >= 0
        idx_c = jnp.where(mask, idx, 0).reshape(-1)
        kg = k[:, :, idx_c, :].reshape(B, H, S, W, Dh)
        vg = v[:, :, idx_c, :].reshape(B, H, S, W, Dh)
        logits = jnp.einsum('bhsd,bhswd->bhsw', q, kg) * scale
        logits = jnp.where(mask[None, None, :, :], logits, -1000000000.0)
        attn = _softmax(logits, axis=-1)
        o = jnp.einsum('bhsw,bhswd->bhsd', attn, vg)
        return (lambda x, *d: x.transpose(*d))(o, 0, 2, 1, 3).reshape(B, S, D) @ wo
    x = A_x
    g = _sigmoid((x * gate_w).sum(-1, keepdims=True))
    a = _A_ref(x, A_mem0, A_Wq, A_Wk, A_Wv, A_Wo, A_seg_len)
    b = _B_ref(x, B_wqkv, B_wo)
    return g * a + (1 - g) * b
```

```python
import functools

import jax
import jax.numpy as jnp
from jax import lax
import jax.experimental.pallas as pl
import jax.experimental.pallas.tpu as pltpu

F32 = jnp.float32
BF16 = jnp.bfloat16

S = 2048
D = 640
H_A, DH_A = 32, 192
M_A = 8
SEG = 32
L = M_A + SEG
NPAIR = H_A // 2
PAIR = 2 * DH_A
H_B, DH_B = 32, 20
WIN, DIL = 8, 2
HALO = 16
NEG = -1000000000.0

B_CHUNK = 256
B_ROWS = 16

NT = (((1,), (1,)), ((), ()))
NN = (((1,), (0,)), ((), ()))


def _dot(a, b, dn=NN):
    return lax.dot_general(a, b, dn, preferred_element_type=F32)


def _pack(x):
    return pltpu.bitcast(x, jnp.uint32)


def _unpack(x):
    return pltpu.bitcast(x, BF16)


def _recip(d):
    r = pl.reciprocal(d, approx=True)
    return r * (2.0 - d * r)


def _kernel(seg_len,
            xa_hbm, mem0_hbm, wqT_hbm, wkT_hbm, wvT_hbm, woA_hbm,
            xb_hbm, wqkvB_hbm, woB_hbm, gw_hbm,
            out_hbm,
            xa_v, mem0_v, wT_v, wqkv_v, woA_raw, woA_v,
            xb_v, wB_raw, woB_raw, wB_v, woB_v, gw_v,
            qB, kB, vB, oB, bmix,
            mem_v, o_v, out_v,
            sems, out_sem):
    del seg_len
    cp_wB = pltpu.make_async_copy(wqkvB_hbm, wB_raw, sems.at[0])
    cp_woB = pltpu.make_async_copy(woB_hbm, woB_raw, sems.at[1])
    cp_xb = pltpu.make_async_copy(xb_hbm, xb_v, sems.at[2])
    cp_wq = pltpu.make_async_copy(wqT_hbm, wT_v.at[0], sems.at[3])
    cp_wk = pltpu.make_async_copy(wkT_hbm, wT_v.at[1], sems.at[4])
    cp_wv = pltpu.make_async_copy(wvT_hbm, wT_v.at[2], sems.at[5])
    cp_woA = pltpu.make_async_copy(woA_hbm, woA_raw, sems.at[6])
    cp_xa = pltpu.make_async_copy(xa_hbm, xa_v, sems.at[7])
    cp_m0 = pltpu.make_async_copy(mem0_hbm, mem0_v, sems.at[8])
    cp_gw = pltpu.make_async_copy(gw_hbm, gw_v, sems.at[9])
    for cp in (cp_wB, cp_woB, cp_xb, cp_wq, cp_wk, cp_wv, cp_woA, cp_xa, cp_m0, cp_gw):
        cp.start()

    old = lax.broadcasted_iota(jnp.int32, (D, D), 0)
    new = lax.broadcasted_iota(jnp.int32, (D, D), 1)
    perm = (old == (new % H_B) * DH_B + new // H_B)
    pm = jnp.where(perm, 1.0, 0.0).astype(BF16)
    newr = lax.broadcasted_iota(jnp.int32, (D, D), 0)
    oldc = lax.broadcasted_iota(jnp.int32, (D, D), 1)
    pmT = jnp.where(oldc == (newr % H_B) * DH_B + newr // H_B, 1.0, 0.0).astype(BF16)
    cp_wB.wait()
    for j in range(3):
        wB_v[:, j * D:(j + 1) * D] = _dot(wB_raw[:, j * D:(j + 1) * D], pm).astype(BF16)
    cp_woB.wait()
    woB_v[...] = _dot(pmT, woB_raw[...]).astype(BF16)

    zero_halo = jnp.zeros((HALO, 128), F32)
    for j in range(5):
        kB[j, 0:HALO, :] = zero_halo
        vB[j, 0:HALO, :] = zero_halo
    cp_xb.wait()
    scale_b = DH_B ** (-0.5)

    def b_chunk(c, carry):
        r0 = pl.multiple_of(c * B_CHUNK, B_CHUNK)
        xc = xb_v[pl.ds(r0, B_CHUNK), :]
        qkv = _dot(xc, wB_v[...])
        for j in range(5):
            qB[j, :, :] = qkv[:, j * 128:(j + 1) * 128]
            kB[j, pl.ds(HALO + r0, B_CHUNK), :] = qkv[:, D + j * 128:D + (j + 1) * 128]
            vB[j, pl.ds(HALO + r0, B_CHUNK), :] = qkv[:, 2 * D + j * 128:2 * D + (j + 1) * 128]

        def blk(b, carry2):
            lr = pl.multiple_of(b * B_ROWS, B_ROWS)
            gr = pl.multiple_of(r0 + lr, B_ROWS)
            pos = gr + lax.broadcasted_iota(jnp.int32, (B_ROWS, 128), 0)
            q = [qB[j, pl.ds(lr, B_ROWS), :] for j in range(5)]
            logits = []
            for w in range(WIN):
                s = q[0] * kB[0, pl.ds(HALO + gr - DIL * w, B_ROWS), :]
                for j in range(1, 5):
                    s = s + q[j] * kB[j, pl.ds(HALO + gr - DIL * w, B_ROWS), :]
                s = s + pltpu.roll(s, 64, 1)
                s = s + pltpu.roll(s, 32, 1)
                s = s * scale_b
                s = jnp.where(pos >= DIL * w, s, NEG)
                logits.append(s)
            m = logits[0]
            for w in range(1, WIN):
                m = jnp.maximum(m, logits[w])
            e = [jnp.exp(l - m) for l in logits]
            den = e[0]
            for w in range(1, WIN):
                den = den + e[w]
            inv = _recip(den)
            for j in range(5):
                acc = e[0] * vB[j, pl.ds(HALO + gr, B_ROWS), :]
                for w in range(1, WIN):
                    acc = acc + e[w] * vB[j, pl.ds(HALO + gr - DIL * w, B_ROWS), :]
                oB[pl.ds(lr, B_ROWS), j * 128:(j + 1) * 128] = acc * inv
            return carry2

        lax.fori_loop(0, B_CHUNK // B_ROWS, blk, 0)
        bmix[pl.ds(r0, B_CHUNK), :] = _dot(oB[...], woB_v[...])
        return carry

    lax.fori_loop(0, S // B_CHUNK, b_chunk, 0)

    er = lax.broadcasted_iota(jnp.int32, (128, 128), 0)
    ec = lax.broadcasted_iota(jnp.int32, (128, 128), 1)
    eye = jnp.where(er == ec, 1.0, 0.0).astype(BF16)
    cp_wq.wait()
    cp_wk.wait()
    cp_wv.wait()

    def xpose_pair(p, carry):
        r = pl.multiple_of(p * PAIR, 128)
        for t in range(3):
            blocks = (wT_v[t, pl.ds(r, 128), :],
                      wT_v[t, pl.ds(r + 192, 128), :],
                      jnp.concatenate([wT_v[t, pl.ds(r + 128, 64), :],
                                       wT_v[t, pl.ds(r + 320, 64), :]], axis=0))
            for k in range(3):
                col = (t * 3 + k) * 128
                for j in range(5):
                    tile = blocks[k][:, j * 128:(j + 1) * 128]
                    wqkv_v[p, j * 64:(j + 1) * 64, col:col + 128] = _pack(
                        _dot(eye, tile, NT).astype(BF16))
        return carry

    lax.fori_loop(0, NPAIR, xpose_pair, 0)

    cp_woA.wait()

    def repack_wo(p, carry):
        r = pl.multiple_of(p * PAIR, 128)
        rp = pl.multiple_of(p * (PAIR // 2), 64)
        woA_v[pl.ds(rp, 64), :] = _pack(woA_raw[pl.ds(r, 128), :])
        woA_v[pl.ds(rp + 64, 64), :] = _pack(woA_raw[pl.ds(r + 192, 128), :])
        woA_v[pl.ds(rp + 128, 32), :] = _pack(woA_raw[pl.ds(r + 128, 64), :])
        woA_v[pl.ds(rp + 160, 32), :] = _pack(woA_raw[pl.ds(r + 320, 64), :])
        return carry

    lax.fori_loop(0, NPAIR, repack_wo, 0)
    cp_xa.wait()
    cp_m0.wait()
    cp_gw.wait()
    mem_v[...] = mem0_v[...].astype(F32)

    scale_a = DH_A ** (-0.5)
    qi = lax.broadcasted_iota(jnp.int32, (L, L), 0)
    ki = lax.broadcasted_iota(jnp.int32, (L, L), 1)
    mask = (qi < M_A) | (qi >= ki)
    lane = lax.broadcasted_iota(jnp.int32, (L, 128), 1)
    lo = lane < 64

    def softmax(s):
        s = jnp.where(mask, s * scale_a, NEG)
        m = jnp.max(s, axis=1, keepdims=True)
        e = jnp.exp(s - m)
        den = jnp.sum(e, axis=1, keepdims=True)
        return e * _recip(den)

    def seg_step(s, carry):
        r0 = pl.multiple_of(s * SEG, SEG)
        xs = xa_v[pl.ds(r0, SEG), :].astype(F32)
        h = jnp.concatenate([mem_v[...], xs], axis=0)

        def qkv_proj(p):
            return _dot(h, _unpack(wqkv_v[p]))

        def scores(y):
            q0, q1, q2 = (y[:, k * 128:(k + 1) * 128] for k in range(3))
            k0, k1, k2 = (y[:, (3 + k) * 128:(4 + k) * 128] for k in range(3))
            q2a = jnp.where(lo, q2, 0.0)
            q2b = jnp.where(lo, 0.0, q2)
            sa = _dot(q0, k0, NT) + _dot(q2a, k2, NT)
            sb = _dot(q1, k1, NT) + _dot(q2b, k2, NT)
            return softmax(sa), softmax(sb)

        def pv(p, y, probs):
            pa, pb = probs
            v0, v1, v2 = (y[:, (6 + k) * 128:(7 + k) * 128] for k in range(3))
            o_v[:, p * PAIR:p * PAIR + 128] = _dot(pa, v0)
            o_v[:, p * PAIR + 128:p * PAIR + 256] = _dot(pb, v1)
            o_v[:, p * PAIR + 256:p * PAIR + 384] = jnp.where(lo, _dot(pa, v2), _dot(pb, v2))

        def out_proj(p, acc):
            w = _unpack(woA_v[p * (PAIR // 2):(p + 1) * (PAIR // 2), :])
            t = _dot(o_v[:, p * PAIR:(p + 1) * PAIR], w)
            return t if acc is None else acc + t

        ys, probs = {}, {}
        acc = None
        wo_next = 0
        for i in range(NPAIR + 2):
            if i < NPAIR:
                ys[i] = qkv_proj(i)
            else:
                for _ in range(3):
                    acc = out_proj(wo_next, acc)
                    wo_next += 1
            if 1 <= i <= NPAIR:
                probs[i - 1] = scores(ys[i - 1])
            if i >= 2:
                pv(i - 2, ys.pop(i - 2), probs.pop(i - 2))
        while wo_next < NPAIR:
            acc = out_proj(wo_next, acc)
            wo_next += 1
        mem_v[...] = acc[:M_A]
        a = acc[M_A:]
        g = jax.nn.sigmoid(jnp.sum(xs * gw_v[...].astype(F32), axis=1, keepdims=True))
        res = g * a + (1.0 - g) * bmix[pl.ds(r0, SEG), :]
        out_v[pl.ds(r0, SEG), :] = res.astype(BF16)
        pltpu.make_async_copy(out_v.at[pl.ds(r0, SEG), :], out_hbm.at[pl.ds(r0, SEG), :],
                              out_sem).start()
        return carry

    lax.fori_loop(0, S // SEG, seg_step, 0)
    pltpu.make_async_copy(out_v, out_hbm, out_sem).wait()


def pallas_gated_mix__memory_aug_recurrent_mem_tr__sliding_local_dilated__prompt_kernel(
    A_x, A_mem0, A_Wq, A_Wk, A_Wv, A_Wo, A_seg_len, B_x, B_wqkv, B_wo, gate_w,
):
    assert int(A_seg_len) == SEG
    hd = H_A * DH_A
    xa = A_x.reshape(S, D)
    mem0 = A_mem0.reshape(M_A, D)
    wqT = A_Wq.transpose(1, 2, 0).reshape(hd, D)
    wkT = A_Wk.transpose(1, 2, 0).reshape(hd, D)
    wvT = A_Wv.transpose(1, 2, 0).reshape(hd, D)
    woA = A_Wo.reshape(hd, D)
    xb = B_x.reshape(S, D)
    gw = gate_w.reshape(1, D)

    scratch = [
        pltpu.VMEM((S, D), BF16),
        pltpu.VMEM((M_A, D), BF16),
        pltpu.VMEM((3, hd, D), BF16),
        pltpu.VMEM((NPAIR, D // 2, 9 * 128), jnp.uint32),
        pltpu.VMEM((hd, D), BF16),
        pltpu.VMEM((hd // 2, D), jnp.uint32),
        pltpu.VMEM((S, D), BF16),
        pltpu.VMEM((D, 3 * D), BF16),
        pltpu.VMEM((D, D), BF16),
        pltpu.VMEM((D, 3 * D), BF16),
        pltpu.VMEM((D, D), BF16),
        pltpu.VMEM((1, D), BF16),
        pltpu.VMEM((5, B_CHUNK, 128), F32),
        pltpu.VMEM((5, HALO + S, 128), F32),
        pltpu.VMEM((5, HALO + S, 128), F32),
        pltpu.VMEM((B_CHUNK, D), F32),
        pltpu.VMEM((S, D), F32),
        pltpu.VMEM((M_A, D), F32),
        pltpu.VMEM((L, hd), F32),
        pltpu.VMEM((S, D), BF16),
        pltpu.SemaphoreType.DMA((10,)),
        pltpu.SemaphoreType.DMA,
    ]
    out = pl.pallas_call(
        functools.partial(_kernel, SEG),
        out_shape=jax.ShapeDtypeStruct((S, D), BF16),
        in_specs=[pl.BlockSpec(memory_space=pl.ANY)] * 10,
        out_specs=pl.BlockSpec(memory_space=pl.ANY),
        scratch_shapes=scratch,
        compiler_params=pltpu.CompilerParams(vmem_limit_bytes=120 * 1024 * 1024),
    )(xa, mem0, wqT, wkT, wvT, woA, xb, B_wqkv, B_wo, gw)
    return out.reshape(1, S, D)
```

```python
import functools

import jax
import jax.numpy as jnp
from jax import lax
import jax.experimental.pallas as pl
import jax.experimental.pallas.tpu as pltpu

F32 = jnp.float32
BF16 = jnp.bfloat16

S = 2048
D = 640
H_A, DH_A = 32, 192
M_A = 8
SEG = 32
L = M_A + SEG
NPAIR = H_A // 2
PAIR = 2 * DH_A
H_B, DH_B = 32, 20
WIN, DIL = 8, 2
HALO = 16
NEG = -1000000000.0

B_CHUNK = 256
B_ROWS = 16

NT = (((1,), (1,)), ((), ()))
NN = (((1,), (0,)), ((), ()))


def _dot(a, b, dn=NN):
    return lax.dot_general(a, b, dn, preferred_element_type=F32)


def _pack(x):
    return pltpu.bitcast(x, jnp.uint32)


def _unpack(x):
    return pltpu.bitcast(x, BF16)


def _recip(d):
    r = pl.reciprocal(d, approx=True)
    return r * (2.0 - d * r)


def _kernel(seg_len,
            xa_hbm, mem0_hbm, wqT_hbm, wkT_hbm, wvT_hbm, woA_hbm,
            wqkvB_hbm, woB_hbm, gw_hbm,
            out_hbm,
            xa_v, mem0_v, wT_v, wqkv_v, woA_raw, woA_v,
            wB_raw, woB_raw, wB_v, woB_v, gw_v,
            qB, kB, vB, oB, bmix,
            mem_v, o_v, out_v,
            sems, out_sem):
    del seg_len
    cp_wB = pltpu.make_async_copy(wqkvB_hbm, wB_raw, sems.at[0])
    cp_woB = pltpu.make_async_copy(woB_hbm, woB_raw, sems.at[1])
    cp_wq = pltpu.make_async_copy(wqT_hbm, wT_v.at[0], sems.at[3])
    cp_wk = pltpu.make_async_copy(wkT_hbm, wT_v.at[1], sems.at[4])
    cp_wv = pltpu.make_async_copy(wvT_hbm, wT_v.at[2], sems.at[5])
    cp_woA = pltpu.make_async_copy(woA_hbm, woA_raw, sems.at[6])
    cp_xa = pltpu.make_async_copy(xa_hbm, xa_v, sems.at[2])
    cp_m0 = pltpu.make_async_copy(mem0_hbm, mem0_v, sems.at[7])
    cp_gw = pltpu.make_async_copy(gw_hbm, gw_v, sems.at[8])
    for cp in (cp_wB, cp_xa, cp_woB, cp_wq, cp_wk, cp_wv, cp_woA, cp_m0, cp_gw):
        cp.start()

    old = lax.broadcasted_iota(jnp.int32, (D, D), 0)
    new = lax.broadcasted_iota(jnp.int32, (D, D), 1)
    perm = (old == (new % H_B) * DH_B + new // H_B)
    pm = jnp.where(perm, 1.0, 0.0).astype(BF16)
    newr = lax.broadcasted_iota(jnp.int32, (D, D), 0)
    oldc = lax.broadcasted_iota(jnp.int32, (D, D), 1)
    pmT = jnp.where(oldc == (newr % H_B) * DH_B + newr // H_B, 1.0, 0.0).astype(BF16)
    cp_wB.wait()
    for j in range(3):
        wB_v[:, j * D:(j + 1) * D] = _dot(wB_raw[:, j * D:(j + 1) * D], pm).astype(BF16)
    cp_woB.wait()
    woB_v[...] = _dot(pmT, woB_raw[...]).astype(BF16)

    zero_halo = jnp.zeros((HALO, 128), F32)
    for j in range(5):
        kB[j, 0:HALO, :] = zero_halo
        vB[j, 0:HALO, :] = zero_halo
    cp_xa.wait()
    scale_b = DH_B ** (-0.5)

    def b_chunk(c, carry):
        r0 = pl.multiple_of(c * B_CHUNK, B_CHUNK)
        xc = xa_v[pl.ds(r0, B_CHUNK), :]
        qkv = _dot(xc, wB_v[...])
        for j in range(5):
            qB[j, :, :] = qkv[:, j * 128:(j + 1) * 128]
            kB[j, pl.ds(HALO + r0, B_CHUNK), :] = qkv[:, D + j * 128:D + (j + 1) * 128]
            vB[j, pl.ds(HALO + r0, B_CHUNK), :] = qkv[:, 2 * D + j * 128:2 * D + (j + 1) * 128]

        def blk(b, carry2):
            lr = pl.multiple_of(b * B_ROWS, B_ROWS)
            gr = pl.multiple_of(r0 + lr, B_ROWS)
            pos = gr + lax.broadcasted_iota(jnp.int32, (B_ROWS, 128), 0)
            q = [qB[j, pl.ds(lr, B_ROWS), :] for j in range(5)]
            logits = []
            for w in range(WIN):
                s = q[0] * kB[0, pl.ds(HALO + gr - DIL * w, B_ROWS), :]
                for j in range(1, 5):
                    s = s + q[j] * kB[j, pl.ds(HALO + gr - DIL * w, B_ROWS), :]
                s = s + pltpu.roll(s, 64, 1)
                s = s + pltpu.roll(s, 32, 1)
                s = s * scale_b
                s = jnp.where(pos >= DIL * w, s, NEG)
                logits.append(s)
            m = logits[0]
            for w in range(1, WIN):
                m = jnp.maximum(m, logits[w])
            e = [jnp.exp(l - m) for l in logits]
            den = e[0]
            for w in range(1, WIN):
                den = den + e[w]
            inv = _recip(den)
            for j in range(5):
                acc = e[0] * vB[j, pl.ds(HALO + gr, B_ROWS), :]
                for w in range(1, WIN):
                    acc = acc + e[w] * vB[j, pl.ds(HALO + gr - DIL * w, B_ROWS), :]
                oB[pl.ds(lr, B_ROWS), j * 128:(j + 1) * 128] = acc * inv
            return carry2

        lax.fori_loop(0, B_CHUNK // B_ROWS, blk, 0)
        bmix[pl.ds(r0, B_CHUNK), :] = _dot(oB[...], woB_v[...])
        return carry

    lax.fori_loop(0, S // B_CHUNK, b_chunk, 0)

    er = lax.broadcasted_iota(jnp.int32, (128, 128), 0)
    ec = lax.broadcasted_iota(jnp.int32, (128, 128), 1)
    eye = jnp.where(er == ec, 1.0, 0.0).astype(BF16)
    cp_wq.wait()
    cp_wk.wait()
    cp_wv.wait()

    def xpose_pair(p, carry):
        r = pl.multiple_of(p * PAIR, 128)
        for t in range(3):
            blocks = (wT_v[t, pl.ds(r, 128), :],
                      wT_v[t, pl.ds(r + 192, 128), :],
                      jnp.concatenate([wT_v[t, pl.ds(r + 128, 64), :],
                                       wT_v[t, pl.ds(r + 320, 64), :]], axis=0))
            for k in range(3):
                col = (t * 3 + k) * 128
                for j in range(5):
                    tile = blocks[k][:, j * 128:(j + 1) * 128]
                    wqkv_v[p, j * 64:(j + 1) * 64, col:col + 128] = _pack(
                        _dot(eye, tile, NT).astype(BF16))
        return carry

    lax.fori_loop(0, NPAIR, xpose_pair, 0)

    cp_woA.wait()

    def repack_wo(p, carry):
        r = pl.multiple_of(p * PAIR, 128)
        rp = pl.multiple_of(p * (PAIR // 2), 64)
        woA_v[pl.ds(rp, 64), :] = _pack(woA_raw[pl.ds(r, 128), :])
        woA_v[pl.ds(rp + 64, 64), :] = _pack(woA_raw[pl.ds(r + 192, 128), :])
        woA_v[pl.ds(rp + 128, 32), :] = _pack(woA_raw[pl.ds(r + 128, 64), :])
        woA_v[pl.ds(rp + 160, 32), :] = _pack(woA_raw[pl.ds(r + 320, 64), :])
        return carry

    lax.fori_loop(0, NPAIR, repack_wo, 0)
    cp_m0.wait()
    cp_gw.wait()
    mem_v[...] = mem0_v[...].astype(F32)

    scale_a = DH_A ** (-0.5)
    qi = lax.broadcasted_iota(jnp.int32, (L, L), 0)
    ki = lax.broadcasted_iota(jnp.int32, (L, L), 1)
    mask = (qi < M_A) | (qi >= ki)
    lane = lax.broadcasted_iota(jnp.int32, (L, 128), 1)
    lo = lane < 64

    def softmax(s):
        s = jnp.where(mask, s * scale_a, NEG)
        m = jnp.max(s, axis=1, keepdims=True)
        e = jnp.exp(s - m)
        den = jnp.sum(e, axis=1, keepdims=True)
        return e * _recip(den)

    def seg_step(s, carry):
        r0 = pl.multiple_of(s * SEG, SEG)
        xs = xa_v[pl.ds(r0, SEG), :].astype(F32)
        h = jnp.concatenate([mem_v[...], xs], axis=0)

        def qkv_proj(p):
            return _dot(h, _unpack(wqkv_v[p]))

        def scores(y):
            q0, q1, q2 = (y[:, k * 128:(k + 1) * 128] for k in range(3))
            k0, k1, k2 = (y[:, (3 + k) * 128:(4 + k) * 128] for k in range(3))
            q2a = jnp.where(lo, q2, 0.0)
            q2b = jnp.where(lo, 0.0, q2)
            sa = _dot(q0, k0, NT) + _dot(q2a, k2, NT)
            sb = _dot(q1, k1, NT) + _dot(q2b, k2, NT)
            return softmax(sa), softmax(sb)

        def pv(p, y, probs):
            pa, pb = probs
            v0, v1, v2 = (y[:, (6 + k) * 128:(7 + k) * 128] for k in range(3))
            o_v[:, p * PAIR:p * PAIR + 128] = _dot(pa, v0)
            o_v[:, p * PAIR + 128:p * PAIR + 256] = _dot(pb, v1)
            o_v[:, p * PAIR + 256:p * PAIR + 384] = jnp.where(lo, _dot(pa, v2), _dot(pb, v2))

        def out_proj(p, acc):
            w = _unpack(woA_v[p * (PAIR // 2):(p + 1) * (PAIR // 2), :])
            t = _dot(o_v[:, p * PAIR:(p + 1) * PAIR], w)
            return t if acc is None else acc + t

        ys, probs = {}, {}
        acc = None
        wo_next = 0
        for i in range(NPAIR + 2):
            if i < NPAIR:
                ys[i] = qkv_proj(i)
            else:
                for _ in range(3):
                    acc = out_proj(wo_next, acc)
                    wo_next += 1
            if 1 <= i <= NPAIR:
                probs[i - 1] = scores(ys[i - 1])
            if i >= 2:
                pv(i - 2, ys.pop(i - 2), probs.pop(i - 2))
        while wo_next < NPAIR:
            acc = out_proj(wo_next, acc)
            wo_next += 1
        mem_v[...] = acc[:M_A]
        a = acc[M_A:]
        g = jax.nn.sigmoid(jnp.sum(xs * gw_v[...].astype(F32), axis=1, keepdims=True))
        res = g * a + (1.0 - g) * bmix[pl.ds(r0, SEG), :]
        out_v[pl.ds(r0, SEG), :] = res.astype(BF16)
        pltpu.make_async_copy(out_v.at[pl.ds(r0, SEG), :], out_hbm.at[pl.ds(r0, SEG), :],
                              out_sem).start()
        return carry

    lax.fori_loop(0, S // SEG, seg_step, 0)
    pltpu.make_async_copy(out_v, out_hbm, out_sem).wait()


def pallas_gated_mix__memory_aug_recurrent_mem_tr__sliding_local_dilated__prompt_kernel(
    A_x, A_mem0, A_Wq, A_Wk, A_Wv, A_Wo, A_seg_len, B_x, B_wqkv, B_wo, gate_w,
):
    del B_x
    assert int(A_seg_len) == SEG
    hd = H_A * DH_A
    xa = A_x.reshape(S, D)
    mem0 = A_mem0.reshape(M_A, D)
    wqT = A_Wq.transpose(1, 2, 0).reshape(hd, D)
    wkT = A_Wk.transpose(1, 2, 0).reshape(hd, D)
    wvT = A_Wv.transpose(1, 2, 0).reshape(hd, D)
    woA = A_Wo.reshape(hd, D)
    gw = gate_w.reshape(1, D)

    scratch = [
        pltpu.VMEM((S, D), BF16),
        pltpu.VMEM((M_A, D), BF16),
        pltpu.VMEM((3, hd, D), BF16),
        pltpu.VMEM((NPAIR, D // 2, 9 * 128), jnp.uint32),
        pltpu.VMEM((hd, D), BF16),
        pltpu.VMEM((hd // 2, D), jnp.uint32),
        pltpu.VMEM((D, 3 * D), BF16),
        pltpu.VMEM((D, D), BF16),
        pltpu.VMEM((D, 3 * D), BF16),
        pltpu.VMEM((D, D), BF16),
        pltpu.VMEM((1, D), BF16),
        pltpu.VMEM((5, B_CHUNK, 128), F32),
        pltpu.VMEM((5, HALO + S, 128), F32),
        pltpu.VMEM((5, HALO + S, 128), F32),
        pltpu.VMEM((B_CHUNK, D), F32),
        pltpu.VMEM((S, D), F32),
        pltpu.VMEM((M_A, D), F32),
        pltpu.VMEM((L, hd), F32),
        pltpu.VMEM((S, D), BF16),
        pltpu.SemaphoreType.DMA((9,)),
        pltpu.SemaphoreType.DMA,
    ]
    out = pl.pallas_call(
        functools.partial(_kernel, SEG),
        out_shape=jax.ShapeDtypeStruct((S, D), BF16),
        in_specs=[pl.BlockSpec(memory_space=pl.ANY)] * 9,
        out_specs=pl.BlockSpec(memory_space=pl.ANY),
        scratch_shapes=scratch,
        compiler_params=pltpu.CompilerParams(vmem_limit_bytes=120 * 1024 * 1024),
    )(xa, mem0, wqT, wkT, wvT, woA, B_wqkv, B_wo, gw)
    return out.reshape(1, S, D)
```

```python
import jax
import jax.numpy as jnp
from jax import lax
import jax.experimental.pallas as pl
import jax.experimental.pallas.tpu as pltpu

F32 = jnp.float32
BF16 = jnp.bfloat16

S = 2048
D = 640
H_A, DH_A = 32, 192
M_A = 8
SEG = 32
L = M_A + SEG
NPAIR = H_A // 2
PAIR = 2 * DH_A
H_B, DH_B = 32, 20
WIN, DIL = 8, 2
HALO = 16
NEG = -1000000000.0

B_ROWS = 8
XPOSE_MXU = False

NT = (((1,), (1,)), ((), ()))
NN = (((1,), (0,)), ((), ()))


def _dot(a, b, dn=NN):
    return lax.dot_general(a, b, dn, preferred_element_type=F32)


def _pack(x):
    return pltpu.bitcast(x, jnp.uint32)


def _unpack(x):
    return pltpu.bitcast(x, BF16)


def _recip(d):
    r = pl.reciprocal(d, approx=True)
    return r * (2.0 - d * r)


def _kernel(xa_hbm, mem0_hbm, wqT_hbm, wkT_hbm, wvT_hbm, woA_hbm,
            wqkvB_hbm, woB_hbm, gw_hbm,
            out_hbm,
            xa_v, mem0_v, wT_v, wqkv_v, woA_v,
            wB_raw, woB_raw, wB_v, woB_v, gw_v,
            qB, kB, vB,
            mem_v, o_v, out_v,
            sems, pair_sems, out_sem):
    cp_wB = pltpu.make_async_copy(wqkvB_hbm, wB_raw, sems.at[0])
    cp_xa = pltpu.make_async_copy(xa_hbm, xa_v, sems.at[1])
    cp_woB = pltpu.make_async_copy(woB_hbm, woB_raw, sems.at[2])
    cp_m0 = pltpu.make_async_copy(mem0_hbm, mem0_v, sems.at[3])
    cp_gw = pltpu.make_async_copy(gw_hbm, gw_v, sems.at[4])

    def pair_copies(p):
        r = pl.multiple_of(p * PAIR, 128)
        return [pltpu.make_async_copy(w.at[pl.ds(r, PAIR), :], wT_v.at[t, pl.ds(r, PAIR), :],
                                      pair_sems.at[p])
                for t, w in enumerate((wqT_hbm, wkT_hbm, wvT_hbm, woA_hbm))]

    for cp in (cp_wB, cp_woB, cp_xa, cp_m0, cp_gw):
        cp.start()
    for p in range(NPAIR):
        for cp in pair_copies(p):
            cp.start()

    old = lax.broadcasted_iota(jnp.int32, (D, D), 0)
    new = lax.broadcasted_iota(jnp.int32, (D, D), 1)
    pm = jnp.where(old == (new % H_B) * DH_B + new // H_B, 1.0, 0.0).astype(BF16)
    cp_wB.wait()
    for j in range(3):
        wB_v[:, j * D:(j + 1) * D] = _pack(
            _dot(wB_raw[:, j * D:(j + 1) * D], pm).astype(BF16))
    newr = lax.broadcasted_iota(jnp.int32, (D, D), 0)
    oldc = lax.broadcasted_iota(jnp.int32, (D, D), 1)
    pmT = jnp.where(oldc == (newr % H_B) * DH_B + newr // H_B, 1.0, 0.0).astype(BF16)
    cp_woB.wait()
    woB_v[...] = _pack(_dot(pmT, woB_raw[...]).astype(BF16))

    zero_halo = jnp.zeros((HALO, 128), F32)
    for j in range(5):
        kB[j, 0:HALO, :] = zero_halo
        vB[j, 0:HALO, :] = zero_halo
    cp_xa.wait()

    rows_b = S // NPAIR
    er = lax.broadcasted_iota(jnp.int32, (128, 128), 0)
    ec = lax.broadcasted_iota(jnp.int32, (128, 128), 1)
    eye = jnp.where(er == ec, 1.0, 0.0).astype(BF16)

    def prologue_step(p, carry):
        for cp in pair_copies(p):
            cp.wait()
        r = pl.multiple_of(p * PAIR, 128)

        def pair_blocks(t):
            return (wT_v[t, pl.ds(r, 128), :],
                    wT_v[t, pl.ds(r + 192, 128), :],
                    jnp.concatenate([wT_v[t, pl.ds(r + 128, 64), :],
                                     wT_v[t, pl.ds(r + 320, 64), :]], axis=0))

        r0 = pl.multiple_of(p * rows_b, rows_b)
        qkv = _dot(xa_v[pl.ds(r0, rows_b), :], _unpack(wB_v[...]))
        for j in range(5):
            qB[j, pl.ds(r0, rows_b), :] = qkv[:, j * 128:(j + 1) * 128]
            kB[j, pl.ds(HALO + r0, rows_b), :] = qkv[:, D + j * 128:D + (j + 1) * 128]
            vB[j, pl.ds(HALO + r0, rows_b), :] = qkv[:, 2 * D + j * 128:2 * D + (j + 1) * 128]
        for t in range(3):
            blocks = pair_blocks(t)
            for k in range(3):
                col = (t * 3 + k) * 128
                for j in range(5):
                    tile = blocks[k][:, j * 128:(j + 1) * 128]
                    if XPOSE_MXU:
                        tt = _dot(eye, tile, NT).astype(BF16)
                    else:
                        tt = tile.T
                    wqkv_v[p, j * 64:(j + 1) * 64, col:col + 128] = _pack(tt)
        for k, blk in enumerate(pair_blocks(3)):
            woA_v[p, k * 64:(k + 1) * 64, :] = _pack(blk)
        return carry

    lax.fori_loop(0, NPAIR, prologue_step, 0)

    cp_m0.wait()
    cp_gw.wait()
    mem_v[...] = mem0_v[...].astype(F32)

    scale_a = DH_A ** (-0.5)
    scale_b = DH_B ** (-0.5)
    qi = lax.broadcasted_iota(jnp.int32, (L, 2 * L), 0)
    kl = lax.broadcasted_iota(jnp.int32, (L, 2 * L), 1)
    head_a = kl < L
    ki = jnp.where(head_a, kl, kl - L)
    mask = (qi < M_A) | (qi >= ki)
    lane = lax.broadcasted_iota(jnp.int32, (L, 128), 1)
    lo = lane < 64
    zblk = jnp.zeros((L, 128), F32)

    def softmax_pair(s):
        s = jnp.where(mask, s * scale_a, NEG)
        ma = jnp.max(jnp.where(head_a, s, -jnp.inf), axis=1, keepdims=True)
        mb = jnp.max(jnp.where(head_a, -jnp.inf, s), axis=1, keepdims=True)
        e = jnp.exp(s - jnp.where(head_a, ma, mb))
        da = jnp.sum(jnp.where(head_a, e, 0.0), axis=1, keepdims=True)
        db = jnp.sum(jnp.where(head_a, 0.0, e), axis=1, keepdims=True)
        return e * _recip(jnp.where(head_a, da, db))

    def b_attend(gr):
        pos = gr + lax.broadcasted_iota(jnp.int32, (B_ROWS, 128), 0)
        q = [qB[j, pl.ds(gr, B_ROWS), :] for j in range(5)]
        logits = []
        for w in range(WIN):
            s = q[0] * kB[0, pl.ds(HALO + gr - DIL * w, B_ROWS), :]
            for j in range(1, 5):
                s = s + q[j] * kB[j, pl.ds(HALO + gr - DIL * w, B_ROWS), :]
            s = s + pltpu.roll(s, 64, 1)
            s = s + pltpu.roll(s, 32, 1)
            logits.append(jnp.where(pos >= DIL * w, s * scale_b, NEG))
        m = logits[0]
        for w in range(1, WIN):
            m = jnp.maximum(m, logits[w])
        e = [jnp.exp(l - m) for l in logits]
        den = e[0]
        for w in range(1, WIN):
            den = den + e[w]
        inv = _recip(den)
        cols = []
        for j in range(5):
            acc = e[0] * vB[j, pl.ds(HALO + gr, B_ROWS), :]
            for w in range(1, WIN):
                acc = acc + e[w] * vB[j, pl.ds(HALO + gr - DIL * w, B_ROWS), :]
            cols.append(acc * inv)
        return jnp.concatenate(cols, axis=1)

    def seg_step(s, carry):
        r0 = pl.multiple_of(s * SEG, SEG)
        xs = xa_v[pl.ds(r0, SEG), :].astype(F32)
        h = jnp.concatenate([mem_v[...], xs], axis=0)
        o_b = jnp.concatenate(
            [b_attend(pl.multiple_of(r0 + i * B_ROWS, B_ROWS)) for i in range(SEG // B_ROWS)],
            axis=0)

        def qkv_proj(p):
            return _dot(h, _unpack(wqkv_v[p]))

        def scores(y):
            q0, q1, q2 = (y[:, k * 128:(k + 1) * 128] for k in range(3))
            k0, k1, k2 = (y[:, (3 + k) * 128:(4 + k) * 128] for k in range(3))
            k2n = jnp.concatenate([jnp.where(lo, k2, 0.0), jnp.where(lo, 0.0, k2)], axis=0)
            sc = (_dot(q0, jnp.concatenate([k0, zblk], axis=0), NT)
                  + _dot(q1, jnp.concatenate([zblk, k1], axis=0), NT)
                  + _dot(q2, k2n, NT))
            return softmax_pair(sc)

        def pv(p, y, pr):
            v0, v1, v2 = (y[:, (6 + k) * 128:(7 + k) * 128] for k in range(3))
            v2n = jnp.concatenate([jnp.where(lo, v2, 0.0), jnp.where(lo, 0.0, v2)], axis=0)
            o_v[:, p * PAIR:p * PAIR + 128] = _dot(pr, jnp.concatenate([v0, zblk], axis=0))
            o_v[:, p * PAIR + 128:p * PAIR + 256] = _dot(pr, jnp.concatenate([zblk, v1], axis=0))
            o_v[:, p * PAIR + 256:p * PAIR + 384] = _dot(pr, v2n)

        def out_proj(p, acc):
            w = _unpack(woA_v[p])
            t = _dot(o_v[:, p * PAIR:(p + 1) * PAIR], w)
            return t if acc is None else acc + t

        ys, probs = {}, {}
        acc = None
        b = None
        wo_next = 0
        for i in range(NPAIR + 2):
            if i < NPAIR:
                ys[i] = qkv_proj(i)
            else:
                if b is None:
                    b = _dot(o_b, _unpack(woB_v[...]))
                for _ in range(2 if i == NPAIR else 3):
                    acc = out_proj(wo_next, acc)
                    wo_next += 1
            if 1 <= i <= NPAIR:
                probs[i - 1] = scores(ys[i - 1])
            if i >= 2:
                pv(i - 2, ys.pop(i - 2), probs.pop(i - 2))
        while wo_next < NPAIR:
            acc = out_proj(wo_next, acc)
            wo_next += 1
        mem_v[...] = acc[:M_A]
        a = acc[M_A:]
        g = jax.nn.sigmoid(jnp.sum(xs * gw_v[...].astype(F32), axis=1, keepdims=True))
        res = g * a + (1.0 - g) * b
        out_v[pl.ds(r0, SEG), :] = res.astype(BF16)
        pltpu.make_async_copy(out_v.at[pl.ds(r0, SEG), :], out_hbm.at[pl.ds(r0, SEG), :],
                              out_sem).start()
        return carry

    lax.fori_loop(0, S // SEG, seg_step, 0)
    pltpu.make_async_copy(out_v, out_hbm, out_sem).wait()


def pallas_gated_mix__memory_aug_recurrent_mem_tr__sliding_local_dilated__prompt_kernel(
    A_x, A_mem0, A_Wq, A_Wk, A_Wv, A_Wo, A_seg_len, B_x, B_wqkv, B_wo, gate_w,
):
    del B_x
    assert int(A_seg_len) == SEG
    hd = H_A * DH_A
    xa = A_x.reshape(S, D)
    mem0 = A_mem0.reshape(M_A, D)
    wqT = A_Wq.transpose(1, 2, 0).reshape(hd, D)
    wkT = A_Wk.transpose(1, 2, 0).reshape(hd, D)
    wvT = A_Wv.transpose(1, 2, 0).reshape(hd, D)
    woA = A_Wo.reshape(hd, D)
    gw = gate_w.reshape(1, D)

    scratch = [
        pltpu.VMEM((S, D), BF16),
        pltpu.VMEM((M_A, D), BF16),
        pltpu.VMEM((4, hd, D), BF16),
        pltpu.VMEM((NPAIR, D // 2, 9 * 128), jnp.uint32),
        pltpu.VMEM((NPAIR, PAIR // 2, D), jnp.uint32),
        pltpu.VMEM((D, 3 * D), BF16),
        pltpu.VMEM((D, D), BF16),
        pltpu.VMEM((D // 2, 3 * D), jnp.uint32),
        pltpu.VMEM((D // 2, D), jnp.uint32),
        pltpu.VMEM((1, D), BF16),
        pltpu.VMEM((5, S, 128), F32),
        pltpu.VMEM((5, HALO + S, 128), F32),
        pltpu.VMEM((5, HALO + S, 128), F32),
        pltpu.VMEM((M_A, D), F32),
        pltpu.VMEM((L, hd), F32),
        pltpu.VMEM((S, D), BF16),
        pltpu.SemaphoreType.DMA((5,)),
        pltpu.SemaphoreType.DMA((NPAIR,)),
        pltpu.SemaphoreType.DMA,
    ]
    out = pl.pallas_call(
        _kernel,
        out_shape=jax.ShapeDtypeStruct((S, D), BF16),
        in_specs=[pl.BlockSpec(memory_space=pl.ANY)] * 9,
        out_specs=pl.BlockSpec(memory_space=pl.ANY),
        scratch_shapes=scratch,
        compiler_params=pltpu.CompilerParams(vmem_limit_bytes=120 * 1024 * 1024),
    )(xa, mem0, wqT, wkT, wvT, woA, B_wqkv, B_wo, gw)
    return out.reshape(1, S, D)
```

```python
import functools

import jax
import jax.numpy as jnp
from jax import lax
import jax.experimental.pallas as pl
import jax.experimental.pallas.tpu as pltpu

F32 = jnp.float32
BF16 = jnp.bfloat16

S = 2048
D = 640
H_A, DH_A = 32, 192
M_A = 8
SEG = 32
L = M_A + SEG
NPAIR = H_A // 2
PAIR = 2 * DH_A
H_B, DH_B = 32, 20
WIN, DIL = 8, 2
HALO = 16
NEG = -1000000000.0

B_ROWS = 8
XPOSE_MXU = False
NSTEPS = S // SEG
UNROLL = 4
DMA_AHEAD = 3
VPU_START = 0
VPU_END = 20
VPU_FIRST = False

NT = (((1,), (1,)), ((), ()))
NN = (((1,), (0,)), ((), ()))


def _dot(a, b, dn=NN):
    return lax.dot_general(a, b, dn, preferred_element_type=F32)


def _pack(x):
    return pltpu.bitcast(x, jnp.uint32)


def _unpack(x):
    return pltpu.bitcast(x, BF16)


def _recip(d):
    r = pl.reciprocal(d, approx=True)
    return r * (2.0 - d * r)


def _kernel(xa_hbm, mem0_hbm, wqT_hbm, wkT_hbm, wvT_hbm, woA_hbm,
            wqkvB_hbm, woB_hbm, gw_hbm,
            out_hbm,
            xa_v, mem0_v, wT_v, wqkv_v, woA_v,
            wB_raw, woB_raw, w32, wBT_v, woB_v, gw_v,
            qB, kB, vB, oB, bmix,
            mem_v, o_v, out_v,
            sems, pair_sems, out_sem):
    cp_wB = pltpu.make_async_copy(wqkvB_hbm, wB_raw, sems.at[0])
    cp_xa = pltpu.make_async_copy(xa_hbm, xa_v, sems.at[1])
    cp_woB = pltpu.make_async_copy(woB_hbm, woB_raw, sems.at[2])
    cp_m0 = pltpu.make_async_copy(mem0_hbm, mem0_v, sems.at[3])
    cp_gw = pltpu.make_async_copy(gw_hbm, gw_v, sems.at[4])

    def pair_copies(p):
        r = pl.multiple_of(p * PAIR, 128)
        return [pltpu.make_async_copy(w.at[pl.ds(r, PAIR), :], wT_v.at[t, pl.ds(r, PAIR), :],
                                      pair_sems.at[p])
                for t, w in enumerate((wqT_hbm, wkT_hbm, wvT_hbm, woA_hbm))]

    for cp in (cp_wB, cp_woB, cp_xa, cp_m0, cp_gw):
        cp.start()
    for p in range(DMA_AHEAD):
        for cp in pair_copies(p):
            cp.start()

    def gather_rows(base, dst, dst_base):
        for d in range(DH_B):
            r = (dst_base + d * H_B) // 2
            for c in range(5):
                g = w32[c, pl.ds(base + d, H_B, stride=DH_B), :]
                dst[r:r + H_B // 2, c * 128:(c + 1) * 128] = _pack(g.astype(BF16))

    cp_wB.wait()
    for cb in range(15):
        for rb in range(5):
            tile = wB_raw[rb * 128:(rb + 1) * 128, cb * 128:(cb + 1) * 128]
            w32[rb, cb * 128:(cb + 1) * 128, :] = tile.T.astype(F32)
    for which in range(3):
        gather_rows(which * D, wBT_v, which * D)
    cp_woB.wait()
    for c in range(5):
        w32[c, 3 * D:4 * D, :] = woB_raw[:, c * 128:(c + 1) * 128].astype(F32)
    gather_rows(3 * D, woB_v, 0)

    zero_halo = jnp.zeros((HALO, 128), F32)
    for j in range(5):
        kB[j, 0:HALO, :] = zero_halo
        vB[j, 0:HALO, :] = zero_halo
    cp_xa.wait()

    rows_b = S // NPAIR
    scale_b = DH_B ** (-0.5)
    er = lax.broadcasted_iota(jnp.int32, (128, 128), 0)
    ec = lax.broadcasted_iota(jnp.int32, (128, 128), 1)
    eye = jnp.where(er == ec, 1.0, 0.0).astype(BF16)

    def b_attend(gr):
        pos = gr + lax.broadcasted_iota(jnp.int32, (B_ROWS, 128), 0)
        q = [qB[j, pl.ds(gr, B_ROWS), :] for j in range(5)]
        logits = []
        for w in range(WIN):
            s = q[0] * kB[0, pl.ds(HALO + gr - DIL * w, B_ROWS), :]
            for j in range(1, 5):
                s = s + q[j] * kB[j, pl.ds(HALO + gr - DIL * w, B_ROWS), :]
            s = s + pltpu.roll(s, 64, 1)
            s = s + pltpu.roll(s, 32, 1)
            logits.append(jnp.where(pos >= DIL * w, s * scale_b, NEG))
        m = logits[0]
        for w in range(1, WIN):
            m = jnp.maximum(m, logits[w])
        e = [jnp.exp(l - m) for l in logits]
        den = e[0]
        for w in range(1, WIN):
            den = den + e[w]
        inv = _recip(den)
        cols = []
        for j in range(5):
            acc = e[0] * vB[j, pl.ds(HALO + gr, B_ROWS), :]
            for w in range(1, WIN):
                acc = acc + e[w] * vB[j, pl.ds(HALO + gr - DIL * w, B_ROWS), :]
            cols.append(acc * inv)
        return jnp.concatenate(cols, axis=1)

    def b_project_tile(blk, n):
        r0 = pl.multiple_of(blk * rows_b, rows_b)
        t = _dot(xa_v[pl.ds(r0, rows_b), :], _unpack(wBT_v[n * 64:(n + 1) * 64, :]), NT)
        if n < 5:
            qB[n, pl.ds(r0, rows_b), :] = t
        elif n < 10:
            kB[n - 5, pl.ds(HALO + r0, rows_b), :] = t
        else:
            vB[n - 10, pl.ds(HALO + r0, rows_b), :] = t

    def b_out_tile(blk, slot, n):
        r0 = pl.multiple_of(blk * rows_b, rows_b)
        bmix[pl.ds(r0, rows_b), n * 128:(n + 1) * 128] = _dot(
            oB[slot], _unpack(woB_v[:, n * 128:(n + 1) * 128]))

    for n in range(15):
        b_project_tile(0, n)
    oB[...] = jnp.zeros(oB.shape, F32)

    def prologue_step(p, carry):
        @pl.when(p + DMA_AHEAD < NPAIR)
        def _():
            for cp in pair_copies(p + DMA_AHEAD):
                cp.start()

        for cp in pair_copies(p):
            cp.wait()
        r = pl.multiple_of(p * PAIR, 128)

        def pair_block(t, k):
            if k == 0:
                return wT_v[t, pl.ds(r, 128), :]
            if k == 1:
                return wT_v[t, pl.ds(r + 192, 128), :]
            return jnp.concatenate([wT_v[t, pl.ds(r + 128, 64), :],
                                    wT_v[t, pl.ds(r + 320, 64), :]], axis=0)

        def xpose_block(t, k):
            blk = pair_block(t, k)
            col = (t * 3 + k) * 128
            for j in range(5):
                tile = blk[:, j * 128:(j + 1) * 128]
                if XPOSE_MXU:
                    tt = _dot(eye, tile, NT).astype(BF16)
                else:
                    tt = tile.T
                wqkv_v[p, j * 64:(j + 1) * 64, col:col + 128] = _pack(tt)

        def repack_block(k):
            woA_v[p, k * 64:(k + 1) * 64, :] = _pack(pair_block(3, k))

        r0 = pl.multiple_of(p * rows_b, rows_b)

        def attend_block(i):
            oB[p % 2, i * B_ROWS:(i + 1) * B_ROWS, :] = b_attend(
                pl.multiple_of(r0 + i * B_ROWS, B_ROWS))

        prev_blk = jnp.maximum(p - 1, 0)
        next_blk = jnp.minimum(p + 1, NPAIR - 1)
        mxu = ([functools.partial(b_out_tile, prev_blk, (p + 1) % 2, n) for n in range(5)]
               + [functools.partial(b_project_tile, next_blk, n) for n in range(15)])
        xlu = ([functools.partial(xpose_block, t, k) for t in range(3) for k in range(3)]
               + [functools.partial(repack_block, k) for k in range(3)])
        vpu = [functools.partial(attend_block, i) for i in range(rows_b // B_ROWS)]
        n = len(mxu)
        nv = VPU_END - VPU_START
        for i in range(n):
            if not VPU_FIRST:
                mxu[i]()
            for u in xlu[i * len(xlu) // n:(i + 1) * len(xlu) // n]:
                u()
            if VPU_START <= i < VPU_END:
                k = i - VPU_START
                for u in vpu[k * len(vpu) // nv:(k + 1) * len(vpu) // nv]:
                    u()
            if VPU_FIRST:
                mxu[i]()
        return carry

    lax.fori_loop(0, NPAIR, prologue_step, 0)
    for n in range(5):
        b_out_tile(NPAIR - 1, (NPAIR - 1) % 2, n)

    cp_m0.wait()
    cp_gw.wait()
    mem_v[...] = mem0_v[...].astype(F32)

    scale_a = DH_A ** (-0.5)
    qi = lax.broadcasted_iota(jnp.int32, (L, 2 * L), 0)
    kl = lax.broadcasted_iota(jnp.int32, (L, 2 * L), 1)
    head_a = kl < L
    ki = jnp.where(head_a, kl, kl - L)
    mask = (qi < M_A) | (qi >= ki)
    lane = lax.broadcasted_iota(jnp.int32, (L, 128), 1)
    lo = lane < 64
    zblk = jnp.zeros((L, 128), F32)

    def softmax_pair(s):
        s = jnp.where(mask, s * scale_a, NEG)
        ma = jnp.max(jnp.where(head_a, s, -jnp.inf), axis=1, keepdims=True)
        mb = jnp.max(jnp.where(head_a, -jnp.inf, s), axis=1, keepdims=True)
        e = jnp.exp(s - jnp.where(head_a, ma, mb))
        da = jnp.sum(jnp.where(head_a, e, 0.0), axis=1, keepdims=True)
        db = jnp.sum(jnp.where(head_a, 0.0, e), axis=1, keepdims=True)
        return e * _recip(jnp.where(head_a, da, db))

    def segment(r0, mem):
        xs = xa_v[pl.ds(r0, SEG), :].astype(F32)
        h = [jnp.concatenate([mem[j], xs[:, j * 128:(j + 1) * 128]], axis=0) for j in range(5)]
        h_full = jnp.concatenate(h, axis=1)

        def qkv_proj(p):
            if p == 0:
                y = None
                for j in range(5):
                    t = _dot(h[j], _unpack(wqkv_v[p, j * 64:(j + 1) * 64, :]))
                    y = t if y is None else y + t
                return y
            return _dot(h_full, _unpack(wqkv_v[p]))

        def scores(y):
            q0, q1, q2 = (y[:, k * 128:(k + 1) * 128] for k in range(3))
            k0, k1, k2 = (y[:, (3 + k) * 128:(4 + k) * 128] for k in range(3))
            k2n = jnp.concatenate([jnp.where(lo, k2, 0.0), jnp.where(lo, 0.0, k2)], axis=0)
            sc = (_dot(q0, jnp.concatenate([k0, zblk], axis=0), NT)
                  + _dot(q1, jnp.concatenate([zblk, k1], axis=0), NT)
                  + _dot(q2, k2n, NT))
            return softmax_pair(sc)

        def pv(p, y, pr):
            v0, v1, v2 = (y[:, (6 + k) * 128:(7 + k) * 128] for k in range(3))
            v2n = jnp.concatenate([jnp.where(lo, v2, 0.0), jnp.where(lo, 0.0, v2)], axis=0)
            o_v[:, p * PAIR:p * PAIR + 128] = _dot(pr, jnp.concatenate([v0, zblk], axis=0))
            o_v[:, p * PAIR + 128:p * PAIR + 256] = _dot(pr, jnp.concatenate([zblk, v1], axis=0))
            o_v[:, p * PAIR + 256:p * PAIR + 384] = _dot(pr, v2n)

        def out_proj(p, acc):
            t = _dot(o_v[:, p * PAIR:(p + 1) * PAIR], _unpack(woA_v[p]))
            return t if acc is None else acc + t

        ys, probs = {}, {}
        acc = None
        wo_next = 0
        for i in range(NPAIR + 2):
            if i < NPAIR:
                ys[i] = qkv_proj(i)
            else:
                for _ in range(3):
                    acc = out_proj(wo_next, acc)
                    wo_next += 1
            if 1 <= i <= NPAIR:
                probs[i - 1] = scores(ys[i - 1])
            if i >= 2:
                pv(i - 2, ys.pop(i - 2), probs.pop(i - 2))
        n_tail = 2
        while wo_next < NPAIR - n_tail:
            acc = out_proj(wo_next, acc)
            wo_next += 1
        accs = []
        for j in range(5):
            t = acc[:, j * 128:(j + 1) * 128]
            for p in range(NPAIR - n_tail, NPAIR):
                t = t + _dot(o_v[:, p * PAIR:(p + 1) * PAIR],
                             _unpack(woA_v[p, :, j * 128:(j + 1) * 128]))
            accs.append(t)
        a = jnp.concatenate([t[M_A:] for t in accs], axis=1)
        g = jax.nn.sigmoid(jnp.sum(xs * gw_v[...].astype(F32), axis=1, keepdims=True))
        res = g * a + (1.0 - g) * bmix[pl.ds(r0, SEG), :]
        out_v[pl.ds(r0, SEG), :] = res.astype(BF16)
        return [t[:M_A] for t in accs]

    def seg_step(it, carry):
        rows = UNROLL * SEG
        base = pl.multiple_of(it * rows, rows)
        mem = [mem_v[:, j * 128:(j + 1) * 128] for j in range(5)]
        for u in range(UNROLL):
            mem = segment(pl.multiple_of(base + u * SEG, SEG), mem)
        for j in range(5):
            mem_v[:, j * 128:(j + 1) * 128] = mem[j]
        pltpu.make_async_copy(out_v.at[pl.ds(base, rows), :], out_hbm.at[pl.ds(base, rows), :],
                              out_sem).start()
        return carry

    lax.fori_loop(0, NSTEPS // UNROLL, seg_step, 0)
    pltpu.make_async_copy(out_v.at[pl.ds(0, NSTEPS * SEG), :], out_hbm.at[pl.ds(0, NSTEPS * SEG), :],
                          out_sem).wait()


def pallas_gated_mix__memory_aug_recurrent_mem_tr__sliding_local_dilated__prompt_kernel(
    A_x, A_mem0, A_Wq, A_Wk, A_Wv, A_Wo, A_seg_len, B_x, B_wqkv, B_wo, gate_w,
):
    del B_x
    assert int(A_seg_len) == SEG
    hd = H_A * DH_A
    xa = A_x.reshape(S, D)
    mem0 = A_mem0.reshape(M_A, D)
    wqT = A_Wq.transpose(1, 2, 0).reshape(hd, D)
    wkT = A_Wk.transpose(1, 2, 0).reshape(hd, D)
    wvT = A_Wv.transpose(1, 2, 0).reshape(hd, D)
    woA = A_Wo.reshape(hd, D)
    gw = gate_w.reshape(1, D)

    scratch = [
        pltpu.VMEM((S, D), BF16),
        pltpu.VMEM((M_A, D), BF16),
        pltpu.VMEM((4, hd, D), BF16),
        pltpu.VMEM((NPAIR, D // 2, 9 * 128), jnp.uint32),
        pltpu.VMEM((NPAIR, PAIR // 2, D), jnp.uint32),
        pltpu.VMEM((D, 3 * D), BF16),
        pltpu.VMEM((D, D), BF16),
        pltpu.VMEM((5, 4 * D + 32, 128), F32),
        pltpu.VMEM((3 * D // 2, D), jnp.uint32),
        pltpu.VMEM((D // 2, D), jnp.uint32),
        pltpu.VMEM((1, D), BF16),
        pltpu.VMEM((5, S, 128), F32),
        pltpu.VMEM((5, HALO + S, 128), F32),
        pltpu.VMEM((5, HALO + S, 128), F32),
        pltpu.VMEM((2, S // NPAIR, D), F32),
        pltpu.VMEM((S, D), F32),
        pltpu.VMEM((M_A, D), F32),
        pltpu.VMEM((L, hd), F32),
        pltpu.VMEM((S, D), BF16),
        pltpu.SemaphoreType.DMA((5,)),
        pltpu.SemaphoreType.DMA((NPAIR,)),
        pltpu.SemaphoreType.DMA,
    ]
    out = pl.pallas_call(
        _kernel,
        out_shape=jax.ShapeDtypeStruct((S, D), BF16),
        in_specs=[pl.BlockSpec(memory_space=pl.ANY)] * 9,
        out_specs=pl.BlockSpec(memory_space=pl.ANY),
        scratch_shapes=scratch,
        compiler_params=pltpu.CompilerParams(vmem_limit_bytes=120 * 1024 * 1024),
    )(xa, mem0, wqT, wkT, wvT, woA, B_wqkv, B_wo, gw)
    return out.reshape(1, S, D)
```

```python
import functools

import jax
import jax.numpy as jnp
from jax import lax
import jax.experimental.pallas as pl
import jax.experimental.pallas.tpu as pltpu

F32 = jnp.float32
BF16 = jnp.bfloat16

S = 2048
D = 640
H_A, DH_A = 32, 192
M_A = 8
SEG = 32
L = M_A + SEG
NPAIR = H_A // 2
PAIR = 2 * DH_A
H_B, DH_B = 32, 20
WIN, DIL = 8, 2
HALO = 16
NEG = -1000000000.0

B_ROWS = 8
XPOSE_MXU = False
NSTEPS = S // SEG
UNROLL = 4
NO_BOUNDS = True
XLU_START = 0
XLU_END = 6
VPU_START = 6
VPU_END = 20
LEAD = 2
LEAD_VS = 0
LEAD_VE = 20

NT = (((1,), (1,)), ((), ()))
NN = (((1,), (0,)), ((), ()))


def _dot(a, b, dn=NN):
    return lax.dot_general(a, b, dn, preferred_element_type=F32)


def _pack(x):
    return pltpu.bitcast(x, jnp.uint32)


def _unpack(x):
    return pltpu.bitcast(x, BF16)


def _recip(d):
    r = pl.reciprocal(d, approx=True)
    return r * (2.0 - d * r)


def _kernel(xa_hbm, mem0_hbm, wqT_hbm, wkT_hbm, wvT_hbm, woA_hbm,
            wqkvB_hbm, woB_hbm, gw_hbm,
            out_hbm,
            xa_v, mem0_v, wT_v, wqkv_v, woA_v,
            wB_raw, woB_raw, w32, wBT_v, woB_v, gw_v,
            xp, qB, kB, vB, oB0, oB1, bmix,
            mem_v, o_v, out_v,
            sems, pair_sems, out_sem):
    cp_wB = pltpu.make_async_copy(wqkvB_hbm, wB_raw, sems.at[0])
    cp_xa = pltpu.make_async_copy(xa_hbm, xa_v, sems.at[1])
    cp_woB = pltpu.make_async_copy(woB_hbm, woB_raw, sems.at[2])
    cp_m0 = pltpu.make_async_copy(mem0_hbm, mem0_v, sems.at[3])
    cp_gw = pltpu.make_async_copy(gw_hbm, gw_v, sems.at[4])

    def pair_copies(p):
        r = pl.multiple_of(p * PAIR, 128)
        return [pltpu.make_async_copy(w.at[pl.ds(r, PAIR), :], wT_v.at[t, pl.ds(r, PAIR), :],
                                      pair_sems.at[p])
                for t, w in enumerate((wqT_hbm, wkT_hbm, wvT_hbm, woA_hbm))]

    for cp in (cp_wB, cp_woB, cp_xa, cp_m0, cp_gw):
        cp.start()
    for p in range(NPAIR):
        for cp in pair_copies(p):
            cp.start()

    def gather_rows(base, dst, dst_base):
        for d in range(DH_B):
            r = (dst_base + d * H_B) // 2
            for c in range(5):
                g = w32[c, pl.ds(base + d, H_B, stride=DH_B), :]
                dst[r:r + H_B // 2, c * 128:(c + 1) * 128] = _pack(g.astype(BF16))

    cp_wB.wait()
    for cb in range(15):
        for rb in range(5):
            tile = wB_raw[rb * 128:(rb + 1) * 128, cb * 128:(cb + 1) * 128]
            w32[rb, cb * 128:(cb + 1) * 128, :] = tile.T.astype(F32)
    for which in range(3):
        gather_rows(which * D, wBT_v, which * D)
    cp_woB.wait()
    for c in range(5):
        w32[c, 3 * D:4 * D, :] = woB_raw[:, c * 128:(c + 1) * 128].astype(F32)
    gather_rows(3 * D, woB_v, 0)

    zero_halo = jnp.zeros((HALO, 128), F32)
    for j in range(5):
        kB[j, 0:HALO, :] = zero_halo
        vB[j, 0:HALO, :] = zero_halo
    cp_xa.wait()

    rows_b = S // NPAIR
    scale_b = DH_B ** (-0.5)
    er = lax.broadcasted_iota(jnp.int32, (128, 128), 0)
    ec = lax.broadcasted_iota(jnp.int32, (128, 128), 1)
    eye = jnp.where(er == ec, 1.0, 0.0).astype(BF16)

    def b_attend(gr):
        nsub = B_ROWS // 8
        offs = sorted({8 * i - DIL * w for i in range(nsub) for w in range(WIN)})

        def windows(ref, j):
            return {off: ref[j, pl.ds(HALO + gr + off, 8), :] for off in offs}

        def shifted(win, w):
            return jnp.concatenate([win[8 * i - DIL * w] for i in range(nsub)], axis=0)

        pos = gr + lax.broadcasted_iota(jnp.int32, (B_ROWS, 128), 0)
        part = [None] * WIN
        for j in range(5):
            q = qB[j, pl.ds(gr, B_ROWS), :]
            win = windows(kB, j)
            for w in range(WIN):
                t = q * shifted(win, w)
                part[w] = t if part[w] is None else part[w] + t
        logits = []
        for w in range(WIN):
            s = part[w]
            s = s + pltpu.roll(s, 64, 1)
            s = s + pltpu.roll(s, 32, 1)
            logits.append(jnp.where(pos >= DIL * w, s * scale_b, NEG))
        m = logits[0]
        for w in range(1, WIN):
            m = jnp.maximum(m, logits[w])
        e = [jnp.exp(l - m) for l in logits]
        den = e[0]
        for w in range(1, WIN):
            den = den + e[w]
        inv = _recip(den)
        cols = []
        for j in range(5):
            win = windows(vB, j)
            acc = e[0] * shifted(win, 0)
            for w in range(1, WIN):
                acc = acc + e[w] * shifted(win, w)
            cols.append(acc * inv)
        return jnp.concatenate(cols, axis=1)

    def _row0(blk):
        return blk * rows_b if isinstance(blk, int) else pl.multiple_of(blk * rows_b, rows_b)

    def b_pack_x(blk):
        r0 = _row0(blk)
        xp[...] = _pack(xa_v[pl.ds(r0, rows_b), :])

    def b_project_tile(blk, n):
        r0 = _row0(blk)
        t = _dot(_unpack(xp[...]), _unpack(wBT_v[n * 64:(n + 1) * 64, :]), NT)
        if n < 5:
            qB[n, pl.ds(r0, rows_b), :] = t
        elif n < 10:
            kB[n - 5, pl.ds(HALO + r0, rows_b), :] = t
        else:
            vB[n - 10, pl.ds(HALO + r0, rows_b), :] = t

    def b_out_tile(blk, slot, n):
        r0 = _row0(blk)
        bmix[pl.ds(r0, rows_b), n * 128:(n + 1) * 128] = _dot(
            oB[slot][...], _unpack(woB_v[:, n * 128:(n + 1) * 128]))

    def xlu_pieces(p):
        r = p * PAIR if isinstance(p, int) else pl.multiple_of(p * PAIR, 128)

        def pair_block(t, k):
            if k == 0:
                return wT_v[t, pl.ds(r, 128), :]
            if k == 1:
                return wT_v[t, pl.ds(r + 192, 128), :]
            return jnp.concatenate([wT_v[t, pl.ds(r + 128, 64), :],
                                    wT_v[t, pl.ds(r + 320, 64), :]], axis=0)

        def xpose_block(t, k):
            blk = pair_block(t, k)
            col = (t * 3 + k) * 128
            for j in range(5):
                tile = blk[:, j * 128:(j + 1) * 128]
                wqkv_v[p, j * 64:(j + 1) * 64, col:col + 128] = _pack(tile.T)

        def repack_block(k):
            woA_v[p, k * 64:(k + 1) * 64, :] = _pack(pair_block(3, k))

        return ([functools.partial(xpose_block, t, k) for t in range(3) for k in range(3)]
                + [functools.partial(repack_block, k) for k in range(3)])

    def b_step(attn_blk, attn_slot, out_blk, proj_blk, xlu, vpu_range=None):
        mxu, vpu = [], []
        if out_blk is not None:
            mxu += [functools.partial(b_out_tile, out_blk, 1 - attn_slot, n) for n in range(5)]
        if proj_blk is not None:
            b_pack_x(proj_blk)
            mxu += [functools.partial(b_project_tile, proj_blk, n) for n in range(15)]
        if attn_blk is not None:
            r0 = attn_blk * rows_b
            if not isinstance(r0, int):
                r0 = pl.multiple_of(r0, rows_b)

            def attend_block(i):
                gr = r0 + i * B_ROWS
                if not isinstance(gr, int):
                    gr = pl.multiple_of(gr, B_ROWS)
                oB[attn_slot][i * B_ROWS:(i + 1) * B_ROWS, :] = b_attend(gr)

            vpu = [functools.partial(attend_block, i) for i in range(rows_b // B_ROWS)]
        n = len(mxu)
        xs, xe = XLU_START * n // 20, XLU_END * n // 20
        vs, ve = vpu_range or (VPU_START, VPU_END)
        vs, ve = vs * n // 20, ve * n // 20
        for i in range(n):
            mxu[i]()
            if xs <= i < xe:
                k, c = i - xs, xe - xs
                for u in xlu[k * len(xlu) // c:(k + 1) * len(xlu) // c]:
                    u()
            if vs <= i < ve:
                k, c = i - vs, ve - vs
                for u in vpu[k * len(vpu) // c:(k + 1) * len(vpu) // c]:
                    u()

    def wait_pair(p):
        for cp in pair_copies(p):
            cp.wait()

    b_pack_x(0)
    for n in range(15):
        b_project_tile(0, n)
    oB = (oB0, oB1)
    oB1[...] = jnp.zeros(oB1.shape, F32)

    def lead_step(it, carry):
        for u in range(2):
            i = 2 * it + u
            b_step(i, u, jnp.maximum(i - 1, 0), i + 1, [], (LEAD_VS, LEAD_VE))
        return carry

    lax.fori_loop(0, LEAD // 2, lead_step, 0)

    def prologue_step(it, carry):
        for u in range(2):
            p = 2 * it + u
            wait_pair(p)
            b_step(p + LEAD, u, p + LEAD - 1, jnp.minimum(p + LEAD + 1, NPAIR - 1),
                   xlu_pieces(p))
        return carry

    lax.fori_loop(0, (NPAIR - LEAD) // 2, prologue_step, 0)
    for p in range(NPAIR - LEAD, NPAIR):
        wait_pair(p)
        if p == NPAIR - LEAD:
            b_step(None, 0, NPAIR - 1, None, xlu_pieces(p))
        else:
            for u in xlu_pieces(p):
                u()

    cp_m0.wait()
    cp_gw.wait()
    mem_v[...] = mem0_v[...].astype(F32)

    scale_a = DH_A ** (-0.5)
    qi = lax.broadcasted_iota(jnp.int32, (L, 2 * L), 0)
    kl = lax.broadcasted_iota(jnp.int32, (L, 2 * L), 1)
    head_a = kl < L
    ki = jnp.where(head_a, kl, kl - L)
    mask = (qi < M_A) | (qi >= ki)
    lane = lax.broadcasted_iota(jnp.int32, (L, 128), 1)
    lo = lane < 64
    zblk = jnp.zeros((L, 128), F32)

    def softmax_pair(s):
        s = jnp.where(mask, s * scale_a, NEG)
        ma = jnp.max(jnp.where(head_a, s, -jnp.inf), axis=1, keepdims=True)
        mb = jnp.max(jnp.where(head_a, -jnp.inf, s), axis=1, keepdims=True)
        e = jnp.exp(s - jnp.where(head_a, ma, mb))
        da = jnp.sum(jnp.where(head_a, e, 0.0), axis=1, keepdims=True)
        db = jnp.sum(jnp.where(head_a, 0.0, e), axis=1, keepdims=True)
        return e * _recip(jnp.where(head_a, da, db))

    def segment(r0, mem):
        xs = xa_v[pl.ds(r0, SEG), :].astype(F32)
        h = [jnp.concatenate([mem[j], xs[:, j * 128:(j + 1) * 128]], axis=0) for j in range(5)]
        h_full = jnp.concatenate(h, axis=1)

        def qkv_proj(p):
            if p == 0:
                y = None
                for j in range(5):
                    t = _dot(h[j], _unpack(wqkv_v[p, j * 64:(j + 1) * 64, :]))
                    y = t if y is None else y + t
                return y
            return _dot(h_full, _unpack(wqkv_v[p]))

        def scores(y):
            q0, q1, q2 = (y[:, k * 128:(k + 1) * 128] for k in range(3))
            k0, k1, k2 = (y[:, (3 + k) * 128:(4 + k) * 128] for k in range(3))
            k2n = jnp.concatenate([jnp.where(lo, k2, 0.0), jnp.where(lo, 0.0, k2)], axis=0)
            sc = (_dot(q0, jnp.concatenate([k0, zblk], axis=0), NT)
                  + _dot(q1, jnp.concatenate([zblk, k1], axis=0), NT)
                  + _dot(q2, k2n, NT))
            return softmax_pair(sc)

        def pv(p, y, pr):
            v0, v1, v2 = (y[:, (6 + k) * 128:(7 + k) * 128] for k in range(3))
            v2n = jnp.concatenate([jnp.where(lo, v2, 0.0), jnp.where(lo, 0.0, v2)], axis=0)
            o_v[:, p * PAIR:p * PAIR + 128] = _dot(pr, jnp.concatenate([v0, zblk], axis=0))
            o_v[:, p * PAIR + 128:p * PAIR + 256] = _dot(pr, jnp.concatenate([zblk, v1], axis=0))
            o_v[:, p * PAIR + 256:p * PAIR + 384] = _dot(pr, v2n)

        def out_proj(p, acc):
            t = _dot(o_v[:, p * PAIR:(p + 1) * PAIR], _unpack(woA_v[p]))
            return t if acc is None else acc + t

        ys, probs = {}, {}
        acc = None
        wo_next = 0
        for i in range(NPAIR + 2):
            if i < NPAIR:
                ys[i] = qkv_proj(i)
            else:
                for _ in range(3):
                    acc = out_proj(wo_next, acc)
                    wo_next += 1
            if 1 <= i <= NPAIR:
                probs[i - 1] = scores(ys[i - 1])
            if i >= 2:
                pv(i - 2, ys.pop(i - 2), probs.pop(i - 2))
        n_tail = 2
        while wo_next < NPAIR - n_tail:
            acc = out_proj(wo_next, acc)
            wo_next += 1
        accs = []
        for j in range(5):
            t = acc[:, j * 128:(j + 1) * 128]
            for p in range(NPAIR - n_tail, NPAIR):
                t = t + _dot(o_v[:, p * PAIR:(p + 1) * PAIR],
                             _unpack(woA_v[p, :, j * 128:(j + 1) * 128]))
            accs.append(t)
        a = jnp.concatenate([t[M_A:] for t in accs], axis=1)
        g = jax.nn.sigmoid(jnp.sum(xs * gw_v[...].astype(F32), axis=1, keepdims=True))
        res = g * a + (1.0 - g) * bmix[pl.ds(r0, SEG), :]
        out_v[pl.ds(r0, SEG), :] = res.astype(BF16)
        return [t[:M_A] for t in accs]

    def seg_step(it, carry):
        rows = UNROLL * SEG
        base = pl.multiple_of(it * rows, rows)
        mem = [mem_v[:, j * 128:(j + 1) * 128] for j in range(5)]
        for u in range(UNROLL):
            mem = segment(pl.multiple_of(base + u * SEG, SEG), mem)
        for j in range(5):
            mem_v[:, j * 128:(j + 1) * 128] = mem[j]
        pltpu.make_async_copy(out_v.at[pl.ds(base, rows), :], out_hbm.at[pl.ds(base, rows), :],
                              out_sem).start()
        return carry

    lax.fori_loop(0, NSTEPS // UNROLL, seg_step, 0)
    pltpu.make_async_copy(out_v.at[pl.ds(0, NSTEPS * SEG), :], out_hbm.at[pl.ds(0, NSTEPS * SEG), :],
                          out_sem).wait()


def pallas_gated_mix__memory_aug_recurrent_mem_tr__sliding_local_dilated__prompt_kernel(
    A_x, A_mem0, A_Wq, A_Wk, A_Wv, A_Wo, A_seg_len, B_x, B_wqkv, B_wo, gate_w,
):
    del B_x
    assert int(A_seg_len) == SEG
    hd = H_A * DH_A
    xa = A_x.reshape(S, D)
    mem0 = A_mem0.reshape(M_A, D)
    wqT = A_Wq.transpose(1, 2, 0).reshape(hd, D)
    wkT = A_Wk.transpose(1, 2, 0).reshape(hd, D)
    wvT = A_Wv.transpose(1, 2, 0).reshape(hd, D)
    woA = A_Wo.reshape(hd, D)
    gw = gate_w.reshape(1, D)

    scratch = [
        pltpu.VMEM((S, D), BF16),
        pltpu.VMEM((M_A, D), BF16),
        pltpu.VMEM((4, hd, D), BF16),
        pltpu.VMEM((NPAIR, D // 2, 9 * 128), jnp.uint32),
        pltpu.VMEM((NPAIR, PAIR // 2, D), jnp.uint32),
        pltpu.VMEM((D, 3 * D), BF16),
        pltpu.VMEM((D, D), BF16),
        pltpu.VMEM((5, 4 * D + 32, 128), F32),
        pltpu.VMEM((3 * D // 2, D), jnp.uint32),
        pltpu.VMEM((D // 2, D), jnp.uint32),
        pltpu.VMEM((1, D), BF16),
        pltpu.VMEM((S // NPAIR // 2, D), jnp.uint32),
        pltpu.VMEM((5, S, 128), F32),
        pltpu.VMEM((5, HALO + S, 128), F32),
        pltpu.VMEM((5, HALO + S, 128), F32),
        pltpu.VMEM((S // NPAIR, D), F32),
        pltpu.VMEM((S // NPAIR, D), F32),
        pltpu.VMEM((S, D), F32),
        pltpu.VMEM((M_A, D), F32),
        pltpu.VMEM((L, hd), F32),
        pltpu.VMEM((S, D), BF16),
        pltpu.SemaphoreType.DMA((5,)),
        pltpu.SemaphoreType.DMA((NPAIR,)),
        pltpu.SemaphoreType.DMA,
    ]
    out = pl.pallas_call(
        _kernel,
        out_shape=jax.ShapeDtypeStruct((S, D), BF16),
        in_specs=[pl.BlockSpec(memory_space=pl.ANY)] * 9,
        out_specs=pl.BlockSpec(memory_space=pl.ANY),
        scratch_shapes=scratch,
        compiler_params=pltpu.CompilerParams(vmem_limit_bytes=120 * 1024 * 1024,
                                             disable_bounds_checks=NO_BOUNDS),
    )(xa, mem0, wqT, wkT, wvT, woA, B_wqkv, B_wo, gw)
    return out.reshape(1, S, D)
```

```python
import functools

import jax
import jax.numpy as jnp
from jax import lax
import jax.experimental.pallas as pl
import jax.experimental.pallas.tpu as pltpu

F32 = jnp.float32
BF16 = jnp.bfloat16

S = 2048
D = 640
H_A, DH_A = 32, 192
M_A = 8
SEG = 32
L = M_A + SEG
NPAIR = H_A // 2
PAIR = 2 * DH_A
H_B, DH_B = 32, 20
WIN, DIL = 8, 2
HALO = 16
NEG = -1000000000.0

B_ROWS = 8
XPOSE_MXU = False
NSTEPS = S // SEG
UNROLL = 4
NO_BOUNDS = True
XLU_START = 0
XLU_END = 6
VPU_START = 6
VPU_END = 20
LEAD = 2
LEAD_VS = 0
LEAD_VE = 20

NT = (((1,), (1,)), ((), ()))
NN = (((1,), (0,)), ((), ()))


def _dot(a, b, dn=NN):
    return lax.dot_general(a, b, dn, preferred_element_type=F32)


def _pack(x):
    return pltpu.bitcast(x, jnp.uint32)


def _unpack(x):
    return pltpu.bitcast(x, BF16)


def _recip(d):
    r = pl.reciprocal(d, approx=True)
    return r * (2.0 - d * r)


def _kernel(xa_hbm, mem0_hbm, wqT_hbm, wkT_hbm, wvT_hbm, woA_hbm,
            wqkvB_hbm, woB_hbm, gw_hbm,
            out_hbm,
            xa_v, mem0_v, wT_v, wqkv_v, woA_v,
            wB_raw, woB_raw, w32, wBT_v, woB_v, gw_v,
            xp, qB, kB, vB, oB0, oB1, bmix,
            mem_v, o_v, out_v,
            sems, pair_sems, out_sem):
    cp_wB = pltpu.make_async_copy(wqkvB_hbm, wB_raw, sems.at[0])
    cp_xa = pltpu.make_async_copy(xa_hbm, xa_v, sems.at[1])
    cp_woB = pltpu.make_async_copy(woB_hbm, woB_raw, sems.at[2])
    cp_m0 = pltpu.make_async_copy(mem0_hbm, mem0_v, sems.at[3])
    cp_gw = pltpu.make_async_copy(gw_hbm, gw_v, sems.at[4])

    def pair_copies(p):
        r = pl.multiple_of(p * PAIR, 128)
        return [pltpu.make_async_copy(w.at[pl.ds(r, PAIR), :], wT_v.at[t, pl.ds(r, PAIR), :],
                                      pair_sems.at[p])
                for t, w in enumerate((wqT_hbm, wkT_hbm, wvT_hbm, woA_hbm))]

    for cp in (cp_wB, cp_woB, cp_xa, cp_m0, cp_gw):
        cp.start()

    def gather_rows(base, dst, dst_base):
        for d in range(DH_B):
            r = (dst_base + d * H_B) // 2
            for c in range(5):
                g = w32[c, pl.ds(base + d, H_B, stride=DH_B), :]
                dst[r:r + H_B // 2, c * 128:(c + 1) * 128] = _pack(g.astype(BF16))

    cp_wB.wait()
    for p in range(NPAIR):
        for cp in pair_copies(p):
            cp.start()
    for cb in range(15):
        for rb in range(5):
            tile = wB_raw[rb * 128:(rb + 1) * 128, cb * 128:(cb + 1) * 128]
            w32[rb, cb * 128:(cb + 1) * 128, :] = tile.T.astype(F32)
    for which in range(3):
        gather_rows(which * D, wBT_v, which * D)
    cp_woB.wait()
    for c in range(5):
        w32[c, 3 * D:4 * D, :] = woB_raw[:, c * 128:(c + 1) * 128].astype(F32)
    gather_rows(3 * D, woB_v, 0)

    zero_halo = jnp.zeros((HALO, 128), F32)
    for j in range(5):
        kB[j, 0:HALO, :] = zero_halo
        vB[j, 0:HALO, :] = zero_halo
    cp_xa.wait()

    rows_b = S // NPAIR
    scale_b = DH_B ** (-0.5)
    er = lax.broadcasted_iota(jnp.int32, (128, 128), 0)
    ec = lax.broadcasted_iota(jnp.int32, (128, 128), 1)
    eye = jnp.where(er == ec, 1.0, 0.0).astype(BF16)

    def b_attend(gr):
        nsub = B_ROWS // 8
        offs = sorted({8 * i - DIL * w for i in range(nsub) for w in range(WIN)})

        def windows(ref, j):
            return {off: ref[j, pl.ds(HALO + gr + off, 8), :] for off in offs}

        def shifted(win, w):
            return jnp.concatenate([win[8 * i - DIL * w] for i in range(nsub)], axis=0)

        pos = gr + lax.broadcasted_iota(jnp.int32, (B_ROWS, 128), 0)
        part = [None] * WIN
        for j in range(5):
            q = qB[j, pl.ds(gr, B_ROWS), :]
            win = windows(kB, j)
            for w in range(WIN):
                t = q * shifted(win, w)
                part[w] = t if part[w] is None else part[w] + t
        logits = []
        for w in range(WIN):
            s = part[w]
            s = s + pltpu.roll(s, 64, 1)
            s = s + pltpu.roll(s, 32, 1)
            logits.append(jnp.where(pos >= DIL * w, s * scale_b, NEG))
        m = logits[0]
        for w in range(1, WIN):
            m = jnp.maximum(m, logits[w])
        e = [jnp.exp(l - m) for l in logits]
        den = e[0]
        for w in range(1, WIN):
            den = den + e[w]
        inv = _recip(den)
        cols = []
        for j in range(5):
            win = windows(vB, j)
            acc = e[0] * shifted(win, 0)
            for w in range(1, WIN):
                acc = acc + e[w] * shifted(win, w)
            cols.append(acc * inv)
        return jnp.concatenate(cols, axis=1)

    def _row0(blk):
        return blk * rows_b if isinstance(blk, int) else pl.multiple_of(blk * rows_b, rows_b)

    def b_pack_x(blk):
        r0 = _row0(blk)
        xp[...] = _pack(xa_v[pl.ds(r0, rows_b), :])

    def b_project_tile(blk, n):
        r0 = _row0(blk)
        t = _dot(_unpack(xp[...]), _unpack(wBT_v[n * 64:(n + 1) * 64, :]), NT)
        if n < 5:
            qB[n, pl.ds(r0, rows_b), :] = t
        elif n < 10:
            kB[n - 5, pl.ds(HALO + r0, rows_b), :] = t
        else:
            vB[n - 10, pl.ds(HALO + r0, rows_b), :] = t

    def b_out_tile(blk, slot, n):
        r0 = _row0(blk)
        bmix[pl.ds(r0, rows_b), n * 128:(n + 1) * 128] = _dot(
            oB[slot][...], _unpack(woB_v[:, n * 128:(n + 1) * 128]))

    def xlu_pieces(p):
        r = p * PAIR if isinstance(p, int) else pl.multiple_of(p * PAIR, 128)

        def pair_block(t, k):
            if k == 0:
                return wT_v[t, pl.ds(r, 128), :]
            if k == 1:
                return wT_v[t, pl.ds(r + 192, 128), :]
            return jnp.concatenate([wT_v[t, pl.ds(r + 128, 64), :],
                                    wT_v[t, pl.ds(r + 320, 64), :]], axis=0)

        def xpose_block(t, k):
            blk = pair_block(t, k)
            col = (t * 3 + k) * 128
            for j in range(5):
                tile = blk[:, j * 128:(j + 1) * 128]
                wqkv_v[p, j * 64:(j + 1) * 64, col:col + 128] = _pack(tile.T)

        def repack_block(k):
            woA_v[p, k * 64:(k + 1) * 64, :] = _pack(pair_block(3, k))

        return ([functools.partial(xpose_block, t, k) for t in range(3) for k in range(3)]
                + [functools.partial(repack_block, k) for k in range(3)])

    def b_step(attn_blk, attn_slot, out_blk, proj_blk, xlu, vpu_range=None):
        mxu, vpu = [], []
        if out_blk is not None:
            mxu += [functools.partial(b_out_tile, out_blk, 1 - attn_slot, n) for n in range(5)]
        if proj_blk is not None:
            b_pack_x(proj_blk)
            mxu += [functools.partial(b_project_tile, proj_blk, n) for n in range(15)]
        if attn_blk is not None:
            r0 = attn_blk * rows_b
            if not isinstance(r0, int):
                r0 = pl.multiple_of(r0, rows_b)

            def attend_block(i):
                gr = r0 + i * B_ROWS
                if not isinstance(gr, int):
                    gr = pl.multiple_of(gr, B_ROWS)
                oB[attn_slot][i * B_ROWS:(i + 1) * B_ROWS, :] = b_attend(gr)

            vpu = [functools.partial(attend_block, i) for i in range(rows_b // B_ROWS)]
        n = len(mxu)
        xs, xe = XLU_START * n // 20, XLU_END * n // 20
        vs, ve = vpu_range or (VPU_START, VPU_END)
        vs, ve = vs * n // 20, ve * n // 20
        for i in range(n):
            mxu[i]()
            if xs <= i < xe:
                k, c = i - xs, xe - xs
                for u in xlu[k * len(xlu) // c:(k + 1) * len(xlu) // c]:
                    u()
            if vs <= i < ve:
                k, c = i - vs, ve - vs
                for u in vpu[k * len(vpu) // c:(k + 1) * len(vpu) // c]:
                    u()

    def wait_pair(p):
        for cp in pair_copies(p):
            cp.wait()

    b_pack_x(0)
    for n in range(15):
        b_project_tile(0, n)
    oB = (oB0, oB1)
    oB1[...] = jnp.zeros(oB1.shape, F32)

    def lead_step(it, carry):
        for u in range(2):
            i = 2 * it + u
            b_step(i, u, jnp.maximum(i - 1, 0), i + 1, [], (LEAD_VS, LEAD_VE))
        return carry

    lax.fori_loop(0, LEAD // 2, lead_step, 0)

    def prologue_step(it, carry):
        for u in range(2):
            p = 2 * it + u
            wait_pair(p)
            b_step(p + LEAD, u, p + LEAD - 1, jnp.minimum(p + LEAD + 1, NPAIR - 1),
                   xlu_pieces(p))
        return carry

    lax.fori_loop(0, (NPAIR - LEAD) // 2, prologue_step, 0)
    for p in range(NPAIR - LEAD, NPAIR):
        wait_pair(p)
        if p == NPAIR - LEAD:
            b_step(None, 0, NPAIR - 1, None, xlu_pieces(p))
        else:
            for u in xlu_pieces(p):
                u()

    cp_m0.wait()
    cp_gw.wait()
    mem_v[...] = mem0_v[...].astype(F32)

    scale_a = DH_A ** (-0.5)
    qi = lax.broadcasted_iota(jnp.int32, (L, 2 * L), 0)
    kl = lax.broadcasted_iota(jnp.int32, (L, 2 * L), 1)
    head_a = kl < L
    ki = jnp.where(head_a, kl, kl - L)
    mask = (qi < M_A) | (qi >= ki)
    lane = lax.broadcasted_iota(jnp.int32, (L, 128), 1)
    lo = lane < 64
    zblk = jnp.zeros((L, 128), F32)

    def softmax_pair(s):
        s = jnp.where(mask, s * scale_a, NEG)
        ma = jnp.max(jnp.where(head_a, s, -jnp.inf), axis=1, keepdims=True)
        mb = jnp.max(jnp.where(head_a, -jnp.inf, s), axis=1, keepdims=True)
        e = jnp.exp(s - jnp.where(head_a, ma, mb))
        da = jnp.sum(jnp.where(head_a, e, 0.0), axis=1, keepdims=True)
        db = jnp.sum(jnp.where(head_a, 0.0, e), axis=1, keepdims=True)
        return e * _recip(jnp.where(head_a, da, db))

    def segment(r0, mem):
        xs = xa_v[pl.ds(r0, SEG), :].astype(F32)
        h = [jnp.concatenate([mem[j], xs[:, j * 128:(j + 1) * 128]], axis=0) for j in range(5)]
        h_full = jnp.concatenate(h, axis=1)

        def qkv_proj(p):
            if p == 0:
                y = None
                for j in range(5):
                    t = _dot(h[j], _unpack(wqkv_v[p, j * 64:(j + 1) * 64, :]))
                    y = t if y is None else y + t
                return y
            return _dot(h_full, _unpack(wqkv_v[p]))

        def scores(y):
            q0, q1, q2 = (y[:, k * 128:(k + 1) * 128] for k in range(3))
            k0, k1, k2 = (y[:, (3 + k) * 128:(4 + k) * 128] for k in range(3))
            k2n = jnp.concatenate([jnp.where(lo, k2, 0.0), jnp.where(lo, 0.0, k2)], axis=0)
            sc = (_dot(q0, jnp.concatenate([k0, zblk], axis=0), NT)
                  + _dot(q1, jnp.concatenate([zblk, k1], axis=0), NT)
                  + _dot(q2, k2n, NT))
            return softmax_pair(sc)

        def pv(p, y, pr):
            v0, v1, v2 = (y[:, (6 + k) * 128:(7 + k) * 128] for k in range(3))
            v2n = jnp.concatenate([jnp.where(lo, v2, 0.0), jnp.where(lo, 0.0, v2)], axis=0)
            o_v[:, p * PAIR:p * PAIR + 128] = _dot(pr, jnp.concatenate([v0, zblk], axis=0))
            o_v[:, p * PAIR + 128:p * PAIR + 256] = _dot(pr, jnp.concatenate([zblk, v1], axis=0))
            o_v[:, p * PAIR + 256:p * PAIR + 384] = _dot(pr, v2n)

        def out_proj(p, acc):
            t = _dot(o_v[:, p * PAIR:(p + 1) * PAIR], _unpack(woA_v[p]))
            return t if acc is None else acc + t

        ys, probs = {}, {}
        acc = None
        wo_next = 0
        for i in range(NPAIR + 2):
            if i < NPAIR:
                ys[i] = qkv_proj(i)
            else:
                for _ in range(3):
                    acc = out_proj(wo_next, acc)
                    wo_next += 1
            if 1 <= i <= NPAIR:
                probs[i - 1] = scores(ys[i - 1])
            if i >= 2:
                pv(i - 2, ys.pop(i - 2), probs.pop(i - 2))
        n_tail = 2
        while wo_next < NPAIR - n_tail:
            acc = out_proj(wo_next, acc)
            wo_next += 1
        accs = []
        for j in range(5):
            t = acc[:, j * 128:(j + 1) * 128]
            for p in range(NPAIR - n_tail, NPAIR):
                t = t + _dot(o_v[:, p * PAIR:(p + 1) * PAIR],
                             _unpack(woA_v[p, :, j * 128:(j + 1) * 128]))
            accs.append(t)
        a = jnp.concatenate([t[M_A:] for t in accs], axis=1)
        gw = gw_v[...].astype(F32)
        gx = xs[:, 0:128] * gw[0:1, :]
        for j in range(1, 5):
            gx = gx + xs[:, j * 128:(j + 1) * 128] * gw[j:j + 1, :]
        g = jax.nn.sigmoid(jnp.sum(gx, axis=1, keepdims=True))
        res = g * a + (1.0 - g) * bmix[pl.ds(r0, SEG), :]
        out_v[pl.ds(r0, SEG), :] = res.astype(BF16)
        return [t[:M_A] for t in accs]

    def seg_step(it, carry):
        rows = UNROLL * SEG
        base = pl.multiple_of(it * rows, rows)
        mem = [mem_v[:, j * 128:(j + 1) * 128] for j in range(5)]
        for u in range(UNROLL):
            mem = segment(pl.multiple_of(base + u * SEG, SEG), mem)
        for j in range(5):
            mem_v[:, j * 128:(j + 1) * 128] = mem[j]
        pltpu.make_async_copy(out_v.at[pl.ds(base, rows), :], out_hbm.at[pl.ds(base, rows), :],
                              out_sem).start()
        return carry

    lax.fori_loop(0, NSTEPS // UNROLL, seg_step, 0)
    pltpu.make_async_copy(out_v.at[pl.ds(0, NSTEPS * SEG), :], out_hbm.at[pl.ds(0, NSTEPS * SEG), :],
                          out_sem).wait()


def pallas_gated_mix__memory_aug_recurrent_mem_tr__sliding_local_dilated__prompt_kernel(
    A_x, A_mem0, A_Wq, A_Wk, A_Wv, A_Wo, A_seg_len, B_x, B_wqkv, B_wo, gate_w,
):
    del B_x
    assert int(A_seg_len) == SEG
    hd = H_A * DH_A
    xa = A_x.reshape(S, D)
    mem0 = A_mem0.reshape(M_A, D)
    wqT = A_Wq.transpose(1, 2, 0).reshape(hd, D)
    wkT = A_Wk.transpose(1, 2, 0).reshape(hd, D)
    wvT = A_Wv.transpose(1, 2, 0).reshape(hd, D)
    woA = A_Wo.reshape(hd, D)
    gw = gate_w.reshape(5, 128)

    scratch = [
        pltpu.VMEM((S, D), BF16),
        pltpu.VMEM((M_A, D), BF16),
        pltpu.VMEM((4, hd, D), BF16),
        pltpu.VMEM((NPAIR, D // 2, 9 * 128), jnp.uint32),
        pltpu.VMEM((NPAIR, PAIR // 2, D), jnp.uint32),
        pltpu.VMEM((D, 3 * D), BF16),
        pltpu.VMEM((D, D), BF16),
        pltpu.VMEM((5, 4 * D + 32, 128), F32),
        pltpu.VMEM((3 * D // 2, D), jnp.uint32),
        pltpu.VMEM((D // 2, D), jnp.uint32),
        pltpu.VMEM((5, 128), BF16),
        pltpu.VMEM((S // NPAIR // 2, D), jnp.uint32),
        pltpu.VMEM((5, S, 128), F32),
        pltpu.VMEM((5, HALO + S, 128), F32),
        pltpu.VMEM((5, HALO + S, 128), F32),
        pltpu.VMEM((S // NPAIR, D), F32),
        pltpu.VMEM((S // NPAIR, D), F32),
        pltpu.VMEM((S, D), F32),
        pltpu.VMEM((M_A, D), F32),
        pltpu.VMEM((L, hd), F32),
        pltpu.VMEM((S, D), BF16),
        pltpu.SemaphoreType.DMA((5,)),
        pltpu.SemaphoreType.DMA((NPAIR,)),
        pltpu.SemaphoreType.DMA,
    ]
    out = pl.pallas_call(
        _kernel,
        out_shape=jax.ShapeDtypeStruct((S, D), BF16),
        in_specs=[pl.BlockSpec(memory_space=pl.ANY)] * 9,
        out_specs=pl.BlockSpec(memory_space=pl.ANY),
        scratch_shapes=scratch,
        compiler_params=pltpu.CompilerParams(vmem_limit_bytes=120 * 1024 * 1024,
                                             disable_bounds_checks=NO_BOUNDS),
    )(xa, mem0, wqT, wkT, wvT, woA, B_wqkv, B_wo, gw)
    return out.reshape(1, S, D)
```

```python
import functools

import jax
import jax.numpy as jnp
from jax import lax
import jax.experimental.pallas as pl
import jax.experimental.pallas.tpu as pltpu

F32 = jnp.float32
BF16 = jnp.bfloat16

S = 2048
D = 640
H_A, DH_A = 32, 192
M_A = 8
SEG = 32
L = M_A + SEG
NPAIR = H_A // 2
PAIR = 2 * DH_A
H_B, DH_B = 32, 20
WIN, DIL = 8, 2
HALO = 16
NEG = -1000000000.0

B_ROWS = 8
XPOSE_MXU = False
NSTEPS = S // SEG
UNROLL = 4
NO_BOUNDS = True
XLU_START = 0
XLU_END = 6
VPU_START = 6
VPU_END = 20
LEAD = 2
LEAD_VS = 0
LEAD_VE = 20

NT = (((1,), (1,)), ((), ()))
NN = (((1,), (0,)), ((), ()))


def _dot(a, b, dn=NN):
    return lax.dot_general(a, b, dn, preferred_element_type=F32)


def _pack(x):
    return pltpu.bitcast(x, jnp.uint32)


def _unpack(x):
    return pltpu.bitcast(x, BF16)


def _recip(d):
    r = pl.reciprocal(d, approx=True)
    return r * (2.0 - d * r)


def _kernel(xa_hbm, mem0_hbm, wqT_hbm, wkT_hbm, wvT_hbm, woA_hbm,
            wqkvB_hbm, woB_hbm, gw_hbm,
            out_hbm,
            xa_v, mem0_v, wT_v, wqkv_v, woA_v,
            wB_raw, woB_raw, w32, wBT_v, woB_v, gw_v,
            xp, qB, kB, vB, oB0, oB1, bmix,
            mem_v, o_v, out_v,
            sems, pair_sems, out_sem):
    XA_HEAD = 2 * (S // NPAIR)
    cp_wB = [pltpu.make_async_copy(wqkvB_hbm.at[:, j * D:(j + 1) * D],
                                   wB_raw.at[:, j * D:(j + 1) * D], sems.at[j]) for j in range(3)]
    cp_xa0 = pltpu.make_async_copy(xa_hbm.at[0:XA_HEAD, :], xa_v.at[0:XA_HEAD, :], sems.at[3])
    cp_woB = pltpu.make_async_copy(woB_hbm, woB_raw, sems.at[4])
    cp_xa1 = pltpu.make_async_copy(xa_hbm.at[XA_HEAD:S, :], xa_v.at[XA_HEAD:S, :], sems.at[5])
    cp_m0 = pltpu.make_async_copy(mem0_hbm, mem0_v, sems.at[6])
    cp_gw = pltpu.make_async_copy(gw_hbm, gw_v, sems.at[7])

    def pair_copies(p):
        r = pl.multiple_of(p * PAIR, 128)
        return [pltpu.make_async_copy(w.at[pl.ds(r, PAIR), :], wT_v.at[t, pl.ds(r, PAIR), :],
                                      pair_sems.at[p])
                for t, w in enumerate((wqT_hbm, wkT_hbm, wvT_hbm, woA_hbm))]

    for cp in cp_wB + [cp_xa0, cp_woB, cp_xa1, cp_m0, cp_gw]:
        cp.start()

    def gather_rows(base, dst, dst_base):
        for d in range(DH_B):
            r = (dst_base + d * H_B) // 2
            for c in range(5):
                g = w32[c, pl.ds(base + d, H_B, stride=DH_B), :]
                dst[r:r + H_B // 2, c * 128:(c + 1) * 128] = _pack(g.astype(BF16))

    for which in range(3):
        cp_wB[which].wait()
        if which == 0:
            for p in range(NPAIR):
                for cp in pair_copies(p):
                    cp.start()
        for cb in range(5 * which, 5 * which + 5):
            for rb in range(5):
                tile = wB_raw[rb * 128:(rb + 1) * 128, cb * 128:(cb + 1) * 128]
                w32[rb, cb * 128:(cb + 1) * 128, :] = tile.T.astype(F32)
        gather_rows(which * D, wBT_v, which * D)

    zero_halo = jnp.zeros((HALO, 128), F32)
    for j in range(5):
        kB[j, 0:HALO, :] = zero_halo
        vB[j, 0:HALO, :] = zero_halo

    rows_b = S // NPAIR
    scale_b = DH_B ** (-0.5)
    er = lax.broadcasted_iota(jnp.int32, (128, 128), 0)
    ec = lax.broadcasted_iota(jnp.int32, (128, 128), 1)
    eye = jnp.where(er == ec, 1.0, 0.0).astype(BF16)

    def b_attend(gr):
        nsub = B_ROWS // 8
        offs = sorted({8 * i - DIL * w for i in range(nsub) for w in range(WIN)})

        def windows(ref, j):
            return {off: ref[j, pl.ds(HALO + gr + off, 8), :] for off in offs}

        def shifted(win, w):
            return jnp.concatenate([win[8 * i - DIL * w] for i in range(nsub)], axis=0)

        pos = gr + lax.broadcasted_iota(jnp.int32, (B_ROWS, 128), 0)
        part = [None] * WIN
        for j in range(5):
            q = qB[j, pl.ds(gr, B_ROWS), :]
            win = windows(kB, j)
            for w in range(WIN):
                t = q * shifted(win, w)
                part[w] = t if part[w] is None else part[w] + t
        logits = []
        for w in range(WIN):
            s = part[w]
            s = s + pltpu.roll(s, 64, 1)
            s = s + pltpu.roll(s, 32, 1)
            logits.append(jnp.where(pos >= DIL * w, s * scale_b, NEG))
        m = logits[0]
        for w in range(1, WIN):
            m = jnp.maximum(m, logits[w])
        e = [jnp.exp(l - m) for l in logits]
        den = e[0]
        for w in range(1, WIN):
            den = den + e[w]
        inv = _recip(den)
        cols = []
        for j in range(5):
            win = windows(vB, j)
            acc = e[0] * shifted(win, 0)
            for w in range(1, WIN):
                acc = acc + e[w] * shifted(win, w)
            cols.append(acc * inv)
        return jnp.concatenate(cols, axis=1)

    def _row0(blk):
        return blk * rows_b if isinstance(blk, int) else pl.multiple_of(blk * rows_b, rows_b)

    def b_pack_x(blk):
        r0 = _row0(blk)
        xp[...] = _pack(xa_v[pl.ds(r0, rows_b), :])

    def b_project_tile(blk, n):
        r0 = _row0(blk)
        t = _dot(_unpack(xp[...]), _unpack(wBT_v[n * 64:(n + 1) * 64, :]), NT)
        if n < 5:
            qB[n, pl.ds(r0, rows_b), :] = t
        elif n < 10:
            kB[n - 5, pl.ds(HALO + r0, rows_b), :] = t
        else:
            vB[n - 10, pl.ds(HALO + r0, rows_b), :] = t

    def b_out_tile(blk, slot, n):
        r0 = _row0(blk)
        bmix[pl.ds(r0, rows_b), n * 128:(n + 1) * 128] = _dot(
            oB[slot][...], _unpack(woB_v[:, n * 128:(n + 1) * 128]))

    def xlu_pieces(p):
        r = p * PAIR if isinstance(p, int) else pl.multiple_of(p * PAIR, 128)

        def pair_block(t, k):
            if k == 0:
                return wT_v[t, pl.ds(r, 128), :]
            if k == 1:
                return wT_v[t, pl.ds(r + 192, 128), :]
            return jnp.concatenate([wT_v[t, pl.ds(r + 128, 64), :],
                                    wT_v[t, pl.ds(r + 320, 64), :]], axis=0)

        def xpose_block(t, k):
            blk = pair_block(t, k)
            col = (t * 3 + k) * 128
            for j in range(5):
                tile = blk[:, j * 128:(j + 1) * 128]
                wqkv_v[p, j * 64:(j + 1) * 64, col:col + 128] = _pack(tile.T)

        def repack_block(k):
            woA_v[p, k * 64:(k + 1) * 64, :] = _pack(pair_block(3, k))

        return ([functools.partial(xpose_block, t, k) for t in range(3) for k in range(3)]
                + [functools.partial(repack_block, k) for k in range(3)])

    def b_step(attn_blk, attn_slot, out_blk, proj_blk, xlu, vpu_range=None):
        mxu, vpu = [], []
        if out_blk is not None:
            mxu += [functools.partial(b_out_tile, out_blk, 1 - attn_slot, n) for n in range(5)]
        if proj_blk is not None:
            b_pack_x(proj_blk)
            mxu += [functools.partial(b_project_tile, proj_blk, n) for n in range(15)]
        if attn_blk is not None:
            r0 = attn_blk * rows_b
            if not isinstance(r0, int):
                r0 = pl.multiple_of(r0, rows_b)

            def attend_block(i):
                gr = r0 + i * B_ROWS
                if not isinstance(gr, int):
                    gr = pl.multiple_of(gr, B_ROWS)
                oB[attn_slot][i * B_ROWS:(i + 1) * B_ROWS, :] = b_attend(gr)

            vpu = [functools.partial(attend_block, i) for i in range(rows_b // B_ROWS)]
        n = len(mxu)
        xs, xe = XLU_START * n // 20, XLU_END * n // 20
        vs, ve = vpu_range or (VPU_START, VPU_END)
        vs, ve = vs * n // 20, ve * n // 20
        for i in range(n):
            mxu[i]()
            if xs <= i < xe:
                k, c = i - xs, xe - xs
                for u in xlu[k * len(xlu) // c:(k + 1) * len(xlu) // c]:
                    u()
            if vs <= i < ve:
                k, c = i - vs, ve - vs
                for u in vpu[k * len(vpu) // c:(k + 1) * len(vpu) // c]:
                    u()

    def wait_pair(p):
        for cp in pair_copies(p):
            cp.wait()

    oB = (oB0, oB1)
    cp_xa0.wait()
    b_pack_x(0)
    for n in range(15):
        b_project_tile(0, n)
    b_step(0, 0, None, 1, [], (LEAD_VS, LEAD_VE))
    cp_woB.wait()
    for c in range(5):
        w32[c, 3 * D:4 * D, :] = woB_raw[:, c * 128:(c + 1) * 128].astype(F32)
    gather_rows(3 * D, woB_v, 0)
    cp_xa1.wait()
    b_step(1, 1, 0, 2, [], (LEAD_VS, LEAD_VE))

    def prologue_step(it, carry):
        for u in range(2):
            p = 2 * it + u
            wait_pair(p)
            b_step(p + LEAD, u, p + LEAD - 1, jnp.minimum(p + LEAD + 1, NPAIR - 1),
                   xlu_pieces(p))
        return carry

    lax.fori_loop(0, (NPAIR - LEAD) // 2, prologue_step, 0)
    wait_pair(NPAIR - 2)
    b_step(None, 0, NPAIR - 1, None, xlu_pieces(NPAIR - 2))
    wait_pair(NPAIR - 1)
    for u in xlu_pieces(NPAIR - 1):
        u()

    cp_m0.wait()
    cp_gw.wait()
    mem_v[...] = mem0_v[...].astype(F32)

    scale_a = DH_A ** (-0.5)
    qi = lax.broadcasted_iota(jnp.int32, (L, 2 * L), 0)
    kl = lax.broadcasted_iota(jnp.int32, (L, 2 * L), 1)
    head_a = kl < L
    ki = jnp.where(head_a, kl, kl - L)
    mask = (qi < M_A) | (qi >= ki)
    lane = lax.broadcasted_iota(jnp.int32, (L, 128), 1)
    lo = lane < 64
    zblk = jnp.zeros((L, 128), F32)

    def softmax_pair(s):
        s = jnp.where(mask, s * scale_a, NEG)
        ma = jnp.max(jnp.where(head_a, s, -jnp.inf), axis=1, keepdims=True)
        mb = jnp.max(jnp.where(head_a, -jnp.inf, s), axis=1, keepdims=True)
        e = jnp.exp(s - jnp.where(head_a, ma, mb))
        da = jnp.sum(jnp.where(head_a, e, 0.0), axis=1, keepdims=True)
        db = jnp.sum(jnp.where(head_a, 0.0, e), axis=1, keepdims=True)
        return e * _recip(jnp.where(head_a, da, db))

    def segment(r0, mem):
        xs = xa_v[pl.ds(r0, SEG), :].astype(F32)
        h = [jnp.concatenate([mem[j], xs[:, j * 128:(j + 1) * 128]], axis=0) for j in range(5)]
        h_full = jnp.concatenate(h, axis=1)

        def qkv_proj(p):
            if p == 0:
                y = None
                for j in range(5):
                    t = _dot(h[j], _unpack(wqkv_v[p, j * 64:(j + 1) * 64, :]))
                    y = t if y is None else y + t
                return y
            return _dot(h_full, _unpack(wqkv_v[p]))

        def scores(y):
            q0, q1, q2 = (y[:, k * 128:(k + 1) * 128] for k in range(3))
            k0, k1, k2 = (y[:, (3 + k) * 128:(4 + k) * 128] for k in range(3))
            k2n = jnp.concatenate([jnp.where(lo, k2, 0.0), jnp.where(lo, 0.0, k2)], axis=0)
            sc = (_dot(q0, jnp.concatenate([k0, zblk], axis=0), NT)
                  + _dot(q1, jnp.concatenate([zblk, k1], axis=0), NT)
                  + _dot(q2, k2n, NT))
            return softmax_pair(sc)

        def pv(p, y, pr):
            v0, v1, v2 = (y[:, (6 + k) * 128:(7 + k) * 128] for k in range(3))
            v2n = jnp.concatenate([jnp.where(lo, v2, 0.0), jnp.where(lo, 0.0, v2)], axis=0)
            o_v[:, p * PAIR:p * PAIR + 128] = _dot(pr, jnp.concatenate([v0, zblk], axis=0))
            o_v[:, p * PAIR + 128:p * PAIR + 256] = _dot(pr, jnp.concatenate([zblk, v1], axis=0))
            o_v[:, p * PAIR + 256:p * PAIR + 384] = _dot(pr, v2n)

        def out_proj(p, acc):
            t = _dot(o_v[:, p * PAIR:(p + 1) * PAIR], _unpack(woA_v[p]))
            return t if acc is None else acc + t

        ys, probs = {}, {}
        acc = None
        wo_next = 0
        for i in range(NPAIR + 2):
            if i < NPAIR:
                ys[i] = qkv_proj(i)
            else:
                for _ in range(3):
                    acc = out_proj(wo_next, acc)
                    wo_next += 1
            if 1 <= i <= NPAIR:
                probs[i - 1] = scores(ys[i - 1])
            if i >= 2:
                pv(i - 2, ys.pop(i - 2), probs.pop(i - 2))
        n_tail = 2
        while wo_next < NPAIR - n_tail:
            acc = out_proj(wo_next, acc)
            wo_next += 1
        accs = []
        for j in range(5):
            t = acc[:, j * 128:(j + 1) * 128]
            for p in range(NPAIR - n_tail, NPAIR):
                t = t + _dot(o_v[:, p * PAIR:(p + 1) * PAIR],
                             _unpack(woA_v[p, :, j * 128:(j + 1) * 128]))
            accs.append(t)
        a = jnp.concatenate([t[M_A:] for t in accs], axis=1)
        gw = gw_v[...].astype(F32)
        gx = xs[:, 0:128] * gw[0:1, :]
        for j in range(1, 5):
            gx = gx + xs[:, j * 128:(j + 1) * 128] * gw[j:j + 1, :]
        g = jax.nn.sigmoid(jnp.sum(gx, axis=1, keepdims=True))
        res = g * a + (1.0 - g) * bmix[pl.ds(r0, SEG), :]
        out_v[pl.ds(r0, SEG), :] = res.astype(BF16)
        return [t[:M_A] for t in accs]

    def seg_step(it, carry):
        rows = UNROLL * SEG
        base = pl.multiple_of(it * rows, rows)
        mem = [mem_v[:, j * 128:(j + 1) * 128] for j in range(5)]
        for u in range(UNROLL):
            mem = segment(pl.multiple_of(base + u * SEG, SEG), mem)
        for j in range(5):
            mem_v[:, j * 128:(j + 1) * 128] = mem[j]
        pltpu.make_async_copy(out_v.at[pl.ds(base, rows), :], out_hbm.at[pl.ds(base, rows), :],
                              out_sem).start()
        return carry

    lax.fori_loop(0, NSTEPS // UNROLL, seg_step, 0)
    pltpu.make_async_copy(out_v.at[pl.ds(0, NSTEPS * SEG), :], out_hbm.at[pl.ds(0, NSTEPS * SEG), :],
                          out_sem).wait()


def pallas_gated_mix__memory_aug_recurrent_mem_tr__sliding_local_dilated__prompt_kernel(
    A_x, A_mem0, A_Wq, A_Wk, A_Wv, A_Wo, A_seg_len, B_x, B_wqkv, B_wo, gate_w,
):
    del B_x
    assert int(A_seg_len) == SEG
    hd = H_A * DH_A
    xa = A_x.reshape(S, D)
    mem0 = A_mem0.reshape(M_A, D)
    wqT = A_Wq.transpose(1, 2, 0).reshape(hd, D)
    wkT = A_Wk.transpose(1, 2, 0).reshape(hd, D)
    wvT = A_Wv.transpose(1, 2, 0).reshape(hd, D)
    woA = A_Wo.reshape(hd, D)
    gw = gate_w.reshape(5, 128)

    scratch = [
        pltpu.VMEM((S, D), BF16),
        pltpu.VMEM((M_A, D), BF16),
        pltpu.VMEM((4, hd, D), BF16),
        pltpu.VMEM((NPAIR, D // 2, 9 * 128), jnp.uint32),
        pltpu.VMEM((NPAIR, PAIR // 2, D), jnp.uint32),
        pltpu.VMEM((D, 3 * D), BF16),
        pltpu.VMEM((D, D), BF16),
        pltpu.VMEM((5, 4 * D + 32, 128), F32),
        pltpu.VMEM((3 * D // 2, D), jnp.uint32),
        pltpu.VMEM((D // 2, D), jnp.uint32),
        pltpu.VMEM((5, 128), BF16),
        pltpu.VMEM((S // NPAIR // 2, D), jnp.uint32),
        pltpu.VMEM((5, S, 128), F32),
        pltpu.VMEM((5, HALO + S, 128), F32),
        pltpu.VMEM((5, HALO + S, 128), F32),
        pltpu.VMEM((S // NPAIR, D), F32),
        pltpu.VMEM((S // NPAIR, D), F32),
        pltpu.VMEM((S, D), F32),
        pltpu.VMEM((M_A, D), F32),
        pltpu.VMEM((L, hd), F32),
        pltpu.VMEM((S, D), BF16),
        pltpu.SemaphoreType.DMA((8,)),
        pltpu.SemaphoreType.DMA((NPAIR,)),
        pltpu.SemaphoreType.DMA,
    ]
    out = pl.pallas_call(
        _kernel,
        out_shape=jax.ShapeDtypeStruct((S, D), BF16),
        in_specs=[pl.BlockSpec(memory_space=pl.ANY)] * 9,
        out_specs=pl.BlockSpec(memory_space=pl.ANY),
        scratch_shapes=scratch,
        compiler_params=pltpu.CompilerParams(vmem_limit_bytes=120 * 1024 * 1024,
                                             disable_bounds_checks=NO_BOUNDS),
    )(xa, mem0, wqT, wkT, wvT, woA, B_wqkv, B_wo, gw)
    return out.reshape(1, S, D)
```

```python
import functools

import jax
import jax.numpy as jnp
from jax import lax
import jax.experimental.pallas as pl
import jax.experimental.pallas.tpu as pltpu

F32 = jnp.float32
BF16 = jnp.bfloat16

S = 2048
D = 640
H_A, DH_A = 32, 192
M_A = 8
SEG = 32
L = M_A + SEG
NPAIR = H_A // 2
PAIR = 2 * DH_A
H_B, DH_B = 32, 20
WIN, DIL = 8, 2
HALO = 16
NEG = -1000000000.0

B_ROWS = 8
XPOSE_MXU = False
NSTEPS = S // SEG
UNROLL = 4
NO_BOUNDS = True
XLU_START = 0
XLU_END = 6
VPU_START = 6
VPU_END = 20
LEAD = 2
LEAD0_RANGE = (0, 20)
LEAD1_RANGE = (0, 20)

NT = (((1,), (1,)), ((), ()))
NN = (((1,), (0,)), ((), ()))


def _dot(a, b, dn=NN):
    return lax.dot_general(a, b, dn, preferred_element_type=F32)


def _pack(x):
    return pltpu.bitcast(x, jnp.uint32)


def _unpack(x):
    return pltpu.bitcast(x, BF16)


def _recip(d):
    r = pl.reciprocal(d, approx=True)
    return r * (2.0 - d * r)


def _kernel(xa_hbm, mem0_hbm, wqT_hbm, wkT_hbm, wvT_hbm, woA_hbm,
            wqkvB_hbm, woB_hbm, gw_hbm,
            out_hbm,
            xa_v, mem0_v, wT_v, wqkv_v, woA_v,
            wB_raw, woB_raw, w32, wBT_v, woB_v, gw_v,
            xp, qB, kB, vB, oB0, oB1, bmix,
            mem_v, o_v, out_v,
            sems, pair_sems, out_sem):
    XA_HEAD = 3 * (S // NPAIR)
    cp_wB = [pltpu.make_async_copy(wqkvB_hbm.at[:, j * D:(j + 1) * D],
                                   wB_raw.at[:, j * D:(j + 1) * D], sems.at[j]) for j in range(3)]
    cp_xa0 = pltpu.make_async_copy(xa_hbm.at[0:XA_HEAD, :], xa_v.at[0:XA_HEAD, :], sems.at[3])
    cp_woB = pltpu.make_async_copy(woB_hbm, woB_raw, sems.at[4])
    cp_xa1 = pltpu.make_async_copy(xa_hbm.at[XA_HEAD:S, :], xa_v.at[XA_HEAD:S, :], sems.at[5])
    cp_m0 = pltpu.make_async_copy(mem0_hbm, mem0_v, sems.at[6])
    cp_gw = pltpu.make_async_copy(gw_hbm, gw_v, sems.at[7])

    def pair_copies(p):
        r = pl.multiple_of(p * PAIR, 128)
        return [pltpu.make_async_copy(w.at[pl.ds(r, PAIR), :], wT_v.at[t, pl.ds(r, PAIR), :],
                                      pair_sems.at[p])
                for t, w in enumerate((wqT_hbm, wkT_hbm, wvT_hbm, woA_hbm))]

    for cp in cp_wB + [cp_xa0, cp_woB, cp_xa1, cp_m0, cp_gw]:
        cp.start()

    def gather_rows(base, dst, dst_base):
        for d in range(DH_B):
            r = (dst_base + d * H_B) // 2
            for c in range(5):
                g = w32[c, pl.ds(base + d, H_B, stride=DH_B), :]
                dst[r:r + H_B // 2, c * 128:(c + 1) * 128] = _pack(g.astype(BF16))

    for which in range(3):
        cp_wB[which].wait()
        if which == 0:
            for p in range(NPAIR):
                for cp in pair_copies(p):
                    cp.start()
        for cb in range(5 * which, 5 * which + 5):
            for rb in range(5):
                tile = wB_raw[rb * 128:(rb + 1) * 128, cb * 128:(cb + 1) * 128]
                w32[rb, cb * 128:(cb + 1) * 128, :] = tile.T.astype(F32)
        gather_rows(which * D, wBT_v, which * D)

    zero_halo = jnp.zeros((HALO, 128), F32)
    for j in range(5):
        kB[j, 0:HALO, :] = zero_halo
        vB[j, 0:HALO, :] = zero_halo

    rows_b = S // NPAIR
    scale_b = DH_B ** (-0.5)
    er = lax.broadcasted_iota(jnp.int32, (128, 128), 0)
    ec = lax.broadcasted_iota(jnp.int32, (128, 128), 1)
    eye = jnp.where(er == ec, 1.0, 0.0).astype(BF16)

    def b_attend(gr):
        nsub = B_ROWS // 8
        offs = sorted({8 * i - DIL * w for i in range(nsub) for w in range(WIN)})

        def windows(ref, j):
            return {off: ref[j, pl.ds(HALO + gr + off, 8), :] for off in offs}

        def shifted(win, w):
            return jnp.concatenate([win[8 * i - DIL * w] for i in range(nsub)], axis=0)

        pos = gr + lax.broadcasted_iota(jnp.int32, (B_ROWS, 128), 0)
        part = [None] * WIN
        for j in range(5):
            q = qB[j, pl.ds(gr, B_ROWS), :]
            win = windows(kB, j)
            for w in range(WIN):
                t = q * shifted(win, w)
                part[w] = t if part[w] is None else part[w] + t
        logits = []
        for w in range(WIN):
            s = part[w]
            s = s + pltpu.roll(s, 64, 1)
            s = s + pltpu.roll(s, 32, 1)
            logits.append(jnp.where(pos >= DIL * w, s * scale_b, NEG))
        m = logits[0]
        for w in range(1, WIN):
            m = jnp.maximum(m, logits[w])
        e = [jnp.exp(l - m) for l in logits]
        den = e[0]
        for w in range(1, WIN):
            den = den + e[w]
        inv = _recip(den)
        cols = []
        for j in range(5):
            win = windows(vB, j)
            acc = e[0] * shifted(win, 0)
            for w in range(1, WIN):
                acc = acc + e[w] * shifted(win, w)
            cols.append(acc * inv)
        return jnp.concatenate(cols, axis=1)

    def _row0(blk):
        return blk * rows_b if isinstance(blk, int) else pl.multiple_of(blk * rows_b, rows_b)

    def b_pack_x(blk):
        r0 = _row0(blk)
        xp[...] = _pack(xa_v[pl.ds(r0, rows_b), :])

    def b_project_tile(blk, n):
        r0 = _row0(blk)
        t = _dot(_unpack(xp[...]), _unpack(wBT_v[n * 64:(n + 1) * 64, :]), NT)
        if n < 5:
            qB[n, pl.ds(r0, rows_b), :] = t
        elif n < 10:
            kB[n - 5, pl.ds(HALO + r0, rows_b), :] = t
        else:
            vB[n - 10, pl.ds(HALO + r0, rows_b), :] = t

    def b_out_tile(blk, slot, n):
        r0 = _row0(blk)
        bmix[pl.ds(r0, rows_b), n * 128:(n + 1) * 128] = _dot(
            oB[slot][...], _unpack(woB_v[:, n * 128:(n + 1) * 128]))

    def xlu_pieces(p):
        r = p * PAIR if isinstance(p, int) else pl.multiple_of(p * PAIR, 128)

        def pair_block(t, k):
            if k == 0:
                return wT_v[t, pl.ds(r, 128), :]
            if k == 1:
                return wT_v[t, pl.ds(r + 192, 128), :]
            return jnp.concatenate([wT_v[t, pl.ds(r + 128, 64), :],
                                    wT_v[t, pl.ds(r + 320, 64), :]], axis=0)

        def xpose_block(t, k):
            blk = pair_block(t, k)
            col = (t * 3 + k) * 128
            for j in range(5):
                tile = blk[:, j * 128:(j + 1) * 128]
                wqkv_v[p, j * 64:(j + 1) * 64, col:col + 128] = _pack(tile.T)

        def repack_block(k):
            woA_v[p, k * 64:(k + 1) * 64, :] = _pack(pair_block(3, k))

        return ([functools.partial(xpose_block, t, k) for t in range(3) for k in range(3)]
                + [functools.partial(repack_block, k) for k in range(3)])

    def b_step(attn_blk, attn_slot, out_blk, proj_blk, xlu, vpu_range=None):
        mxu, vpu = [], []
        if out_blk is not None:
            mxu += [functools.partial(b_out_tile, out_blk, 1 - attn_slot, n) for n in range(5)]
        if proj_blk is not None:
            b_pack_x(proj_blk)
            mxu += [functools.partial(b_project_tile, proj_blk, n) for n in range(15)]
        if attn_blk is not None:
            r0 = attn_blk * rows_b
            if not isinstance(r0, int):
                r0 = pl.multiple_of(r0, rows_b)

            def attend_block(i):
                gr = r0 + i * B_ROWS
                if not isinstance(gr, int):
                    gr = pl.multiple_of(gr, B_ROWS)
                oB[attn_slot][i * B_ROWS:(i + 1) * B_ROWS, :] = b_attend(gr)

            vpu = [functools.partial(attend_block, i) for i in range(rows_b // B_ROWS)]
        n = len(mxu)
        xs, xe = XLU_START * n // 20, XLU_END * n // 20
        vs, ve = vpu_range or (VPU_START, VPU_END)
        vs, ve = vs * n // 20, ve * n // 20
        for i in range(n):
            mxu[i]()
            if xs <= i < xe:
                k, c = i - xs, xe - xs
                for u in xlu[k * len(xlu) // c:(k + 1) * len(xlu) // c]:
                    u()
            if vs <= i < ve:
                k, c = i - vs, ve - vs
                for u in vpu[k * len(vpu) // c:(k + 1) * len(vpu) // c]:
                    u()

    def wait_pair(p):
        for cp in pair_copies(p):
            cp.wait()

    oB = (oB0, oB1)
    cp_xa0.wait()
    b_pack_x(0)
    for n in range(15):
        b_project_tile(0, n)
    cp_woB.wait()
    for c in range(5):
        w32[c, 3 * D:4 * D, :] = woB_raw[:, c * 128:(c + 1) * 128].astype(F32)
    gather_rows(3 * D, woB_v, 0)
    b_step(0, 0, None, 1, [], LEAD0_RANGE)
    b_step(1, 1, 0, 2, [], LEAD1_RANGE)
    cp_xa1.wait()

    def prologue_step(it, carry):
        for u in range(2):
            p = 2 * it + u
            wait_pair(p)
            b_step(p + LEAD, u, p + LEAD - 1, jnp.minimum(p + LEAD + 1, NPAIR - 1),
                   xlu_pieces(p))
        return carry

    lax.fori_loop(0, (NPAIR - LEAD) // 2, prologue_step, 0)
    wait_pair(NPAIR - 2)
    b_step(None, 0, NPAIR - 1, None, xlu_pieces(NPAIR - 2))
    wait_pair(NPAIR - 1)
    for u in xlu_pieces(NPAIR - 1):
        u()

    cp_m0.wait()
    cp_gw.wait()
    mem_v[...] = mem0_v[...].astype(F32)

    scale_a = DH_A ** (-0.5)
    qi = lax.broadcasted_iota(jnp.int32, (L, 2 * L), 0)
    kl = lax.broadcasted_iota(jnp.int32, (L, 2 * L), 1)
    head_a = kl < L
    ki = jnp.where(head_a, kl, kl - L)
    mask = (qi < M_A) | (qi >= ki)
    lane = lax.broadcasted_iota(jnp.int32, (L, 128), 1)
    lo = lane < 64
    zblk = jnp.zeros((L, 128), F32)

    def softmax_pair(s):
        s = jnp.where(mask, s * scale_a, NEG)
        ma = jnp.max(jnp.where(head_a, s, -jnp.inf), axis=1, keepdims=True)
        mb = jnp.max(jnp.where(head_a, -jnp.inf, s), axis=1, keepdims=True)
        e = jnp.exp(s - jnp.where(head_a, ma, mb))
        da = jnp.sum(jnp.where(head_a, e, 0.0), axis=1, keepdims=True)
        db = jnp.sum(jnp.where(head_a, 0.0, e), axis=1, keepdims=True)
        return e * _recip(jnp.where(head_a, da, db))

    def segment(r0, mem):
        xs = xa_v[pl.ds(r0, SEG), :].astype(F32)
        h = [jnp.concatenate([mem[j], xs[:, j * 128:(j + 1) * 128]], axis=0) for j in range(5)]
        h_full = jnp.concatenate(h, axis=1)

        def qkv_proj(p):
            if p == 0:
                y = None
                for j in range(5):
                    t = _dot(h[j], _unpack(wqkv_v[p, j * 64:(j + 1) * 64, :]))
                    y = t if y is None else y + t
                return y
            return _dot(h_full, _unpack(wqkv_v[p]))

        def scores(y):
            q0, q1, q2 = (y[:, k * 128:(k + 1) * 128] for k in range(3))
            k0, k1, k2 = (y[:, (3 + k) * 128:(4 + k) * 128] for k in range(3))
            k2n = jnp.concatenate([jnp.where(lo, k2, 0.0), jnp.where(lo, 0.0, k2)], axis=0)
            sc = (_dot(q0, jnp.concatenate([k0, zblk], axis=0), NT)
                  + _dot(q1, jnp.concatenate([zblk, k1], axis=0), NT)
                  + _dot(q2, k2n, NT))
            return softmax_pair(sc)

        def pv(p, y, pr):
            v0, v1, v2 = (y[:, (6 + k) * 128:(7 + k) * 128] for k in range(3))
            v2n = jnp.concatenate([jnp.where(lo, v2, 0.0), jnp.where(lo, 0.0, v2)], axis=0)
            o_v[:, p * PAIR:p * PAIR + 128] = _dot(pr, jnp.concatenate([v0, zblk], axis=0))
            o_v[:, p * PAIR + 128:p * PAIR + 256] = _dot(pr, jnp.concatenate([zblk, v1], axis=0))
            o_v[:, p * PAIR + 256:p * PAIR + 384] = _dot(pr, v2n)

        def out_proj(p, acc):
            t = _dot(o_v[:, p * PAIR:(p + 1) * PAIR], _unpack(woA_v[p]))
            return t if acc is None else acc + t

        ys, probs = {}, {}
        acc = None
        wo_next = 0
        for i in range(NPAIR + 2):
            if i < NPAIR:
                ys[i] = qkv_proj(i)
            else:
                for _ in range(3):
                    acc = out_proj(wo_next, acc)
                    wo_next += 1
            if 1 <= i <= NPAIR:
                probs[i - 1] = scores(ys[i - 1])
            if i >= 2:
                pv(i - 2, ys.pop(i - 2), probs.pop(i - 2))
        n_tail = 2
        while wo_next < NPAIR - n_tail:
            acc = out_proj(wo_next, acc)
            wo_next += 1
        accs = []
        for j in range(5):
            t = acc[:, j * 128:(j + 1) * 128]
            for p in range(NPAIR - n_tail, NPAIR):
                t = t + _dot(o_v[:, p * PAIR:(p + 1) * PAIR],
                             _unpack(woA_v[p, :, j * 128:(j + 1) * 128]))
            accs.append(t)
        a = jnp.concatenate([t[M_A:] for t in accs], axis=1)
        gw = gw_v[...].astype(F32)
        gx = xs[:, 0:128] * gw[0:1, :]
        for j in range(1, 5):
            gx = gx + xs[:, j * 128:(j + 1) * 128] * gw[j:j + 1, :]
        g = jax.nn.sigmoid(jnp.sum(gx, axis=1, keepdims=True))
        res = g * a + (1.0 - g) * bmix[pl.ds(r0, SEG), :]
        out_v[pl.ds(r0, SEG), :] = res.astype(BF16)
        return [t[:M_A] for t in accs]

    def seg_step(it, carry):
        rows = UNROLL * SEG
        base = pl.multiple_of(it * rows, rows)
        mem = [mem_v[:, j * 128:(j + 1) * 128] for j in range(5)]
        for u in range(UNROLL):
            mem = segment(pl.multiple_of(base + u * SEG, SEG), mem)
        for j in range(5):
            mem_v[:, j * 128:(j + 1) * 128] = mem[j]
        pltpu.make_async_copy(out_v.at[pl.ds(base, rows), :], out_hbm.at[pl.ds(base, rows), :],
                              out_sem).start()
        return carry

    lax.fori_loop(0, NSTEPS // UNROLL, seg_step, 0)
    pltpu.make_async_copy(out_v.at[pl.ds(0, NSTEPS * SEG), :], out_hbm.at[pl.ds(0, NSTEPS * SEG), :],
                          out_sem).wait()


def pallas_gated_mix__memory_aug_recurrent_mem_tr__sliding_local_dilated__prompt_kernel(
    A_x, A_mem0, A_Wq, A_Wk, A_Wv, A_Wo, A_seg_len, B_x, B_wqkv, B_wo, gate_w,
):
    del B_x
    assert int(A_seg_len) == SEG
    hd = H_A * DH_A
    xa = A_x.reshape(S, D)
    mem0 = A_mem0.reshape(M_A, D)
    wqT = A_Wq.transpose(1, 2, 0).reshape(hd, D)
    wkT = A_Wk.transpose(1, 2, 0).reshape(hd, D)
    wvT = A_Wv.transpose(1, 2, 0).reshape(hd, D)
    woA = A_Wo.reshape(hd, D)
    gw = gate_w.reshape(5, 128)

    scratch = [
        pltpu.VMEM((S, D), BF16),
        pltpu.VMEM((M_A, D), BF16),
        pltpu.VMEM((4, hd, D), BF16),
        pltpu.VMEM((NPAIR, D // 2, 9 * 128), jnp.uint32),
        pltpu.VMEM((NPAIR, PAIR // 2, D), jnp.uint32),
        pltpu.VMEM((D, 3 * D), BF16),
        pltpu.VMEM((D, D), BF16),
        pltpu.VMEM((5, 4 * D + 32, 128), F32),
        pltpu.VMEM((3 * D // 2, D), jnp.uint32),
        pltpu.VMEM((D // 2, D), jnp.uint32),
        pltpu.VMEM((5, 128), BF16),
        pltpu.VMEM((S // NPAIR // 2, D), jnp.uint32),
        pltpu.VMEM((5, S, 128), F32),
        pltpu.VMEM((5, HALO + S, 128), F32),
        pltpu.VMEM((5, HALO + S, 128), F32),
        pltpu.VMEM((S // NPAIR, D), F32),
        pltpu.VMEM((S // NPAIR, D), F32),
        pltpu.VMEM((S, D), F32),
        pltpu.VMEM((M_A, D), F32),
        pltpu.VMEM((L, hd), F32),
        pltpu.VMEM((S, D), BF16),
        pltpu.SemaphoreType.DMA((8,)),
        pltpu.SemaphoreType.DMA((NPAIR,)),
        pltpu.SemaphoreType.DMA,
    ]
    out = pl.pallas_call(
        _kernel,
        out_shape=jax.ShapeDtypeStruct((S, D), BF16),
        in_specs=[pl.BlockSpec(memory_space=pl.ANY)] * 9,
        out_specs=pl.BlockSpec(memory_space=pl.ANY),
        scratch_shapes=scratch,
        compiler_params=pltpu.CompilerParams(vmem_limit_bytes=120 * 1024 * 1024,
                                             disable_bounds_checks=NO_BOUNDS),
    )(xa, mem0, wqT, wkT, wvT, woA, B_wqkv, B_wo, gw)
    return out.reshape(1, S, D)
```

```python
import functools

import jax
import jax.numpy as jnp
from jax import lax
import jax.experimental.pallas as pl
import jax.experimental.pallas.tpu as pltpu

F32 = jnp.float32
BF16 = jnp.bfloat16

S = 2048
D = 640
H_A, DH_A = 32, 192
M_A = 8
SEG = 32
L = M_A + SEG
NPAIR = H_A // 2
PAIR = 2 * DH_A
H_B, DH_B = 32, 20
WIN, DIL = 8, 2
HALO = 16
NEG = -1000000000.0

B_ROWS = 8
NSTEPS = S // SEG
UNROLL = 4
NO_BOUNDS = True
XLU_START = 0
XLU_END = 6
VPU_START = 6
VPU_END = 20
LEAD = 2
LEAD0_RANGE = (0, 20)
LEAD1_RANGE = (0, 20)

NT = (((1,), (1,)), ((), ()))
NN = (((1,), (0,)), ((), ()))


def _dot(a, b, dn=NN):
    return lax.dot_general(a, b, dn, preferred_element_type=F32)


def _pack(x):
    return pltpu.bitcast(x, jnp.uint32)


def _unpack(x):
    return pltpu.bitcast(x, BF16)


def _recip(d):
    r = pl.reciprocal(d, approx=True)
    return r * (2.0 - d * r)


def _kernel(xa_hbm, mem0_hbm, wqT_hbm, wkT_hbm, wvT_hbm, woA_hbm,
            wqkvB_hbm, woB_hbm, gw_hbm,
            out_hbm,
            xa_v, mem0_v, wT_v, wqkv_v, woA_v,
            wB_raw, woB_raw, w32, wBT_v, woB_v, gw_v,
            xp, qB, kB, vB, oB0, oB1, bmix,
            mem_v, o_v, out_v,
            sems, pair_sems, out_sem):
    XA_HEAD = 3 * (S // NPAIR)
    cp_wB = [pltpu.make_async_copy(wqkvB_hbm.at[:, j * D:(j + 1) * D],
                                   wB_raw.at[:, j * D:(j + 1) * D], sems.at[j]) for j in range(3)]
    cp_xa0 = pltpu.make_async_copy(xa_hbm.at[0:XA_HEAD, :], xa_v.at[0:XA_HEAD, :], sems.at[3])
    cp_woB = pltpu.make_async_copy(woB_hbm, woB_raw, sems.at[4])
    cp_xa1 = pltpu.make_async_copy(xa_hbm.at[XA_HEAD:S, :], xa_v.at[XA_HEAD:S, :], sems.at[5])
    cp_m0 = pltpu.make_async_copy(mem0_hbm, mem0_v, sems.at[6])
    cp_gw = pltpu.make_async_copy(gw_hbm, gw_v, sems.at[7])

    def pair_copies(p):
        r = pl.multiple_of(p * PAIR, 128)
        return [pltpu.make_async_copy(w.at[pl.ds(r, PAIR), :], wT_v.at[t, pl.ds(r, PAIR), :],
                                      pair_sems.at[p])
                for t, w in enumerate((wqT_hbm, wkT_hbm, wvT_hbm, woA_hbm))]

    for cp in cp_wB + [cp_xa0, cp_woB, cp_xa1, cp_m0, cp_gw]:
        cp.start()

    def gather_rows(base, dst, dst_base):
        for d in range(DH_B):
            r = (dst_base + d * H_B) // 2
            for c in range(5):
                g = w32[c, pl.ds(base + d, H_B, stride=DH_B), :]
                dst[r:r + H_B // 2, c * 128:(c + 1) * 128] = _pack(g.astype(BF16))

    for which in range(3):
        cp_wB[which].wait()
        if which == 0:
            for p in range(NPAIR):
                for cp in pair_copies(p):
                    cp.start()
        for cb in range(5 * which, 5 * which + 5):
            for rb in range(5):
                tile = wB_raw[rb * 128:(rb + 1) * 128, cb * 128:(cb + 1) * 128]
                w32[rb, cb * 128:(cb + 1) * 128, :] = tile.T.astype(F32)
        gather_rows(which * D, wBT_v, which * D)

    zero_halo = jnp.zeros((HALO, 128), F32)
    for j in range(5):
        kB[j, 0:HALO, :] = zero_halo
        vB[j, 0:HALO, :] = zero_halo

    rows_b = S // NPAIR
    scale_b = DH_B ** (-0.5)

    def b_attend(gr):
        nsub = B_ROWS // 8
        offs = sorted({8 * i - DIL * w for i in range(nsub) for w in range(WIN)})

        def windows(ref, j):
            return {off: ref[j, pl.ds(HALO + gr + off, 8), :] for off in offs}

        def shifted(win, w):
            return jnp.concatenate([win[8 * i - DIL * w] for i in range(nsub)], axis=0)

        pos = gr + lax.broadcasted_iota(jnp.int32, (B_ROWS, 128), 0)
        part = [None] * WIN
        for j in range(5):
            q = qB[j, pl.ds(gr, B_ROWS), :]
            win = windows(kB, j)
            for w in range(WIN):
                t = q * shifted(win, w)
                part[w] = t if part[w] is None else part[w] + t
        logits = []
        for w in range(WIN):
            s = part[w]
            s = s + pltpu.roll(s, 64, 1)
            s = s + pltpu.roll(s, 32, 1)
            logits.append(jnp.where(pos >= DIL * w, s * scale_b, NEG))
        m = logits[0]
        for w in range(1, WIN):
            m = jnp.maximum(m, logits[w])
        e = [jnp.exp(l - m) for l in logits]
        den = e[0]
        for w in range(1, WIN):
            den = den + e[w]
        inv = _recip(den)
        cols = []
        for j in range(5):
            win = windows(vB, j)
            acc = e[0] * shifted(win, 0)
            for w in range(1, WIN):
                acc = acc + e[w] * shifted(win, w)
            cols.append(acc * inv)
        return jnp.concatenate(cols, axis=1)

    def _row0(blk):
        return blk * rows_b if isinstance(blk, int) else pl.multiple_of(blk * rows_b, rows_b)

    def b_pack_x(blk):
        r0 = _row0(blk)
        xp[...] = _pack(xa_v[pl.ds(r0, rows_b), :])

    def b_project_tile(blk, n):
        r0 = _row0(blk)
        t = _dot(_unpack(xp[...]), _unpack(wBT_v[n * 64:(n + 1) * 64, :]), NT)
        if n < 5:
            qB[n, pl.ds(r0, rows_b), :] = t
        elif n < 10:
            kB[n - 5, pl.ds(HALO + r0, rows_b), :] = t
        else:
            vB[n - 10, pl.ds(HALO + r0, rows_b), :] = t

    def b_out_tile(blk, slot, n):
        r0 = _row0(blk)
        bmix[pl.ds(r0, rows_b), n * 128:(n + 1) * 128] = _dot(
            oB[slot][...], _unpack(woB_v[:, n * 128:(n + 1) * 128]))

    def xlu_pieces(p):
        r = p * PAIR if isinstance(p, int) else pl.multiple_of(p * PAIR, 128)

        def pair_block(t, k):
            if k == 0:
                return wT_v[t, pl.ds(r, 128), :]
            if k == 1:
                return wT_v[t, pl.ds(r + 192, 128), :]
            return jnp.concatenate([wT_v[t, pl.ds(r + 128, 64), :],
                                    wT_v[t, pl.ds(r + 320, 64), :]], axis=0)

        def xpose_block(t, k):
            blk = pair_block(t, k)
            col = (t * 3 + k) * 128
            for j in range(5):
                tile = blk[:, j * 128:(j + 1) * 128]
                wqkv_v[p, j * 64:(j + 1) * 64, col:col + 128] = _pack(tile.T)

        def repack_block(k):
            woA_v[p, k * 64:(k + 1) * 64, :] = _pack(pair_block(3, k))

        return ([functools.partial(xpose_block, t, k) for t in range(3) for k in range(3)]
                + [functools.partial(repack_block, k) for k in range(3)])

    def b_step(attn_blk, attn_slot, out_blk, proj_blk, xlu, vpu_range=None):
        mxu, vpu = [], []
        if out_blk is not None:
            mxu += [functools.partial(b_out_tile, out_blk, 1 - attn_slot, n) for n in range(5)]
        if proj_blk is not None:
            b_pack_x(proj_blk)
            mxu += [functools.partial(b_project_tile, proj_blk, n) for n in range(15)]
        if attn_blk is not None:
            r0 = attn_blk * rows_b
            if not isinstance(r0, int):
                r0 = pl.multiple_of(r0, rows_b)

            def attend_block(i):
                gr = r0 + i * B_ROWS
                if not isinstance(gr, int):
                    gr = pl.multiple_of(gr, B_ROWS)
                oB[attn_slot][i * B_ROWS:(i + 1) * B_ROWS, :] = b_attend(gr)

            vpu = [functools.partial(attend_block, i) for i in range(rows_b // B_ROWS)]
        n = len(mxu)
        xs, xe = XLU_START * n // 20, XLU_END * n // 20
        vs, ve = vpu_range or (VPU_START, VPU_END)
        vs, ve = vs * n // 20, ve * n // 20
        for i in range(n):
            mxu[i]()
            if xs <= i < xe:
                k, c = i - xs, xe - xs
                for u in xlu[k * len(xlu) // c:(k + 1) * len(xlu) // c]:
                    u()
            if vs <= i < ve:
                k, c = i - vs, ve - vs
                for u in vpu[k * len(vpu) // c:(k + 1) * len(vpu) // c]:
                    u()

    def wait_pair(p):
        for cp in pair_copies(p):
            cp.wait()

    oB = (oB0, oB1)
    cp_xa0.wait()
    b_pack_x(0)
    for n in range(15):
        b_project_tile(0, n)
    cp_woB.wait()
    for c in range(5):
        w32[c, 3 * D:4 * D, :] = woB_raw[:, c * 128:(c + 1) * 128].astype(F32)
    gather_rows(3 * D, woB_v, 0)
    b_step(0, 0, None, 1, [], LEAD0_RANGE)
    b_step(1, 1, 0, 2, [], LEAD1_RANGE)
    cp_xa1.wait()

    def prologue_step(it, carry):
        for u in range(2):
            p = 2 * it + u
            wait_pair(p)
            b_step(p + LEAD, u, p + LEAD - 1, jnp.minimum(p + LEAD + 1, NPAIR - 1),
                   xlu_pieces(p))
        return carry

    lax.fori_loop(0, (NPAIR - LEAD) // 2, prologue_step, 0)
    wait_pair(NPAIR - 2)
    b_step(None, 0, NPAIR - 1, None, xlu_pieces(NPAIR - 2))
    wait_pair(NPAIR - 1)
    for u in xlu_pieces(NPAIR - 1):
        u()

    cp_m0.wait()
    cp_gw.wait()
    mem_v[...] = mem0_v[...].astype(F32)

    scale_a = DH_A ** (-0.5)
    qi = lax.broadcasted_iota(jnp.int32, (L, 2 * L), 0)
    kl = lax.broadcasted_iota(jnp.int32, (L, 2 * L), 1)
    head_a = kl < L
    ki = jnp.where(head_a, kl, kl - L)
    mask = (qi < M_A) | (qi >= ki)
    lane = lax.broadcasted_iota(jnp.int32, (L, 128), 1)
    lo = lane < 64
    zblk = jnp.zeros((L, 128), F32)

    def softmax_pair(s):
        s = jnp.where(mask, s * scale_a, NEG)
        ma = jnp.max(jnp.where(head_a, s, -jnp.inf), axis=1, keepdims=True)
        mb = jnp.max(jnp.where(head_a, -jnp.inf, s), axis=1, keepdims=True)
        e = jnp.exp(s - jnp.where(head_a, ma, mb))
        da = jnp.sum(jnp.where(head_a, e, 0.0), axis=1, keepdims=True)
        db = jnp.sum(jnp.where(head_a, 0.0, e), axis=1, keepdims=True)
        return e * _recip(jnp.where(head_a, da, db))

    def segment(r0, mem):
        xs = xa_v[pl.ds(r0, SEG), :].astype(F32)
        h = [jnp.concatenate([mem[j], xs[:, j * 128:(j + 1) * 128]], axis=0) for j in range(5)]
        h_full = jnp.concatenate(h, axis=1)

        def qkv_proj(p):
            if p == 0:
                y = None
                for j in range(5):
                    t = _dot(h[j], _unpack(wqkv_v[p, j * 64:(j + 1) * 64, :]))
                    y = t if y is None else y + t
                return y
            return _dot(h_full, _unpack(wqkv_v[p]))

        def scores(y):
            q0, q1, q2 = (y[:, k * 128:(k + 1) * 128] for k in range(3))
            k0, k1, k2 = (y[:, (3 + k) * 128:(4 + k) * 128] for k in range(3))
            k2n = jnp.concatenate([jnp.where(lo, k2, 0.0), jnp.where(lo, 0.0, k2)], axis=0)
            sc = (_dot(q0, jnp.concatenate([k0, zblk], axis=0), NT)
                  + _dot(q1, jnp.concatenate([zblk, k1], axis=0), NT)
                  + _dot(q2, k2n, NT))
            return softmax_pair(sc)

        def pv(p, y, pr):
            v0, v1, v2 = (y[:, (6 + k) * 128:(7 + k) * 128] for k in range(3))
            v2n = jnp.concatenate([jnp.where(lo, v2, 0.0), jnp.where(lo, 0.0, v2)], axis=0)
            o_v[:, p * PAIR:p * PAIR + 128] = _dot(pr, jnp.concatenate([v0, zblk], axis=0))
            o_v[:, p * PAIR + 128:p * PAIR + 256] = _dot(pr, jnp.concatenate([zblk, v1], axis=0))
            o_v[:, p * PAIR + 256:p * PAIR + 384] = _dot(pr, v2n)

        def out_proj(p, acc):
            t = _dot(o_v[:, p * PAIR:(p + 1) * PAIR], _unpack(woA_v[p]))
            return t if acc is None else acc + t

        ys, probs = {}, {}
        acc = None
        wo_next = 0
        for i in range(NPAIR + 2):
            if i < NPAIR:
                ys[i] = qkv_proj(i)
            else:
                for _ in range(3):
                    acc = out_proj(wo_next, acc)
                    wo_next += 1
            if 1 <= i <= NPAIR:
                probs[i - 1] = scores(ys[i - 1])
            if i >= 2:
                pv(i - 2, ys.pop(i - 2), probs.pop(i - 2))
        n_tail = 2
        while wo_next < NPAIR - n_tail:
            acc = out_proj(wo_next, acc)
            wo_next += 1
        accs = []
        for j in range(5):
            t = acc[:, j * 128:(j + 1) * 128]
            for p in range(NPAIR - n_tail, NPAIR):
                t = t + _dot(o_v[:, p * PAIR:(p + 1) * PAIR],
                             _unpack(woA_v[p, :, j * 128:(j + 1) * 128]))
            accs.append(t)
        a = jnp.concatenate([t[M_A:] for t in accs], axis=1)
        gw = gw_v[...].astype(F32)
        gx = xs[:, 0:128] * gw[0:1, :]
        for j in range(1, 5):
            gx = gx + xs[:, j * 128:(j + 1) * 128] * gw[j:j + 1, :]
        g = jax.nn.sigmoid(jnp.sum(gx, axis=1, keepdims=True))
        res = g * a + (1.0 - g) * bmix[pl.ds(r0, SEG), :]
        out_v[pl.ds(r0, SEG), :] = res.astype(BF16)
        return [t[:M_A] for t in accs]

    def seg_step(it, carry):
        rows = UNROLL * SEG
        base = pl.multiple_of(it * rows, rows)
        mem = [mem_v[:, j * 128:(j + 1) * 128] for j in range(5)]
        for u in range(UNROLL):
            r0 = pl.multiple_of(base + u * SEG, SEG)
            mem = segment(r0, mem)
            pltpu.make_async_copy(out_v.at[pl.ds(r0, SEG), :], out_hbm.at[pl.ds(r0, SEG), :],
                                  out_sem).start()
        for j in range(5):
            mem_v[:, j * 128:(j + 1) * 128] = mem[j]
        return carry

    lax.fori_loop(0, NSTEPS // UNROLL, seg_step, 0)
    pltpu.make_async_copy(out_v.at[pl.ds(0, NSTEPS * SEG), :], out_hbm.at[pl.ds(0, NSTEPS * SEG), :],
                          out_sem).wait()


def pallas_gated_mix__memory_aug_recurrent_mem_tr__sliding_local_dilated__prompt_kernel(
    A_x, A_mem0, A_Wq, A_Wk, A_Wv, A_Wo, A_seg_len, B_x, B_wqkv, B_wo, gate_w,
):
    del B_x
    if isinstance(A_seg_len, int):
        assert A_seg_len == SEG
    hd = H_A * DH_A
    xa = A_x.reshape(S, D)
    mem0 = A_mem0.reshape(M_A, D)
    wqT = A_Wq.transpose(1, 2, 0).reshape(hd, D)
    wkT = A_Wk.transpose(1, 2, 0).reshape(hd, D)
    wvT = A_Wv.transpose(1, 2, 0).reshape(hd, D)
    woA = A_Wo.reshape(hd, D)
    gw = gate_w.reshape(5, 128)

    scratch = [
        pltpu.VMEM((S, D), BF16),
        pltpu.VMEM((M_A, D), BF16),
        pltpu.VMEM((4, hd, D), BF16),
        pltpu.VMEM((NPAIR, D // 2, 9 * 128), jnp.uint32),
        pltpu.VMEM((NPAIR, PAIR // 2, D), jnp.uint32),
        pltpu.VMEM((D, 3 * D), BF16),
        pltpu.VMEM((D, D), BF16),
        pltpu.VMEM((5, 4 * D + 32, 128), F32),
        pltpu.VMEM((3 * D // 2, D), jnp.uint32),
        pltpu.VMEM((D // 2, D), jnp.uint32),
        pltpu.VMEM((5, 128), BF16),
        pltpu.VMEM((S // NPAIR // 2, D), jnp.uint32),
        pltpu.VMEM((5, S, 128), F32),
        pltpu.VMEM((5, HALO + S, 128), F32),
        pltpu.VMEM((5, HALO + S, 128), F32),
        pltpu.VMEM((S // NPAIR, D), F32),
        pltpu.VMEM((S // NPAIR, D), F32),
        pltpu.VMEM((S, D), F32),
        pltpu.VMEM((M_A, D), F32),
        pltpu.VMEM((L, hd), F32),
        pltpu.VMEM((S, D), BF16),
        pltpu.SemaphoreType.DMA((8,)),
        pltpu.SemaphoreType.DMA((NPAIR,)),
        pltpu.SemaphoreType.DMA,
    ]
    out = pl.pallas_call(
        _kernel,
        out_shape=jax.ShapeDtypeStruct((S, D), BF16),
        in_specs=[pl.BlockSpec(memory_space=pl.ANY)] * 9,
        out_specs=pl.BlockSpec(memory_space=pl.ANY),
        scratch_shapes=scratch,
        compiler_params=pltpu.CompilerParams(vmem_limit_bytes=120 * 1024 * 1024,
                                             disable_bounds_checks=NO_BOUNDS),
    )(xa, mem0, wqT, wkT, wvT, woA, B_wqkv, B_wo, gw)
    return out.reshape(1, S, D)
```

```python
import functools

import jax
import jax.numpy as jnp
from jax import lax
import jax.experimental.pallas as pl
import jax.experimental.pallas.tpu as pltpu

F32 = jnp.float32
BF16 = jnp.bfloat16

S = 2048
D = 640
H_A, DH_A = 32, 192
M_A = 8
SEG = 32
L = M_A + SEG
NPAIR = H_A // 2
PAIR = 2 * DH_A
H_B, DH_B = 32, 20
WIN, DIL = 8, 2
HALO = 16
NEG = -1000000000.0

B_ROWS = 8
NSTEPS = S // SEG
UNROLL = 4
NO_BOUNDS = True
XLU_START = 0
XLU_END = 6
VPU_START = 6
VPU_END = 20
LEAD = 2
LEAD0_RANGE = (0, 20)
LEAD1_RANGE = (0, 20)

NT = (((1,), (1,)), ((), ()))
NN = (((1,), (0,)), ((), ()))


def _dot(a, b, dn=NN):
    return lax.dot_general(a, b, dn, preferred_element_type=F32)


def _pack(x):
    return pltpu.bitcast(x, jnp.uint32)


def _unpack(x):
    return pltpu.bitcast(x, BF16)


def _recip(d):
    r = pl.reciprocal(d, approx=True)
    return r * (2.0 - d * r)


def _kernel(xa_hbm, mem0_hbm, wqT_hbm, wkT_hbm, wvT_hbm, woA_hbm,
            wqkvB_hbm, woB_hbm, gw_hbm,
            out_hbm,
            xa_v, mem0_v, wT_v, wqkv_v, woA_v,
            wB_raw, woB_raw, w32, wBT_v, woB_v, gw_v,
            xp, qB, kB, vB, oB0, oB1, bmix,
            mem_v, o_v, out_v,
            sems, pair_sems, out_sem):
    XA_HEAD = 3 * (S // NPAIR)
    cp_wB = [pltpu.make_async_copy(wqkvB_hbm.at[:, j * D:(j + 1) * D],
                                   wB_raw.at[:, j * D:(j + 1) * D], sems.at[j]) for j in range(3)]
    cp_xa0 = pltpu.make_async_copy(xa_hbm.at[0:XA_HEAD, :], xa_v.at[0:XA_HEAD, :], sems.at[3])
    cp_woB = pltpu.make_async_copy(woB_hbm, woB_raw, sems.at[4])
    cp_xa1 = pltpu.make_async_copy(xa_hbm.at[XA_HEAD:S, :], xa_v.at[XA_HEAD:S, :], sems.at[5])
    cp_m0 = pltpu.make_async_copy(mem0_hbm, mem0_v, sems.at[6])
    cp_gw = pltpu.make_async_copy(gw_hbm, gw_v, sems.at[7])

    def pair_copies(p):
        r = pl.multiple_of(p * PAIR, 128)
        return [pltpu.make_async_copy(w.at[pl.ds(r, PAIR), :], wT_v.at[t, pl.ds(r, PAIR), :],
                                      pair_sems.at[p])
                for t, w in enumerate((wqT_hbm, wkT_hbm, wvT_hbm, woA_hbm))]

    for cp in cp_wB + [cp_xa0, cp_woB, cp_xa1, cp_m0, cp_gw]:
        cp.start()

    def gather_rows(base, dst, dst_base):
        for d in range(DH_B):
            r = (dst_base + d * H_B) // 2
            for c in range(5):
                g = w32[c, pl.ds(base + d, H_B, stride=DH_B), :]
                dst[r:r + H_B // 2, c * 128:(c + 1) * 128] = _pack(g.astype(BF16))

    for which in range(3):
        cp_wB[which].wait()
        if which == 0:
            for p in range(NPAIR):
                for cp in pair_copies(p):
                    cp.start()
        for cb in range(5 * which, 5 * which + 5):
            for rb in range(5):
                tile = wB_raw[rb * 128:(rb + 1) * 128, cb * 128:(cb + 1) * 128]
                w32[rb, cb * 128:(cb + 1) * 128, :] = tile.T.astype(F32)
        gather_rows(which * D, wBT_v, which * D)

    zero_halo = jnp.zeros((HALO, 128), F32)
    for j in range(5):
        kB[j, 0:HALO, :] = zero_halo
        vB[j, 0:HALO, :] = zero_halo

    rows_b = S // NPAIR
    scale_b = DH_B ** (-0.5)

    def b_attend(gr, masked):
        nsub = B_ROWS // 8
        offs = sorted({8 * i - DIL * w for i in range(nsub) for w in range(WIN)})

        def windows(ref, j):
            return {off: ref[j, pl.ds(HALO + gr + off, 8), :] for off in offs}

        def shifted(win, w):
            return jnp.concatenate([win[8 * i - DIL * w] for i in range(nsub)], axis=0)

        part = [None] * WIN
        for j in range(5):
            q = qB[j, pl.ds(gr, B_ROWS), :]
            win = windows(kB, j)
            for w in range(WIN):
                t = q * shifted(win, w)
                part[w] = t if part[w] is None else part[w] + t
        logits = []
        for w in range(WIN):
            s = part[w]
            s = s + pltpu.roll(s, 64, 1)
            s = s + pltpu.roll(s, 32, 1)
            logits.append(s)
        if masked:
            pos = gr + lax.broadcasted_iota(jnp.int32, (B_ROWS, 128), 0)
            logits = [jnp.where(pos >= DIL * w, l * scale_b, NEG) for w, l in enumerate(logits)]
            post = 1.0
        else:
            post = scale_b
        m = logits[0]
        for w in range(1, WIN):
            m = jnp.maximum(m, logits[w])
        e = [jnp.exp((l - m) * post) for l in logits]
        den = e[0]
        for w in range(1, WIN):
            den = den + e[w]
        inv = _recip(den)
        cols = []
        for j in range(5):
            win = windows(vB, j)
            acc = e[0] * shifted(win, 0)
            for w in range(1, WIN):
                acc = acc + e[w] * shifted(win, w)
            cols.append(acc * inv)
        return jnp.concatenate(cols, axis=1)

    def _row0(blk):
        return blk * rows_b if isinstance(blk, int) else pl.multiple_of(blk * rows_b, rows_b)

    def b_pack_x(blk):
        r0 = _row0(blk)
        xp[...] = _pack(xa_v[pl.ds(r0, rows_b), :])

    def b_project_tile(blk, n):
        r0 = _row0(blk)
        t = _dot(_unpack(xp[...]), _unpack(wBT_v[n * 64:(n + 1) * 64, :]), NT)
        if n < 5:
            qB[n, pl.ds(r0, rows_b), :] = t
        elif n < 10:
            kB[n - 5, pl.ds(HALO + r0, rows_b), :] = t
        else:
            vB[n - 10, pl.ds(HALO + r0, rows_b), :] = t

    def b_out_tile(blk, slot, n):
        r0 = _row0(blk)
        bmix[pl.ds(r0, rows_b), n * 128:(n + 1) * 128] = _dot(
            oB[slot][...], _unpack(woB_v[:, n * 128:(n + 1) * 128]))

    def xlu_pieces(p):
        r = p * PAIR if isinstance(p, int) else pl.multiple_of(p * PAIR, 128)

        def pair_block(t, k):
            if k == 0:
                return wT_v[t, pl.ds(r, 128), :]
            if k == 1:
                return wT_v[t, pl.ds(r + 192, 128), :]
            return jnp.concatenate([wT_v[t, pl.ds(r + 128, 64), :],
                                    wT_v[t, pl.ds(r + 320, 64), :]], axis=0)

        def xpose_block(t, k):
            blk = pair_block(t, k)
            col = (t * 3 + k) * 128
            for j in range(5):
                tile = blk[:, j * 128:(j + 1) * 128]
                wqkv_v[p, j * 64:(j + 1) * 64, col:col + 128] = _pack(tile.T)

        def repack_block(k):
            woA_v[p, k * 64:(k + 1) * 64, :] = _pack(pair_block(3, k))

        return ([functools.partial(xpose_block, t, k) for t in range(3) for k in range(3)]
                + [functools.partial(repack_block, k) for k in range(3)])

    def b_step(attn_blk, attn_slot, out_blk, proj_blk, xlu, vpu_range=None):
        mxu, vpu = [], []
        if out_blk is not None:
            mxu += [functools.partial(b_out_tile, out_blk, 1 - attn_slot, n) for n in range(5)]
        if proj_blk is not None:
            b_pack_x(proj_blk)
            mxu += [functools.partial(b_project_tile, proj_blk, n) for n in range(15)]
        if attn_blk is not None:
            r0 = attn_blk * rows_b
            if not isinstance(r0, int):
                r0 = pl.multiple_of(r0, rows_b)

            def attend_block(i):
                gr = r0 + i * B_ROWS
                if not isinstance(gr, int):
                    gr = pl.multiple_of(gr, B_ROWS)
                masked = isinstance(gr, int) and gr < (WIN - 1) * DIL
                oB[attn_slot][i * B_ROWS:(i + 1) * B_ROWS, :] = b_attend(gr, masked)

            vpu = [functools.partial(attend_block, i) for i in range(rows_b // B_ROWS)]
        n = len(mxu)
        xs, xe = XLU_START * n // 20, XLU_END * n // 20
        vs, ve = vpu_range or (VPU_START, VPU_END)
        vs, ve = vs * n // 20, ve * n // 20
        for i in range(n):
            mxu[i]()
            if xs <= i < xe:
                k, c = i - xs, xe - xs
                for u in xlu[k * len(xlu) // c:(k + 1) * len(xlu) // c]:
                    u()
            if vs <= i < ve:
                k, c = i - vs, ve - vs
                for u in vpu[k * len(vpu) // c:(k + 1) * len(vpu) // c]:
                    u()

    def wait_pair(p):
        for cp in pair_copies(p):
            cp.wait()

    oB = (oB0, oB1)
    cp_xa0.wait()
    b_pack_x(0)
    for n in range(15):
        b_project_tile(0, n)
    cp_woB.wait()
    for c in range(5):
        w32[c, 3 * D:4 * D, :] = woB_raw[:, c * 128:(c + 1) * 128].astype(F32)
    gather_rows(3 * D, woB_v, 0)
    b_step(0, 0, None, 1, [], LEAD0_RANGE)
    b_step(1, 1, 0, 2, [], LEAD1_RANGE)
    cp_xa1.wait()

    def prologue_step(it, carry):
        for u in range(2):
            p = 2 * it + u
            wait_pair(p)
            b_step(p + LEAD, u, p + LEAD - 1, jnp.minimum(p + LEAD + 1, NPAIR - 1),
                   xlu_pieces(p))
        return carry

    lax.fori_loop(0, (NPAIR - LEAD) // 2, prologue_step, 0)
    wait_pair(NPAIR - 2)
    b_step(None, 0, NPAIR - 1, None, xlu_pieces(NPAIR - 2))
    wait_pair(NPAIR - 1)
    for u in xlu_pieces(NPAIR - 1):
        u()

    cp_m0.wait()
    cp_gw.wait()
    mem_v[...] = mem0_v[...].astype(F32)

    scale_a = DH_A ** (-0.5)
    qi = lax.broadcasted_iota(jnp.int32, (L, 2 * L), 0)
    kl = lax.broadcasted_iota(jnp.int32, (L, 2 * L), 1)
    head_a = kl < L
    ki = jnp.where(head_a, kl, kl - L)
    mask = (qi < M_A) | (qi >= ki)
    lane = lax.broadcasted_iota(jnp.int32, (L, 128), 1)
    lo = lane < 64
    zblk = jnp.zeros((L, 128), F32)

    def softmax_pair(s):
        s = jnp.where(mask, s * scale_a, NEG)
        ma = jnp.max(jnp.where(head_a, s, -jnp.inf), axis=1, keepdims=True)
        mb = jnp.max(jnp.where(head_a, -jnp.inf, s), axis=1, keepdims=True)
        e = jnp.exp(s - jnp.where(head_a, ma, mb))
        da = jnp.sum(jnp.where(head_a, e, 0.0), axis=1, keepdims=True)
        db = jnp.sum(jnp.where(head_a, 0.0, e), axis=1, keepdims=True)
        return e * _recip(jnp.where(head_a, da, db))

    def segment(r0, mem):
        xs = xa_v[pl.ds(r0, SEG), :].astype(F32)
        h = [jnp.concatenate([mem[j], xs[:, j * 128:(j + 1) * 128]], axis=0) for j in range(5)]
        h_full = jnp.concatenate(h, axis=1)

        def qkv_proj(p):
            if p == 0:
                y = None
                for j in range(5):
                    t = _dot(h[j], _unpack(wqkv_v[p, j * 64:(j + 1) * 64, :]))
                    y = t if y is None else y + t
                return y
            return _dot(h_full, _unpack(wqkv_v[p]))

        def scores(y):
            q0, q1, q2 = (y[:, k * 128:(k + 1) * 128] for k in range(3))
            k0, k1, k2 = (y[:, (3 + k) * 128:(4 + k) * 128] for k in range(3))
            k2n = jnp.concatenate([jnp.where(lo, k2, 0.0), jnp.where(lo, 0.0, k2)], axis=0)
            sc = (_dot(q0, jnp.concatenate([k0, zblk], axis=0), NT)
                  + _dot(q1, jnp.concatenate([zblk, k1], axis=0), NT)
                  + _dot(q2, k2n, NT))
            return softmax_pair(sc)

        def pv(p, y, pr):
            v0, v1, v2 = (y[:, (6 + k) * 128:(7 + k) * 128] for k in range(3))
            v2n = jnp.concatenate([jnp.where(lo, v2, 0.0), jnp.where(lo, 0.0, v2)], axis=0)
            o_v[:, p * PAIR:p * PAIR + 128] = _dot(pr, jnp.concatenate([v0, zblk], axis=0))
            o_v[:, p * PAIR + 128:p * PAIR + 256] = _dot(pr, jnp.concatenate([zblk, v1], axis=0))
            o_v[:, p * PAIR + 256:p * PAIR + 384] = _dot(pr, v2n)

        def out_proj(p, acc):
            t = _dot(o_v[:, p * PAIR:(p + 1) * PAIR], _unpack(woA_v[p]))
            return t if acc is None else acc + t

        ys, probs = {}, {}
        acc = None
        wo_next = 0
        for i in range(NPAIR + 2):
            if i < NPAIR:
                ys[i] = qkv_proj(i)
            else:
                for _ in range(3):
                    acc = out_proj(wo_next, acc)
                    wo_next += 1
            if 1 <= i <= NPAIR:
                probs[i - 1] = scores(ys[i - 1])
            if i >= 2:
                pv(i - 2, ys.pop(i - 2), probs.pop(i - 2))
        n_tail = 2
        while wo_next < NPAIR - n_tail:
            acc = out_proj(wo_next, acc)
            wo_next += 1
        accs = []
        for j in range(5):
            t = acc[:, j * 128:(j + 1) * 128]
            for p in range(NPAIR - n_tail, NPAIR):
                t = t + _dot(o_v[:, p * PAIR:(p + 1) * PAIR],
                             _unpack(woA_v[p, :, j * 128:(j + 1) * 128]))
            accs.append(t)
        a = jnp.concatenate([t[M_A:] for t in accs], axis=1)
        gw = gw_v[...].astype(F32)
        gx = xs[:, 0:128] * gw[0:1, :]
        for j in range(1, 5):
            gx = gx + xs[:, j * 128:(j + 1) * 128] * gw[j:j + 1, :]
        g = jax.nn.sigmoid(jnp.sum(gx, axis=1, keepdims=True))
        res = g * a + (1.0 - g) * bmix[pl.ds(r0, SEG), :]
        out_v[pl.ds(r0, SEG), :] = res.astype(BF16)
        return [t[:M_A] for t in accs]

    def seg_step(it, carry):
        rows = UNROLL * SEG
        base = pl.multiple_of(it * rows, rows)
        mem = [mem_v[:, j * 128:(j + 1) * 128] for j in range(5)]
        for u in range(UNROLL):
            r0 = pl.multiple_of(base + u * SEG, SEG)
            mem = segment(r0, mem)
            pltpu.make_async_copy(out_v.at[pl.ds(r0, SEG), :], out_hbm.at[pl.ds(r0, SEG), :],
                                  out_sem).start()
        for j in range(5):
            mem_v[:, j * 128:(j + 1) * 128] = mem[j]
        return carry

    lax.fori_loop(0, NSTEPS // UNROLL, seg_step, 0)
    pltpu.make_async_copy(out_v.at[pl.ds(0, NSTEPS * SEG), :], out_hbm.at[pl.ds(0, NSTEPS * SEG), :],
                          out_sem).wait()


def pallas_gated_mix__memory_aug_recurrent_mem_tr__sliding_local_dilated__prompt_kernel(
    A_x, A_mem0, A_Wq, A_Wk, A_Wv, A_Wo, A_seg_len, B_x, B_wqkv, B_wo, gate_w,
):
    del B_x
    if isinstance(A_seg_len, int):
        assert A_seg_len == SEG
    hd = H_A * DH_A
    xa = A_x.reshape(S, D)
    mem0 = A_mem0.reshape(M_A, D)
    wqT = A_Wq.transpose(1, 2, 0).reshape(hd, D)
    wkT = A_Wk.transpose(1, 2, 0).reshape(hd, D)
    wvT = A_Wv.transpose(1, 2, 0).reshape(hd, D)
    woA = A_Wo.reshape(hd, D)
    gw = gate_w.reshape(5, 128)

    scratch = [
        pltpu.VMEM((S, D), BF16),
        pltpu.VMEM((M_A, D), BF16),
        pltpu.VMEM((4, hd, D), BF16),
        pltpu.VMEM((NPAIR, D // 2, 9 * 128), jnp.uint32),
        pltpu.VMEM((NPAIR, PAIR // 2, D), jnp.uint32),
        pltpu.VMEM((D, 3 * D), BF16),
        pltpu.VMEM((D, D), BF16),
        pltpu.VMEM((5, 4 * D + 32, 128), F32),
        pltpu.VMEM((3 * D // 2, D), jnp.uint32),
        pltpu.VMEM((D // 2, D), jnp.uint32),
        pltpu.VMEM((5, 128), BF16),
        pltpu.VMEM((S // NPAIR // 2, D), jnp.uint32),
        pltpu.VMEM((5, S, 128), F32),
        pltpu.VMEM((5, HALO + S, 128), F32),
        pltpu.VMEM((5, HALO + S, 128), F32),
        pltpu.VMEM((S // NPAIR, D), F32),
        pltpu.VMEM((S // NPAIR, D), F32),
        pltpu.VMEM((S, D), F32),
        pltpu.VMEM((M_A, D), F32),
        pltpu.VMEM((L, hd), F32),
        pltpu.VMEM((S, D), BF16),
        pltpu.SemaphoreType.DMA((8,)),
        pltpu.SemaphoreType.DMA((NPAIR,)),
        pltpu.SemaphoreType.DMA,
    ]
    out = pl.pallas_call(
        _kernel,
        out_shape=jax.ShapeDtypeStruct((S, D), BF16),
        in_specs=[pl.BlockSpec(memory_space=pl.ANY)] * 9,
        out_specs=pl.BlockSpec(memory_space=pl.ANY),
        scratch_shapes=scratch,
        compiler_params=pltpu.CompilerParams(vmem_limit_bytes=120 * 1024 * 1024,
                                             disable_bounds_checks=NO_BOUNDS),
    )(xa, mem0, wqT, wkT, wvT, woA, B_wqkv, B_wo, gw)
    return out.reshape(1, S, D)
```

```python
import functools

import jax
import jax.numpy as jnp
from jax import lax
import jax.experimental.pallas as pl
import jax.experimental.pallas.tpu as pltpu

F32 = jnp.float32
BF16 = jnp.bfloat16

S = 2048
D = 640
H_A, DH_A = 32, 192
M_A = 8
SEG = 32
L = M_A + SEG
NPAIR = H_A // 2
PAIR = 2 * DH_A
H_B, DH_B = 32, 20
WIN, DIL = 8, 2
HALO = 16
NEG = -1000000000.0

B_ROWS = 8
NSTEPS = S // SEG
UNROLL = 4
LEAD = 2
XLU_START = 0
XLU_END = 6
VPU_START = 6
VPU_END = 20

NT = (((1,), (1,)), ((), ()))
NN = (((1,), (0,)), ((), ()))


def _dot(a, b, dn=NN):
    return lax.dot_general(a, b, dn, preferred_element_type=F32)


def _pack(x):
    return pltpu.bitcast(x, jnp.uint32)


def _unpack(x):
    return pltpu.bitcast(x, BF16)


def _recip(d):
    r = pl.reciprocal(d, approx=True)
    return r * (2.0 - d * r)


def _kernel(xa_hbm, mem0_hbm, wqT_hbm, wkT_hbm, wvT_hbm, woA_hbm,
            wqkvB_hbm, woB_hbm, gw_hbm,
            out_hbm,
            xa_v, mem0_v, wT_v, wqkv_v, woA_v,
            wB_raw, woB_raw, w32, wBT_v, woB_v, gw_v,
            xp, qB, kB, vB, oB0, oB1, bmix,
            mem_v, o_v, out_v,
            sems, pair_sems, out_sem):
    XA_HEAD = 3 * (S // NPAIR)
    cp_wB = [pltpu.make_async_copy(wqkvB_hbm.at[:, j * D:(j + 1) * D],
                                   wB_raw.at[:, j * D:(j + 1) * D], sems.at[j]) for j in range(3)]
    cp_xa0 = pltpu.make_async_copy(xa_hbm.at[0:XA_HEAD, :], xa_v.at[0:XA_HEAD, :], sems.at[3])
    cp_woB = pltpu.make_async_copy(woB_hbm, woB_raw, sems.at[4])
    cp_xa1 = pltpu.make_async_copy(xa_hbm.at[XA_HEAD:S, :], xa_v.at[XA_HEAD:S, :], sems.at[5])
    cp_m0 = pltpu.make_async_copy(mem0_hbm, mem0_v, sems.at[6])
    cp_gw = pltpu.make_async_copy(gw_hbm, gw_v, sems.at[7])

    def pair_copies(p):
        r = pl.multiple_of(p * PAIR, 128)
        return [pltpu.make_async_copy(w.at[pl.ds(r, PAIR), :], wT_v.at[t, pl.ds(r, PAIR), :],
                                      pair_sems.at[p])
                for t, w in enumerate((wqT_hbm, wkT_hbm, wvT_hbm, woA_hbm))]

    for cp in cp_wB + [cp_xa0, cp_woB, cp_xa1, cp_m0, cp_gw]:
        cp.start()

    def gather_rows(base, dst, dst_base):
        for d in range(DH_B):
            r = (dst_base + d * H_B) // 2
            for c in range(5):
                g = w32[c, pl.ds(base + d, H_B, stride=DH_B), :]
                dst[r:r + H_B // 2, c * 128:(c + 1) * 128] = _pack(g.astype(BF16))

    for which in range(3):
        cp_wB[which].wait()
        if which == 0:
            for p in range(NPAIR):
                for cp in pair_copies(p):
                    cp.start()
        for cb in range(5 * which, 5 * which + 5):
            for rb in range(5):
                tile = wB_raw[rb * 128:(rb + 1) * 128, cb * 128:(cb + 1) * 128]
                w32[rb, cb * 128:(cb + 1) * 128, :] = tile.T.astype(F32)
        gather_rows(which * D, wBT_v, which * D)

    zero_halo = jnp.zeros((HALO, 128), F32)
    for j in range(5):
        kB[j, 0:HALO, :] = zero_halo
        vB[j, 0:HALO, :] = zero_halo

    rows_b = S // NPAIR
    scale_b = DH_B ** (-0.5)

    def b_attend(gr, masked):
        nsub = B_ROWS // 8
        offs = sorted({8 * i - DIL * w for i in range(nsub) for w in range(WIN)})

        def windows(ref, j):
            return {off: ref[j, pl.ds(HALO + gr + off, 8), :] for off in offs}

        def shifted(win, w):
            return jnp.concatenate([win[8 * i - DIL * w] for i in range(nsub)], axis=0)

        part = [None] * WIN
        for j in range(5):
            q = qB[j, pl.ds(gr, B_ROWS), :]
            win = windows(kB, j)
            for w in range(WIN):
                t = q * shifted(win, w)
                part[w] = t if part[w] is None else part[w] + t
        logits = []
        for w in range(WIN):
            s = part[w]
            s = s + pltpu.roll(s, 64, 1)
            s = s + pltpu.roll(s, 32, 1)
            logits.append(s)
        if masked:
            pos = gr + lax.broadcasted_iota(jnp.int32, (B_ROWS, 128), 0)
            logits = [jnp.where(pos >= DIL * w, l * scale_b, NEG) for w, l in enumerate(logits)]
            post = 1.0
        else:
            post = scale_b
        m = logits[0]
        for w in range(1, WIN):
            m = jnp.maximum(m, logits[w])
        e = [jnp.exp((l - m) * post) for l in logits]
        den = e[0]
        for w in range(1, WIN):
            den = den + e[w]
        inv = _recip(den)
        cols = []
        for j in range(5):
            win = windows(vB, j)
            acc = e[0] * shifted(win, 0)
            for w in range(1, WIN):
                acc = acc + e[w] * shifted(win, w)
            cols.append(acc * inv)
        return jnp.concatenate(cols, axis=1)

    def _row0(blk):
        return blk * rows_b if isinstance(blk, int) else pl.multiple_of(blk * rows_b, rows_b)

    def b_pack_x(blk):
        r0 = _row0(blk)
        xp[...] = _pack(xa_v[pl.ds(r0, rows_b), :])

    def b_project_tile(blk, n):
        r0 = _row0(blk)
        t = _dot(_unpack(xp[...]), _unpack(wBT_v[n * 64:(n + 1) * 64, :]), NT)
        if n < 5:
            qB[n, pl.ds(r0, rows_b), :] = t
        elif n < 10:
            kB[n - 5, pl.ds(HALO + r0, rows_b), :] = t
        else:
            vB[n - 10, pl.ds(HALO + r0, rows_b), :] = t

    def b_out_tile(blk, slot, n):
        r0 = _row0(blk)
        bmix[pl.ds(r0, rows_b), n * 128:(n + 1) * 128] = _dot(
            oB[slot][...], _unpack(woB_v[:, n * 128:(n + 1) * 128]))

    def xlu_pieces(p):
        r = p * PAIR if isinstance(p, int) else pl.multiple_of(p * PAIR, 128)

        def pair_block(t, k):
            if k == 0:
                return wT_v[t, pl.ds(r, 128), :]
            if k == 1:
                return wT_v[t, pl.ds(r + 192, 128), :]
            return jnp.concatenate([wT_v[t, pl.ds(r + 128, 64), :],
                                    wT_v[t, pl.ds(r + 320, 64), :]], axis=0)

        def xpose_block(t, k):
            blk = pair_block(t, k)
            col = (t * 3 + k) * 128
            for j in range(5):
                tile = blk[:, j * 128:(j + 1) * 128]
                wqkv_v[p, j * 64:(j + 1) * 64, col:col + 128] = _pack(tile.T)

        def repack_block(k):
            woA_v[p, k * 64:(k + 1) * 64, :] = _pack(pair_block(3, k))

        return ([functools.partial(xpose_block, t, k) for t in range(3) for k in range(3)]
                + [functools.partial(repack_block, k) for k in range(3)])

    def b_step(attn_blk, attn_slot, out_blk, proj_blk, xlu, vpu_range=None):
        mxu, vpu = [], []
        if out_blk is not None:
            mxu += [functools.partial(b_out_tile, out_blk, 1 - attn_slot, n) for n in range(5)]
        if proj_blk is not None:
            b_pack_x(proj_blk)
            mxu += [functools.partial(b_project_tile, proj_blk, n) for n in range(15)]
        if attn_blk is not None:
            r0 = attn_blk * rows_b
            if not isinstance(r0, int):
                r0 = pl.multiple_of(r0, rows_b)

            def attend_block(i):
                gr = r0 + i * B_ROWS
                if not isinstance(gr, int):
                    gr = pl.multiple_of(gr, B_ROWS)
                masked = isinstance(gr, int) and gr < (WIN - 1) * DIL
                oB[attn_slot][i * B_ROWS:(i + 1) * B_ROWS, :] = b_attend(gr, masked)

            vpu = [functools.partial(attend_block, i) for i in range(rows_b // B_ROWS)]
        n = len(mxu)
        xs, xe = XLU_START * n // 20, XLU_END * n // 20
        vs, ve = vpu_range or (VPU_START, VPU_END)
        vs, ve = vs * n // 20, ve * n // 20
        for i in range(n):
            mxu[i]()
            if xs <= i < xe:
                k, c = i - xs, xe - xs
                for u in xlu[k * len(xlu) // c:(k + 1) * len(xlu) // c]:
                    u()
            if vs <= i < ve:
                k, c = i - vs, ve - vs
                for u in vpu[k * len(vpu) // c:(k + 1) * len(vpu) // c]:
                    u()

    def wait_pair(p):
        for cp in pair_copies(p):
            cp.wait()

    oB = (oB0, oB1)
    cp_xa0.wait()
    b_pack_x(0)
    for n in range(15):
        b_project_tile(0, n)
    cp_woB.wait()
    for c in range(5):
        w32[c, 3 * D:4 * D, :] = woB_raw[:, c * 128:(c + 1) * 128].astype(F32)
    gather_rows(3 * D, woB_v, 0)
    b_step(0, 0, None, 1, [], (0, 20))
    b_step(1, 1, 0, 2, [], (0, 20))
    cp_xa1.wait()

    def prologue_step(it, carry):
        for u in range(2):
            p = 2 * it + u
            wait_pair(p)
            b_step(p + LEAD, u, p + LEAD - 1, jnp.minimum(p + LEAD + 1, NPAIR - 1),
                   xlu_pieces(p))
        return carry

    lax.fori_loop(0, (NPAIR - LEAD) // 2, prologue_step, 0)
    wait_pair(NPAIR - 2)
    b_step(None, 0, NPAIR - 1, None, xlu_pieces(NPAIR - 2))
    wait_pair(NPAIR - 1)
    for u in xlu_pieces(NPAIR - 1):
        u()

    cp_m0.wait()
    cp_gw.wait()
    mem_v[...] = mem0_v[...].astype(F32)

    scale_a = DH_A ** (-0.5)
    qi = lax.broadcasted_iota(jnp.int32, (L, 2 * L), 0)
    kl = lax.broadcasted_iota(jnp.int32, (L, 2 * L), 1)
    head_a = kl < L
    ki = jnp.where(head_a, kl, kl - L)
    mask = (qi < M_A) | (qi >= ki)
    lane = lax.broadcasted_iota(jnp.int32, (L, 128), 1)
    lo = lane < 64
    zblk = jnp.zeros((L, 128), F32)

    def softmax_pair(s):
        s = jnp.where(mask, s * scale_a, NEG)
        ma = jnp.max(jnp.where(head_a, s, -jnp.inf), axis=1, keepdims=True)
        mb = jnp.max(jnp.where(head_a, -jnp.inf, s), axis=1, keepdims=True)
        e = jnp.exp(s - jnp.where(head_a, ma, mb))
        da = jnp.sum(jnp.where(head_a, e, 0.0), axis=1, keepdims=True)
        db = jnp.sum(jnp.where(head_a, 0.0, e), axis=1, keepdims=True)
        return e * _recip(jnp.where(head_a, da, db))

    def segment(r0, mem):
        xs = xa_v[pl.ds(r0, SEG), :].astype(F32)
        h = [jnp.concatenate([mem[j], xs[:, j * 128:(j + 1) * 128]], axis=0) for j in range(5)]
        h_full = jnp.concatenate(h, axis=1)

        def qkv_proj(p):
            if p == 0:
                y = None
                for j in range(5):
                    t = _dot(h[j], _unpack(wqkv_v[p, j * 64:(j + 1) * 64, :]))
                    y = t if y is None else y + t
                return y
            return _dot(h_full, _unpack(wqkv_v[p]))

        def scores(y):
            q0, q1, q2 = (y[:, k * 128:(k + 1) * 128] for k in range(3))
            k0, k1, k2 = (y[:, (3 + k) * 128:(4 + k) * 128] for k in range(3))
            k2n = jnp.concatenate([jnp.where(lo, k2, 0.0), jnp.where(lo, 0.0, k2)], axis=0)
            sc = (_dot(q0, jnp.concatenate([k0, zblk], axis=0), NT)
                  + _dot(q1, jnp.concatenate([zblk, k1], axis=0), NT)
                  + _dot(q2, k2n, NT))
            return softmax_pair(sc)

        def pv(p, y, pr):
            v0, v1, v2 = (y[:, (6 + k) * 128:(7 + k) * 128] for k in range(3))
            v2n = jnp.concatenate([jnp.where(lo, v2, 0.0), jnp.where(lo, 0.0, v2)], axis=0)
            o_v[:, p * PAIR:p * PAIR + 128] = _dot(pr, jnp.concatenate([v0, zblk], axis=0))
            o_v[:, p * PAIR + 128:p * PAIR + 256] = _dot(pr, jnp.concatenate([zblk, v1], axis=0))
            o_v[:, p * PAIR + 256:p * PAIR + 384] = _dot(pr, v2n)

        def out_proj(p, acc):
            t = _dot(o_v[:, p * PAIR:(p + 1) * PAIR], _unpack(woA_v[p]))
            return t if acc is None else acc + t

        ys, probs = {}, {}
        acc = None
        wo_next = 0
        for i in range(NPAIR + 2):
            if i < NPAIR:
                ys[i] = qkv_proj(i)
            else:
                for _ in range(3):
                    acc = out_proj(wo_next, acc)
                    wo_next += 1
            if 1 <= i <= NPAIR:
                probs[i - 1] = scores(ys[i - 1])
            if i >= 2:
                pv(i - 2, ys.pop(i - 2), probs.pop(i - 2))
        n_tail = 2
        while wo_next < NPAIR - n_tail:
            acc = out_proj(wo_next, acc)
            wo_next += 1
        accs = []
        for j in range(5):
            t = acc[:, j * 128:(j + 1) * 128]
            for p in range(NPAIR - n_tail, NPAIR):
                t = t + _dot(o_v[:, p * PAIR:(p + 1) * PAIR],
                             _unpack(woA_v[p, :, j * 128:(j + 1) * 128]))
            accs.append(t)
        a = jnp.concatenate([t[M_A:] for t in accs], axis=1)
        gw = gw_v[...].astype(F32)
        gx = xs[:, 0:128] * gw[0:1, :]
        for j in range(1, 5):
            gx = gx + xs[:, j * 128:(j + 1) * 128] * gw[j:j + 1, :]
        g = jax.nn.sigmoid(jnp.sum(gx, axis=1, keepdims=True))
        res = g * a + (1.0 - g) * bmix[pl.ds(r0, SEG), :]
        out_v[pl.ds(r0, SEG), :] = res.astype(BF16)
        return [t[:M_A] for t in accs]

    def seg_step(it, carry):
        rows = UNROLL * SEG
        base = pl.multiple_of(it * rows, rows)
        mem = [mem_v[:, j * 128:(j + 1) * 128] for j in range(5)]
        for u in range(UNROLL):
            r0 = pl.multiple_of(base + u * SEG, SEG)
            mem = segment(r0, mem)
            pltpu.make_async_copy(out_v.at[pl.ds(r0, SEG), :], out_hbm.at[pl.ds(r0, SEG), :],
                                  out_sem).start()
        for j in range(5):
            mem_v[:, j * 128:(j + 1) * 128] = mem[j]
        return carry

    lax.fori_loop(0, NSTEPS // UNROLL, seg_step, 0)
    pltpu.make_async_copy(out_v.at[pl.ds(0, NSTEPS * SEG), :], out_hbm.at[pl.ds(0, NSTEPS * SEG), :],
                          out_sem).wait()


def pallas_gated_mix__memory_aug_recurrent_mem_tr__sliding_local_dilated__prompt_kernel(
    A_x, A_mem0, A_Wq, A_Wk, A_Wv, A_Wo, A_seg_len, B_x, B_wqkv, B_wo, gate_w,
):
    del B_x
    if isinstance(A_seg_len, int):
        assert A_seg_len == SEG
    hd = H_A * DH_A
    xa = A_x.reshape(S, D)
    mem0 = A_mem0.reshape(M_A, D)
    wqT = A_Wq.transpose(1, 2, 0).reshape(hd, D)
    wkT = A_Wk.transpose(1, 2, 0).reshape(hd, D)
    wvT = A_Wv.transpose(1, 2, 0).reshape(hd, D)
    woA = A_Wo.reshape(hd, D)
    gw = gate_w.reshape(5, 128)

    scratch = [
        pltpu.VMEM((S, D), BF16),
        pltpu.VMEM((M_A, D), BF16),
        pltpu.VMEM((4, hd, D), BF16),
        pltpu.VMEM((NPAIR, D // 2, 9 * 128), jnp.uint32),
        pltpu.VMEM((NPAIR, PAIR // 2, D), jnp.uint32),
        pltpu.VMEM((D, 3 * D), BF16),
        pltpu.VMEM((D, D), BF16),
        pltpu.VMEM((5, 4 * D + 32, 128), F32),
        pltpu.VMEM((3 * D // 2, D), jnp.uint32),
        pltpu.VMEM((D // 2, D), jnp.uint32),
        pltpu.VMEM((5, 128), BF16),
        pltpu.VMEM((S // NPAIR // 2, D), jnp.uint32),
        pltpu.VMEM((5, S, 128), F32),
        pltpu.VMEM((5, HALO + S, 128), F32),
        pltpu.VMEM((5, HALO + S, 128), F32),
        pltpu.VMEM((S // NPAIR, D), F32),
        pltpu.VMEM((S // NPAIR, D), F32),
        pltpu.VMEM((S, D), F32),
        pltpu.VMEM((M_A, D), F32),
        pltpu.VMEM((L, hd), F32),
        pltpu.VMEM((S, D), BF16),
        pltpu.SemaphoreType.DMA((8,)),
        pltpu.SemaphoreType.DMA((NPAIR,)),
        pltpu.SemaphoreType.DMA,
    ]
    out = pl.pallas_call(
        _kernel,
        out_shape=jax.ShapeDtypeStruct((S, D), BF16),
        in_specs=[pl.BlockSpec(memory_space=pl.ANY)] * 9,
        out_specs=pl.BlockSpec(memory_space=pl.ANY),
        scratch_shapes=scratch,
        compiler_params=pltpu.CompilerParams(vmem_limit_bytes=120 * 1024 * 1024,
                                             disable_bounds_checks=True),
    )(xa, mem0, wqT, wkT, wvT, woA, B_wqkv, B_wo, gw)
    return out.reshape(1, S, D)
```

```python
import functools

import jax
import jax.numpy as jnp
from jax import lax
import jax.experimental.pallas as pl
import jax.experimental.pallas.tpu as pltpu

F32 = jnp.float32
BF16 = jnp.bfloat16

S = 2048
D = 640
H_A, DH_A = 32, 192
M_A = 8
SEG = 32
L = M_A + SEG
NPAIR = H_A // 2
PAIR = 2 * DH_A
H_B, DH_B = 32, 20
WIN, DIL = 8, 2
HALO = 16
NEG = -1000000000.0

B_ROWS = 8
NSTEPS = S // SEG
UNROLL = 4
LEAD = 2
XLU_START = 0
XLU_END = 6
VPU_START = 6
VPU_END = 20

NT = (((1,), (1,)), ((), ()))
NN = (((1,), (0,)), ((), ()))


def _dot(a, b, dn=NN):
    return lax.dot_general(a, b, dn, preferred_element_type=F32)


def _pack(x):
    return pltpu.bitcast(x, jnp.uint32)


def _unpack(x):
    return pltpu.bitcast(x, BF16)


def _recip(d):
    r = pl.reciprocal(d, approx=True)
    return r * (2.0 - d * r)


def _kernel(xa_hbm, mem0_hbm, wqT_hbm, wkT_hbm, wvT_hbm, woA_hbm,
            wqkvB_hbm, woB_hbm, gw_hbm,
            out_hbm,
            xa_v, mem0_v, wT_v, wqkv_v, woA_v,
            wB_raw, woB_raw, w32, wBT_v, woB_v, gw_v,
            xp, qB, kB, vB, oB0, oB1, bmix,
            mem_v, o_v, out_v,
            sems, pair_sems, out_sem):
    XA_HEAD = 3 * (S // NPAIR)
    cp_wB = [pltpu.make_async_copy(wqkvB_hbm.at[:, j * D:(j + 1) * D],
                                   wB_raw.at[:, j * D:(j + 1) * D], sems.at[j]) for j in range(3)]
    cp_xa0 = pltpu.make_async_copy(xa_hbm.at[0:XA_HEAD, :], xa_v.at[0:XA_HEAD, :], sems.at[3])
    cp_woB = pltpu.make_async_copy(woB_hbm, woB_raw, sems.at[4])
    cp_xa1 = pltpu.make_async_copy(xa_hbm.at[XA_HEAD:S, :], xa_v.at[XA_HEAD:S, :], sems.at[5])
    cp_m0 = pltpu.make_async_copy(mem0_hbm, mem0_v, sems.at[6])
    cp_gw = pltpu.make_async_copy(gw_hbm, gw_v, sems.at[7])

    def pair_copies(p):
        r = pl.multiple_of(p * PAIR, 128)
        last = isinstance(p, int) and p == NPAIR - 1
        return [pltpu.make_async_copy(w.at[pl.ds(r, PAIR), :], wT_v.at[t, pl.ds(r, PAIR), :],
                                      sems.at[8] if (last and t == 3) else pair_sems.at[p])
                for t, w in enumerate((wqT_hbm, wkT_hbm, wvT_hbm, woA_hbm))]

    for cp in cp_wB + [cp_xa0, cp_woB, cp_xa1, cp_m0, cp_gw]:
        cp.start()

    def gather_rows(base, dst, dst_base):
        for d in range(DH_B):
            r = (dst_base + d * H_B) // 2
            for c in range(5):
                g = w32[c, pl.ds(base + d, H_B, stride=DH_B), :]
                dst[r:r + H_B // 2, c * 128:(c + 1) * 128] = _pack(g.astype(BF16))

    for which in range(3):
        cp_wB[which].wait()
        if which == 0:
            for p in range(NPAIR):
                for cp in pair_copies(p):
                    cp.start()
        for cb in range(5 * which, 5 * which + 5):
            for rb in range(5):
                tile = wB_raw[rb * 128:(rb + 1) * 128, cb * 128:(cb + 1) * 128]
                w32[rb, cb * 128:(cb + 1) * 128, :] = tile.T.astype(F32)
        gather_rows(which * D, wBT_v, which * D)

    zero_halo = jnp.zeros((HALO, 128), F32)
    for j in range(5):
        kB[j, 0:HALO, :] = zero_halo
        vB[j, 0:HALO, :] = zero_halo

    rows_b = S // NPAIR
    scale_b = DH_B ** (-0.5)

    def b_attend(gr, masked):
        nsub = B_ROWS // 8
        offs = sorted({8 * i - DIL * w for i in range(nsub) for w in range(WIN)})

        def windows(ref, j):
            return {off: ref[j, pl.ds(HALO + gr + off, 8), :] for off in offs}

        def shifted(win, w):
            return jnp.concatenate([win[8 * i - DIL * w] for i in range(nsub)], axis=0)

        part = [None] * WIN
        for j in range(5):
            q = qB[j, pl.ds(gr, B_ROWS), :]
            win = windows(kB, j)
            for w in range(WIN):
                t = q * shifted(win, w)
                part[w] = t if part[w] is None else part[w] + t
        logits = []
        for w in range(WIN):
            s = part[w]
            s = s + pltpu.roll(s, 64, 1)
            s = s + pltpu.roll(s, 32, 1)
            logits.append(s)
        if masked:
            pos = gr + lax.broadcasted_iota(jnp.int32, (B_ROWS, 128), 0)
            logits = [jnp.where(pos >= DIL * w, l * scale_b, NEG) for w, l in enumerate(logits)]
            post = 1.0
        else:
            post = scale_b
        m = logits[0]
        for w in range(1, WIN):
            m = jnp.maximum(m, logits[w])
        e = [jnp.exp((l - m) * post) for l in logits]
        den = e[0]
        for w in range(1, WIN):
            den = den + e[w]
        inv = _recip(den)
        cols = []
        for j in range(5):
            win = windows(vB, j)
            acc = e[0] * shifted(win, 0)
            for w in range(1, WIN):
                acc = acc + e[w] * shifted(win, w)
            cols.append(acc * inv)
        return jnp.concatenate(cols, axis=1)

    def _row0(blk):
        return blk * rows_b if isinstance(blk, int) else pl.multiple_of(blk * rows_b, rows_b)

    def b_pack_x(blk):
        r0 = _row0(blk)
        xp[...] = _pack(xa_v[pl.ds(r0, rows_b), :])

    def b_project_tile(blk, n):
        r0 = _row0(blk)
        t = _dot(_unpack(xp[...]), _unpack(wBT_v[n * 64:(n + 1) * 64, :]), NT)
        if n < 5:
            qB[n, pl.ds(r0, rows_b), :] = t
        elif n < 10:
            kB[n - 5, pl.ds(HALO + r0, rows_b), :] = t
        else:
            vB[n - 10, pl.ds(HALO + r0, rows_b), :] = t

    def b_out_tile(blk, slot, n):
        r0 = _row0(blk)
        bmix[pl.ds(r0, rows_b), n * 128:(n + 1) * 128] = _dot(
            oB[slot][...], _unpack(woB_v[:, n * 128:(n + 1) * 128]))

    def xlu_pieces(p):
        r = p * PAIR if isinstance(p, int) else pl.multiple_of(p * PAIR, 128)

        def pair_block(t, k):
            if k == 0:
                return wT_v[t, pl.ds(r, 128), :]
            if k == 1:
                return wT_v[t, pl.ds(r + 192, 128), :]
            return jnp.concatenate([wT_v[t, pl.ds(r + 128, 64), :],
                                    wT_v[t, pl.ds(r + 320, 64), :]], axis=0)

        def xpose_block(t, k):
            blk = pair_block(t, k)
            col = (t * 3 + k) * 128
            for j in range(5):
                tile = blk[:, j * 128:(j + 1) * 128]
                wqkv_v[p, j * 64:(j + 1) * 64, col:col + 128] = _pack(tile.T)

        def repack_block(k):
            woA_v[p, k * 64:(k + 1) * 64, :] = _pack(pair_block(3, k))

        return ([functools.partial(xpose_block, t, k) for t in range(3) for k in range(3)]
                + [functools.partial(repack_block, k) for k in range(3)])

    def b_step(attn_blk, attn_slot, out_blk, proj_blk, xlu, vpu_range=None):
        mxu, vpu = [], []
        if out_blk is not None:
            mxu += [functools.partial(b_out_tile, out_blk, 1 - attn_slot, n) for n in range(5)]
        if proj_blk is not None:
            b_pack_x(proj_blk)
            mxu += [functools.partial(b_project_tile, proj_blk, n) for n in range(15)]
        if attn_blk is not None:
            r0 = attn_blk * rows_b
            if not isinstance(r0, int):
                r0 = pl.multiple_of(r0, rows_b)

            def attend_block(i):
                gr = r0 + i * B_ROWS
                if not isinstance(gr, int):
                    gr = pl.multiple_of(gr, B_ROWS)
                masked = isinstance(gr, int) and gr < (WIN - 1) * DIL
                oB[attn_slot][i * B_ROWS:(i + 1) * B_ROWS, :] = b_attend(gr, masked)

            vpu = [functools.partial(attend_block, i) for i in range(rows_b // B_ROWS)]
        n = len(mxu)
        xs, xe = XLU_START * n // 20, XLU_END * n // 20
        vs, ve = vpu_range or (VPU_START, VPU_END)
        vs, ve = vs * n // 20, ve * n // 20
        for i in range(n):
            mxu[i]()
            if xs <= i < xe:
                k, c = i - xs, xe - xs
                for u in xlu[k * len(xlu) // c:(k + 1) * len(xlu) // c]:
                    u()
            if vs <= i < ve:
                k, c = i - vs, ve - vs
                for u in vpu[k * len(vpu) // c:(k + 1) * len(vpu) // c]:
                    u()

    def wait_pair(p):
        for cp in pair_copies(p):
            cp.wait()

    oB = (oB0, oB1)
    cp_xa0.wait()
    b_pack_x(0)
    for n in range(15):
        b_project_tile(0, n)
    cp_woB.wait()
    for c in range(5):
        w32[c, 3 * D:4 * D, :] = woB_raw[:, c * 128:(c + 1) * 128].astype(F32)
    gather_rows(3 * D, woB_v, 0)
    b_step(0, 0, None, 1, [], (0, 20))
    b_step(1, 1, 0, 2, [], (0, 20))
    cp_xa1.wait()

    def prologue_step(it, carry):
        for u in range(2):
            p = 2 * it + u
            wait_pair(p)
            b_step(p + LEAD, u, p + LEAD - 1, jnp.minimum(p + LEAD + 1, NPAIR - 1),
                   xlu_pieces(p))
        return carry

    lax.fori_loop(0, (NPAIR - LEAD) // 2, prologue_step, 0)
    wait_pair(NPAIR - 2)
    b_step(None, 0, NPAIR - 1, None, xlu_pieces(NPAIR - 2))
    last_copies, last_pieces = pair_copies(NPAIR - 1), xlu_pieces(NPAIR - 1)
    for cp in last_copies[:3]:
        cp.wait()
    for u in last_pieces[:9]:
        u()
    last_copies[3].wait()
    for u in last_pieces[9:]:
        u()

    cp_m0.wait()
    cp_gw.wait()
    mem_v[...] = mem0_v[...].astype(F32)

    scale_a = DH_A ** (-0.5)
    qi = lax.broadcasted_iota(jnp.int32, (L, 2 * L), 0)
    kl = lax.broadcasted_iota(jnp.int32, (L, 2 * L), 1)
    head_a = kl < L
    ki = jnp.where(head_a, kl, kl - L)
    mask = (qi < M_A) | (qi >= ki)
    lane = lax.broadcasted_iota(jnp.int32, (L, 128), 1)
    lo = lane < 64
    zblk = jnp.zeros((L, 128), F32)

    def softmax_pair(s):
        s = jnp.where(mask, s * scale_a, NEG)
        ma = jnp.max(jnp.where(head_a, s, -jnp.inf), axis=1, keepdims=True)
        mb = jnp.max(jnp.where(head_a, -jnp.inf, s), axis=1, keepdims=True)
        e = jnp.exp(s - jnp.where(head_a, ma, mb))
        da = jnp.sum(jnp.where(head_a, e, 0.0), axis=1, keepdims=True)
        db = jnp.sum(jnp.where(head_a, 0.0, e), axis=1, keepdims=True)
        return e * _recip(jnp.where(head_a, da, db))

    def segment(r0, mem):
        xs = xa_v[pl.ds(r0, SEG), :].astype(F32)
        h = [jnp.concatenate([mem[j], xs[:, j * 128:(j + 1) * 128]], axis=0) for j in range(5)]
        h_full = jnp.concatenate(h, axis=1)

        def qkv_proj(p):
            if p == 0:
                y = None
                for j in range(5):
                    t = _dot(h[j], _unpack(wqkv_v[p, j * 64:(j + 1) * 64, :]))
                    y = t if y is None else y + t
                return y
            return _dot(h_full, _unpack(wqkv_v[p]))

        def scores(y):
            q0, q1, q2 = (y[:, k * 128:(k + 1) * 128] for k in range(3))
            k0, k1, k2 = (y[:, (3 + k) * 128:(4 + k) * 128] for k in range(3))
            k2n = jnp.concatenate([jnp.where(lo, k2, 0.0), jnp.where(lo, 0.0, k2)], axis=0)
            sc = (_dot(q0, jnp.concatenate([k0, zblk], axis=0), NT)
                  + _dot(q1, jnp.concatenate([zblk, k1], axis=0), NT)
                  + _dot(q2, k2n, NT))
            return softmax_pair(sc)

        def pv(p, y, pr):
            v0, v1, v2 = (y[:, (6 + k) * 128:(7 + k) * 128] for k in range(3))
            v2n = jnp.concatenate([jnp.where(lo, v2, 0.0), jnp.where(lo, 0.0, v2)], axis=0)
            o_v[:, p * PAIR:p * PAIR + 128] = _dot(pr, jnp.concatenate([v0, zblk], axis=0))
            o_v[:, p * PAIR + 128:p * PAIR + 256] = _dot(pr, jnp.concatenate([zblk, v1], axis=0))
            o_v[:, p * PAIR + 256:p * PAIR + 384] = _dot(pr, v2n)

        def out_proj(p, acc):
            t = _dot(o_v[:, p * PAIR:(p + 1) * PAIR], _unpack(woA_v[p]))
            return t if acc is None else acc + t

        ys, probs = {}, {}
        acc = None
        wo_next = 0
        for i in range(NPAIR + 2):
            if i < NPAIR:
                ys[i] = qkv_proj(i)
            else:
                for _ in range(3):
                    acc = out_proj(wo_next, acc)
                    wo_next += 1
            if 1 <= i <= NPAIR:
                probs[i - 1] = scores(ys[i - 1])
            if i >= 2:
                pv(i - 2, ys.pop(i - 2), probs.pop(i - 2))
        n_tail = 2
        while wo_next < NPAIR - n_tail:
            acc = out_proj(wo_next, acc)
            wo_next += 1
        accs = []
        for j in range(5):
            t = acc[:, j * 128:(j + 1) * 128]
            for p in range(NPAIR - n_tail, NPAIR):
                t = t + _dot(o_v[:, p * PAIR:(p + 1) * PAIR],
                             _unpack(woA_v[p, :, j * 128:(j + 1) * 128]))
            accs.append(t)
        a = jnp.concatenate([t[M_A:] for t in accs], axis=1)
        gw = gw_v[...].astype(F32)
        gx = xs[:, 0:128] * gw[0:1, :]
        for j in range(1, 5):
            gx = gx + xs[:, j * 128:(j + 1) * 128] * gw[j:j + 1, :]
        g = jax.nn.sigmoid(jnp.sum(gx, axis=1, keepdims=True))
        res = g * a + (1.0 - g) * bmix[pl.ds(r0, SEG), :]
        out_v[pl.ds(r0, SEG), :] = res.astype(BF16)
        return [t[:M_A] for t in accs]

    def seg_step(it, carry):
        rows = UNROLL * SEG
        base = pl.multiple_of(it * rows, rows)
        mem = [mem_v[:, j * 128:(j + 1) * 128] for j in range(5)]
        for u in range(UNROLL):
            r0 = pl.multiple_of(base + u * SEG, SEG)
            mem = segment(r0, mem)
            pltpu.make_async_copy(out_v.at[pl.ds(r0, SEG), :], out_hbm.at[pl.ds(r0, SEG), :],
                                  out_sem).start()
        for j in range(5):
            mem_v[:, j * 128:(j + 1) * 128] = mem[j]
        return carry

    lax.fori_loop(0, NSTEPS // UNROLL, seg_step, 0)
    pltpu.make_async_copy(out_v.at[pl.ds(0, NSTEPS * SEG), :], out_hbm.at[pl.ds(0, NSTEPS * SEG), :],
                          out_sem).wait()


def pallas_gated_mix__memory_aug_recurrent_mem_tr__sliding_local_dilated__prompt_kernel(
    A_x, A_mem0, A_Wq, A_Wk, A_Wv, A_Wo, A_seg_len, B_x, B_wqkv, B_wo, gate_w,
):
    del B_x
    if isinstance(A_seg_len, int):
        assert A_seg_len == SEG
    hd = H_A * DH_A
    xa = A_x.reshape(S, D)
    mem0 = A_mem0.reshape(M_A, D)
    wqT = A_Wq.transpose(1, 2, 0).reshape(hd, D)
    wkT = A_Wk.transpose(1, 2, 0).reshape(hd, D)
    wvT = A_Wv.transpose(1, 2, 0).reshape(hd, D)
    woA = A_Wo.reshape(hd, D)
    gw = gate_w.reshape(5, 128)

    scratch = [
        pltpu.VMEM((S, D), BF16),
        pltpu.VMEM((M_A, D), BF16),
        pltpu.VMEM((4, hd, D), BF16),
        pltpu.VMEM((NPAIR, D // 2, 9 * 128), jnp.uint32),
        pltpu.VMEM((NPAIR, PAIR // 2, D), jnp.uint32),
        pltpu.VMEM((D, 3 * D), BF16),
        pltpu.VMEM((D, D), BF16),
        pltpu.VMEM((5, 4 * D + 32, 128), F32),
        pltpu.VMEM((3 * D // 2, D), jnp.uint32),
        pltpu.VMEM((D // 2, D), jnp.uint32),
        pltpu.VMEM((5, 128), BF16),
        pltpu.VMEM((S // NPAIR // 2, D), jnp.uint32),
        pltpu.VMEM((5, S, 128), F32),
        pltpu.VMEM((5, HALO + S, 128), F32),
        pltpu.VMEM((5, HALO + S, 128), F32),
        pltpu.VMEM((S // NPAIR, D), F32),
        pltpu.VMEM((S // NPAIR, D), F32),
        pltpu.VMEM((S, D), F32),
        pltpu.VMEM((M_A, D), F32),
        pltpu.VMEM((L, hd), F32),
        pltpu.VMEM((S, D), BF16),
        pltpu.SemaphoreType.DMA((9,)),
        pltpu.SemaphoreType.DMA((NPAIR,)),
        pltpu.SemaphoreType.DMA,
    ]
    out = pl.pallas_call(
        _kernel,
        out_shape=jax.ShapeDtypeStruct((S, D), BF16),
        in_specs=[pl.BlockSpec(memory_space=pl.ANY)] * 9,
        out_specs=pl.BlockSpec(memory_space=pl.ANY),
        scratch_shapes=scratch,
        compiler_params=pltpu.CompilerParams(vmem_limit_bytes=120 * 1024 * 1024,
                                             disable_bounds_checks=True),
    )(xa, mem0, wqT, wkT, wvT, woA, B_wqkv, B_wo, gw)
    return out.reshape(1, S, D)
```

```python
import functools

import jax
import jax.numpy as jnp
from jax import lax
import jax.experimental.pallas as pl
import jax.experimental.pallas.tpu as pltpu

F32 = jnp.float32
BF16 = jnp.bfloat16

S = 2048
D = 640
H_A, DH_A = 32, 192
M_A = 8
SEG = 32
L = M_A + SEG
NPAIR = H_A // 2
PAIR = 2 * DH_A
H_B, DH_B = 32, 20
WIN, DIL = 8, 2
HALO = 16
NEG = -1000000000.0

B_ROWS = 8
NSTEPS = S // SEG
UNROLL = 4
LEAD = 2
XLU_START = 0
XLU_END = 6
VPU_START = 6
VPU_END = 20

NT = (((1,), (1,)), ((), ()))
NN = (((1,), (0,)), ((), ()))


def _dot(a, b, dn=NN):
    return lax.dot_general(a, b, dn, preferred_element_type=F32)


def _pack(x):
    return pltpu.bitcast(x, jnp.uint32)


def _unpack(x):
    return pltpu.bitcast(x, BF16)


def _recip(d):
    r = pl.reciprocal(d, approx=True)
    return r * (2.0 - d * r)


def _kernel(xa_hbm, mem0_hbm, wqT_hbm, wkT_hbm, wvT_hbm, woA_hbm,
            wqkvB_hbm, woB_hbm, gw_hbm,
            out_hbm,
            xa_v, mem0_v, wT_v, wqkv_v, woA_v,
            wB_raw, woB_raw, w32, wBT_v, woB_v, gw_v,
            xp, qB, kB, vB, oB0, oB1, bmix,
            mem_v, o_v, out_v,
            sems, pair_sems, out_sem):
    XA_HEAD = 3 * (S // NPAIR)
    cp_wB = [pltpu.make_async_copy(wqkvB_hbm.at[:, j * D:(j + 1) * D],
                                   wB_raw.at[:, j * D:(j + 1) * D], sems.at[j]) for j in range(3)]
    cp_xa0 = pltpu.make_async_copy(xa_hbm.at[0:XA_HEAD, :], xa_v.at[0:XA_HEAD, :], sems.at[3])
    cp_woB = pltpu.make_async_copy(woB_hbm, woB_raw, sems.at[4])
    cp_xa1 = pltpu.make_async_copy(xa_hbm.at[XA_HEAD:S, :], xa_v.at[XA_HEAD:S, :], sems.at[5])
    cp_m0 = pltpu.make_async_copy(mem0_hbm, mem0_v, sems.at[6])
    cp_gw = pltpu.make_async_copy(gw_hbm, gw_v, sems.at[7])

    def pair_copies(p):
        r = pl.multiple_of(p * PAIR, 128)
        last = isinstance(p, int) and p == NPAIR - 1
        return [pltpu.make_async_copy(w.at[pl.ds(r, PAIR), :], wT_v.at[t, pl.ds(r, PAIR), :],
                                      sems.at[8] if (last and t == 3) else pair_sems.at[p])
                for t, w in enumerate((wqT_hbm, wkT_hbm, wvT_hbm, woA_hbm))]

    for cp in [cp_wB[0], cp_xa0, cp_wB[1], cp_wB[2], cp_woB, cp_xa1, cp_m0, cp_gw]:
        cp.start()

    def gather_rows(base, dst, dst_base):
        for d in range(DH_B):
            r = (dst_base + d * H_B) // 2
            for c in range(5):
                g = w32[c, pl.ds(base + d, H_B, stride=DH_B), :]
                dst[r:r + H_B // 2, c * 128:(c + 1) * 128] = _pack(g.astype(BF16))

    def permute_wqkv(which):
        for cb in range(5 * which, 5 * which + 5):
            for rb in range(5):
                tile = wB_raw[rb * 128:(rb + 1) * 128, cb * 128:(cb + 1) * 128]
                w32[rb, cb * 128:(cb + 1) * 128, :] = tile.T.astype(F32)
        gather_rows(which * D, wBT_v, which * D)

    cp_wB[0].wait()
    for p in range(NPAIR):
        for cp in pair_copies(p):
            cp.start()
    permute_wqkv(0)

    zero_halo = jnp.zeros((HALO, 128), F32)
    for j in range(5):
        kB[j, 0:HALO, :] = zero_halo
        vB[j, 0:HALO, :] = zero_halo

    rows_b = S // NPAIR
    scale_b = DH_B ** (-0.5)

    def b_attend(gr, masked):
        nsub = B_ROWS // 8
        offs = sorted({8 * i - DIL * w for i in range(nsub) for w in range(WIN)})

        def windows(ref, j):
            return {off: ref[j, pl.ds(HALO + gr + off, 8), :] for off in offs}

        def shifted(win, w):
            return jnp.concatenate([win[8 * i - DIL * w] for i in range(nsub)], axis=0)

        part = [None] * WIN
        for j in range(5):
            q = qB[j, pl.ds(gr, B_ROWS), :]
            win = windows(kB, j)
            for w in range(WIN):
                t = q * shifted(win, w)
                part[w] = t if part[w] is None else part[w] + t
        logits = []
        for w in range(WIN):
            s = part[w]
            s = s + pltpu.roll(s, 64, 1)
            s = s + pltpu.roll(s, 32, 1)
            logits.append(s)
        if masked:
            pos = gr + lax.broadcasted_iota(jnp.int32, (B_ROWS, 128), 0)
            logits = [jnp.where(pos >= DIL * w, l * scale_b, NEG) for w, l in enumerate(logits)]
            post = 1.0
        else:
            post = scale_b
        m = logits[0]
        for w in range(1, WIN):
            m = jnp.maximum(m, logits[w])
        e = [jnp.exp((l - m) * post) for l in logits]
        den = e[0]
        for w in range(1, WIN):
            den = den + e[w]
        inv = _recip(den)
        cols = []
        for j in range(5):
            win = windows(vB, j)
            acc = e[0] * shifted(win, 0)
            for w in range(1, WIN):
                acc = acc + e[w] * shifted(win, w)
            cols.append(acc * inv)
        return jnp.concatenate(cols, axis=1)

    def _row0(blk):
        return blk * rows_b if isinstance(blk, int) else pl.multiple_of(blk * rows_b, rows_b)

    def b_pack_x(blk):
        r0 = _row0(blk)
        xp[...] = _pack(xa_v[pl.ds(r0, rows_b), :])

    def b_project_tile(blk, n):
        r0 = _row0(blk)
        t = _dot(_unpack(xp[...]), _unpack(wBT_v[n * 64:(n + 1) * 64, :]), NT)
        if n < 5:
            qB[n, pl.ds(r0, rows_b), :] = t
        elif n < 10:
            kB[n - 5, pl.ds(HALO + r0, rows_b), :] = t
        else:
            vB[n - 10, pl.ds(HALO + r0, rows_b), :] = t

    def b_out_tile(blk, slot, n):
        r0 = _row0(blk)
        bmix[pl.ds(r0, rows_b), n * 128:(n + 1) * 128] = _dot(
            oB[slot][...], _unpack(woB_v[:, n * 128:(n + 1) * 128]))

    def xlu_pieces(p):
        r = p * PAIR if isinstance(p, int) else pl.multiple_of(p * PAIR, 128)

        def pair_block(t, k):
            if k == 0:
                return wT_v[t, pl.ds(r, 128), :]
            if k == 1:
                return wT_v[t, pl.ds(r + 192, 128), :]
            return jnp.concatenate([wT_v[t, pl.ds(r + 128, 64), :],
                                    wT_v[t, pl.ds(r + 320, 64), :]], axis=0)

        def xpose_block(t, k):
            blk = pair_block(t, k)
            col = (t * 3 + k) * 128
            for j in range(5):
                tile = blk[:, j * 128:(j + 1) * 128]
                wqkv_v[p, j * 64:(j + 1) * 64, col:col + 128] = _pack(tile.T)

        def repack_block(k):
            woA_v[p, k * 64:(k + 1) * 64, :] = _pack(pair_block(3, k))

        return ([functools.partial(xpose_block, t, k) for t in range(3) for k in range(3)]
                + [functools.partial(repack_block, k) for k in range(3)])

    def b_step(attn_blk, attn_slot, out_blk, proj_blk, xlu, vpu_range=None):
        mxu, vpu = [], []
        if out_blk is not None:
            mxu += [functools.partial(b_out_tile, out_blk, 1 - attn_slot, n) for n in range(5)]
        if proj_blk is not None:
            b_pack_x(proj_blk)
            mxu += [functools.partial(b_project_tile, proj_blk, n) for n in range(15)]
        if attn_blk is not None:
            r0 = attn_blk * rows_b
            if not isinstance(r0, int):
                r0 = pl.multiple_of(r0, rows_b)

            def attend_block(i):
                gr = r0 + i * B_ROWS
                if not isinstance(gr, int):
                    gr = pl.multiple_of(gr, B_ROWS)
                masked = isinstance(gr, int) and gr < (WIN - 1) * DIL
                oB[attn_slot][i * B_ROWS:(i + 1) * B_ROWS, :] = b_attend(gr, masked)

            vpu = [functools.partial(attend_block, i) for i in range(rows_b // B_ROWS)]
        n = len(mxu)
        xs, xe = XLU_START * n // 20, XLU_END * n // 20
        vs, ve = vpu_range or (VPU_START, VPU_END)
        vs, ve = vs * n // 20, ve * n // 20
        for i in range(n):
            mxu[i]()
            if xs <= i < xe:
                k, c = i - xs, xe - xs
                for u in xlu[k * len(xlu) // c:(k + 1) * len(xlu) // c]:
                    u()
            if vs <= i < ve:
                k, c = i - vs, ve - vs
                for u in vpu[k * len(vpu) // c:(k + 1) * len(vpu) // c]:
                    u()

    def wait_pair(p):
        for cp in pair_copies(p):
            cp.wait()

    oB = (oB0, oB1)
    cp_xa0.wait()
    b_pack_x(0)
    for which in range(3):
        if which < 2:
            cp_wB[which + 1].wait()
            permute_wqkv(which + 1)
        for n in range(5 * which, 5 * which + 5):
            b_project_tile(0, n)
    cp_woB.wait()
    for c in range(5):
        w32[c, 3 * D:4 * D, :] = woB_raw[:, c * 128:(c + 1) * 128].astype(F32)
    gather_rows(3 * D, woB_v, 0)
    b_step(0, 0, None, 1, [], (0, 20))
    b_step(1, 1, 0, 2, [], (0, 20))
    cp_xa1.wait()

    def prologue_step(it, carry):
        for u in range(2):
            p = 2 * it + u
            wait_pair(p)
            b_step(p + LEAD, u, p + LEAD - 1, jnp.minimum(p + LEAD + 1, NPAIR - 1),
                   xlu_pieces(p))
        return carry

    lax.fori_loop(0, (NPAIR - LEAD) // 2, prologue_step, 0)
    wait_pair(NPAIR - 2)
    b_step(None, 0, NPAIR - 1, None, xlu_pieces(NPAIR - 2))
    last_copies, last_pieces = pair_copies(NPAIR - 1), xlu_pieces(NPAIR - 1)
    for cp in last_copies[:3]:
        cp.wait()
    for u in last_pieces[:9]:
        u()
    last_copies[3].wait()
    for u in last_pieces[9:]:
        u()

    cp_m0.wait()
    cp_gw.wait()
    mem_v[...] = mem0_v[...].astype(F32)

    scale_a = DH_A ** (-0.5)
    qi = lax.broadcasted_iota(jnp.int32, (L, 2 * L), 0)
    kl = lax.broadcasted_iota(jnp.int32, (L, 2 * L), 1)
    head_a = kl < L
    ki = jnp.where(head_a, kl, kl - L)
    mask = (qi < M_A) | (qi >= ki)
    lane = lax.broadcasted_iota(jnp.int32, (L, 128), 1)
    lo = lane < 64
    zblk = jnp.zeros((L, 128), F32)

    def softmax_pair(s):
        s = jnp.where(mask, s * scale_a, NEG)
        ma = jnp.max(jnp.where(head_a, s, -jnp.inf), axis=1, keepdims=True)
        mb = jnp.max(jnp.where(head_a, -jnp.inf, s), axis=1, keepdims=True)
        e = jnp.exp(s - jnp.where(head_a, ma, mb))
        da = jnp.sum(jnp.where(head_a, e, 0.0), axis=1, keepdims=True)
        db = jnp.sum(jnp.where(head_a, 0.0, e), axis=1, keepdims=True)
        return e * _recip(jnp.where(head_a, da, db))

    def segment(r0, mem):
        xs = xa_v[pl.ds(r0, SEG), :].astype(F32)
        h = [jnp.concatenate([mem[j], xs[:, j * 128:(j + 1) * 128]], axis=0) for j in range(5)]
        h_full = jnp.concatenate(h, axis=1)

        def qkv_proj(p):
            if p == 0:
                y = None
                for j in range(5):
                    t = _dot(h[j], _unpack(wqkv_v[p, j * 64:(j + 1) * 64, :]))
                    y = t if y is None else y + t
                return y
            return _dot(h_full, _unpack(wqkv_v[p]))

        def scores(y):
            q0, q1, q2 = (y[:, k * 128:(k + 1) * 128] for k in range(3))
            k0, k1, k2 = (y[:, (3 + k) * 128:(4 + k) * 128] for k in range(3))
            k2n = jnp.concatenate([jnp.where(lo, k2, 0.0), jnp.where(lo, 0.0, k2)], axis=0)
            sc = (_dot(q0, jnp.concatenate([k0, zblk], axis=0), NT)
                  + _dot(q1, jnp.concatenate([zblk, k1], axis=0), NT)
                  + _dot(q2, k2n, NT))
            return softmax_pair(sc)

        def pv(p, y, pr):
            v0, v1, v2 = (y[:, (6 + k) * 128:(7 + k) * 128] for k in range(3))
            v2n = jnp.concatenate([jnp.where(lo, v2, 0.0), jnp.where(lo, 0.0, v2)], axis=0)
            o_v[:, p * PAIR:p * PAIR + 128] = _dot(pr, jnp.concatenate([v0, zblk], axis=0))
            o_v[:, p * PAIR + 128:p * PAIR + 256] = _dot(pr, jnp.concatenate([zblk, v1], axis=0))
            o_v[:, p * PAIR + 256:p * PAIR + 384] = _dot(pr, v2n)

        def out_proj(p, acc):
            t = _dot(o_v[:, p * PAIR:(p + 1) * PAIR], _unpack(woA_v[p]))
            return t if acc is None else acc + t

        ys, probs = {}, {}
        acc = None
        wo_next = 0
        for i in range(NPAIR + 2):
            if i < NPAIR:
                ys[i] = qkv_proj(i)
            else:
                for _ in range(3):
                    acc = out_proj(wo_next, acc)
                    wo_next += 1
            if 1 <= i <= NPAIR:
                probs[i - 1] = scores(ys[i - 1])
            if i >= 2:
                pv(i - 2, ys.pop(i - 2), probs.pop(i - 2))
        n_tail = 2
        while wo_next < NPAIR - n_tail:
            acc = out_proj(wo_next, acc)
            wo_next += 1
        accs = []
        for j in range(5):
            t = acc[:, j * 128:(j + 1) * 128]
            for p in range(NPAIR - n_tail, NPAIR):
                t = t + _dot(o_v[:, p * PAIR:(p + 1) * PAIR],
                             _unpack(woA_v[p, :, j * 128:(j + 1) * 128]))
            accs.append(t)
        a = jnp.concatenate([t[M_A:] for t in accs], axis=1)
        gw = gw_v[...].astype(F32)
        gx = xs[:, 0:128] * gw[0:1, :]
        for j in range(1, 5):
            gx = gx + xs[:, j * 128:(j + 1) * 128] * gw[j:j + 1, :]
        g = jax.nn.sigmoid(jnp.sum(gx, axis=1, keepdims=True))
        res = g * a + (1.0 - g) * bmix[pl.ds(r0, SEG), :]
        out_v[pl.ds(r0, SEG), :] = res.astype(BF16)
        return [t[:M_A] for t in accs]

    def seg_step(it, carry):
        rows = UNROLL * SEG
        base = pl.multiple_of(it * rows, rows)
        mem = [mem_v[:, j * 128:(j + 1) * 128] for j in range(5)]
        for u in range(UNROLL):
            r0 = pl.multiple_of(base + u * SEG, SEG)
            mem = segment(r0, mem)
            pltpu.make_async_copy(out_v.at[pl.ds(r0, SEG), :], out_hbm.at[pl.ds(r0, SEG), :],
                                  out_sem).start()
        for j in range(5):
            mem_v[:, j * 128:(j + 1) * 128] = mem[j]
        return carry

    lax.fori_loop(0, NSTEPS // UNROLL, seg_step, 0)
    pltpu.make_async_copy(out_v.at[pl.ds(0, NSTEPS * SEG), :], out_hbm.at[pl.ds(0, NSTEPS * SEG), :],
                          out_sem).wait()


def pallas_gated_mix__memory_aug_recurrent_mem_tr__sliding_local_dilated__prompt_kernel(
    A_x, A_mem0, A_Wq, A_Wk, A_Wv, A_Wo, A_seg_len, B_x, B_wqkv, B_wo, gate_w,
):
    del B_x
    if isinstance(A_seg_len, int):
        assert A_seg_len == SEG
    hd = H_A * DH_A
    xa = A_x.reshape(S, D)
    mem0 = A_mem0.reshape(M_A, D)
    wqT = A_Wq.transpose(1, 2, 0).reshape(hd, D)
    wkT = A_Wk.transpose(1, 2, 0).reshape(hd, D)
    wvT = A_Wv.transpose(1, 2, 0).reshape(hd, D)
    woA = A_Wo.reshape(hd, D)
    gw = gate_w.reshape(5, 128)

    scratch = [
        pltpu.VMEM((S, D), BF16),
        pltpu.VMEM((M_A, D), BF16),
        pltpu.VMEM((4, hd, D), BF16),
        pltpu.VMEM((NPAIR, D // 2, 9 * 128), jnp.uint32),
        pltpu.VMEM((NPAIR, PAIR // 2, D), jnp.uint32),
        pltpu.VMEM((D, 3 * D), BF16),
        pltpu.VMEM((D, D), BF16),
        pltpu.VMEM((5, 4 * D + 32, 128), F32),
        pltpu.VMEM((3 * D // 2, D), jnp.uint32),
        pltpu.VMEM((D // 2, D), jnp.uint32),
        pltpu.VMEM((5, 128), BF16),
        pltpu.VMEM((S // NPAIR // 2, D), jnp.uint32),
        pltpu.VMEM((5, S, 128), F32),
        pltpu.VMEM((5, HALO + S, 128), F32),
        pltpu.VMEM((5, HALO + S, 128), F32),
        pltpu.VMEM((S // NPAIR, D), F32),
        pltpu.VMEM((S // NPAIR, D), F32),
        pltpu.VMEM((S, D), F32),
        pltpu.VMEM((M_A, D), F32),
        pltpu.VMEM((L, hd), F32),
        pltpu.VMEM((S, D), BF16),
        pltpu.SemaphoreType.DMA((9,)),
        pltpu.SemaphoreType.DMA((NPAIR,)),
        pltpu.SemaphoreType.DMA,
    ]
    out = pl.pallas_call(
        _kernel,
        out_shape=jax.ShapeDtypeStruct((S, D), BF16),
        in_specs=[pl.BlockSpec(memory_space=pl.ANY)] * 9,
        out_specs=pl.BlockSpec(memory_space=pl.ANY),
        scratch_shapes=scratch,
        compiler_params=pltpu.CompilerParams(vmem_limit_bytes=120 * 1024 * 1024,
                                             disable_bounds_checks=True),
    )(xa, mem0, wqT, wkT, wvT, woA, B_wqkv, B_wo, gw)
    return out.reshape(1, S, D)
```

```python
import functools

import jax
import jax.numpy as jnp
from jax import lax
import jax.experimental.pallas as pl
import jax.experimental.pallas.tpu as pltpu

F32 = jnp.float32
BF16 = jnp.bfloat16

S = 2048
D = 640
H_A, DH_A = 32, 192
M_A = 8
SEG = 32
L = M_A + SEG
NPAIR = H_A // 2
PAIR = 2 * DH_A
H_B, DH_B = 32, 20
WIN, DIL = 8, 2
HALO = 16
NEG = -1000000000.0

B_ROWS = 8
NSTEPS = S // SEG
UNROLL = 4
LEAD = 2
XLU_START = 0
XLU_END = 6
VPU_START = 6
VPU_END = 20

NT = (((1,), (1,)), ((), ()))
NN = (((1,), (0,)), ((), ()))


def _dot(a, b, dn=NN):
    return lax.dot_general(a, b, dn, preferred_element_type=F32)


def _pack(x):
    return pltpu.bitcast(x, jnp.uint32)


def _unpack(x):
    return pltpu.bitcast(x, BF16)


def _recip(d):
    r = pl.reciprocal(d, approx=True)
    return r * (2.0 - d * r)


def _kernel(xa_hbm, mem0_hbm, wqT_hbm, wkT_hbm, wvT_hbm, woA_hbm,
            wqkvB_hbm, woB_hbm, gw_hbm,
            out_hbm,
            xa_v, mem0_v, wT_v, wqkv_v, woA_v,
            wB_raw, woB_raw, w32, wBT_v, woB_v, gw_v,
            xp, qB, kB, vB, oB0, oB1, bmix,
            mem_v, o_v, out_v,
            sems, pair_sems, out_sem):
    XA_HEAD = 3 * (S // NPAIR)
    cp_wB = [pltpu.make_async_copy(wqkvB_hbm.at[:, j * D:(j + 1) * D],
                                   wB_raw.at[:, j * D:(j + 1) * D], sems.at[j]) for j in range(3)]
    cp_xa0 = pltpu.make_async_copy(xa_hbm.at[0:XA_HEAD, :], xa_v.at[0:XA_HEAD, :], sems.at[3])
    cp_woB = pltpu.make_async_copy(woB_hbm, woB_raw, sems.at[4])
    cp_xa1 = pltpu.make_async_copy(xa_hbm.at[XA_HEAD:S, :], xa_v.at[XA_HEAD:S, :], sems.at[5])
    cp_m0 = pltpu.make_async_copy(mem0_hbm, mem0_v, sems.at[6])
    cp_gw = pltpu.make_async_copy(gw_hbm, gw_v, sems.at[7])

    def pair_copies(p):
        r = pl.multiple_of(p * PAIR, 128)
        last = isinstance(p, int) and p == NPAIR - 1
        return [pltpu.make_async_copy(w.at[pl.ds(r, PAIR), :], wT_v.at[t, pl.ds(r, PAIR), :],
                                      sems.at[8] if (last and t == 3) else pair_sems.at[p])
                for t, w in enumerate((wqT_hbm, wkT_hbm, wvT_hbm, woA_hbm))]

    for cp in [cp_wB[0], cp_xa0, cp_wB[1], cp_wB[2], cp_woB, cp_xa1, cp_m0, cp_gw]:
        cp.start()

    def gather_rows(base, dst, dst_base):
        for d in range(DH_B):
            r = (dst_base + d * H_B) // 2
            for c in range(5):
                g = w32[c, pl.ds(base + d, H_B, stride=DH_B), :]
                dst[r:r + H_B // 2, c * 128:(c + 1) * 128] = _pack(g.astype(BF16))

    def permute_wqkv(which):
        for cb in range(5 * which, 5 * which + 5):
            for rb in range(5):
                tile = wB_raw[rb * 128:(rb + 1) * 128, cb * 128:(cb + 1) * 128]
                w32[rb, cb * 128:(cb + 1) * 128, :] = tile.T.astype(F32)
        gather_rows(which * D, wBT_v, which * D)

    cp_wB[0].wait()
    for p in range(NPAIR):
        for cp in pair_copies(p):
            cp.start()
    permute_wqkv(0)

    zero_halo = jnp.zeros((HALO, 128), F32)
    for j in range(5):
        kB[j, 0:HALO, :] = zero_halo
        vB[j, 0:HALO, :] = zero_halo

    rows_b = S // NPAIR
    scale_b = DH_B ** (-0.5)

    def b_attend(gr, masked):
        nsub = B_ROWS // 8
        offs = sorted({8 * i - DIL * w for i in range(nsub) for w in range(WIN)})

        def windows(ref, j):
            return {off: ref[j, pl.ds(HALO + gr + off, 8), :] for off in offs}

        def shifted(win, w):
            return jnp.concatenate([win[8 * i - DIL * w] for i in range(nsub)], axis=0)

        part = [None] * WIN
        for j in range(5):
            q = qB[j, pl.ds(gr, B_ROWS), :]
            win = windows(kB, j)
            for w in range(WIN):
                t = q * shifted(win, w)
                part[w] = t if part[w] is None else part[w] + t
        logits = []
        for w in range(WIN):
            s = part[w]
            s = s + pltpu.roll(s, 64, 1)
            s = s + pltpu.roll(s, 32, 1)
            logits.append(s)
        if masked:
            pos = gr + lax.broadcasted_iota(jnp.int32, (B_ROWS, 128), 0)
            logits = [jnp.where(pos >= DIL * w, l * scale_b, NEG) for w, l in enumerate(logits)]
            post = 1.0
        else:
            post = scale_b
        m = logits[0]
        for w in range(1, WIN):
            m = jnp.maximum(m, logits[w])
        e = [jnp.exp((l - m) * post) for l in logits]
        den = e[0]
        for w in range(1, WIN):
            den = den + e[w]
        inv = _recip(den)
        cols = []
        for j in range(5):
            win = windows(vB, j)
            acc = e[0] * shifted(win, 0)
            for w in range(1, WIN):
                acc = acc + e[w] * shifted(win, w)
            cols.append(acc * inv)
        return jnp.concatenate(cols, axis=1)

    def _row0(blk):
        return blk * rows_b if isinstance(blk, int) else pl.multiple_of(blk * rows_b, rows_b)

    def b_pack_x(blk):
        r0 = _row0(blk)
        xp[...] = _pack(xa_v[pl.ds(r0, rows_b), :])

    def b_project_tile(blk, n):
        r0 = _row0(blk)
        t = _dot(_unpack(xp[...]), _unpack(wBT_v[n * 64:(n + 1) * 64, :]), NT)
        if n < 5:
            qB[n, pl.ds(r0, rows_b), :] = t
        elif n < 10:
            kB[n - 5, pl.ds(HALO + r0, rows_b), :] = t
        else:
            vB[n - 10, pl.ds(HALO + r0, rows_b), :] = t

    def b_out_tile(blk, slot, n):
        r0 = _row0(blk)
        bmix[pl.ds(r0, rows_b), n * 128:(n + 1) * 128] = _dot(
            oB[slot][...], _unpack(woB_v[:, n * 128:(n + 1) * 128]))

    def xlu_pieces(p):
        r = p * PAIR if isinstance(p, int) else pl.multiple_of(p * PAIR, 128)

        def pair_block(t, k):
            if k == 0:
                return wT_v[t, pl.ds(r, 128), :]
            if k == 1:
                return wT_v[t, pl.ds(r + 192, 128), :]
            return jnp.concatenate([wT_v[t, pl.ds(r + 128, 64), :],
                                    wT_v[t, pl.ds(r + 320, 64), :]], axis=0)

        def xpose_block(t, k):
            blk = pair_block(t, k)
            col = (t * 3 + k) * 128
            for j in range(5):
                tile = blk[:, j * 128:(j + 1) * 128]
                wqkv_v[p, j * 64:(j + 1) * 64, col:col + 128] = _pack(tile.T)

        def repack_block(k):
            woA_v[p, k * 64:(k + 1) * 64, :] = _pack(pair_block(3, k))

        return ([functools.partial(xpose_block, t, k) for t in range(3) for k in range(3)]
                + [functools.partial(repack_block, k) for k in range(3)])

    def b_step(attn_blk, attn_slot, out_blk, proj_blk, xlu, vpu_range=None):
        mxu, vpu = [], []
        if out_blk is not None:
            mxu += [functools.partial(b_out_tile, out_blk, 1 - attn_slot, n) for n in range(5)]
        if proj_blk is not None:
            b_pack_x(proj_blk)
            mxu += [functools.partial(b_project_tile, proj_blk, n) for n in range(15)]
        if attn_blk is not None:
            r0 = attn_blk * rows_b
            if not isinstance(r0, int):
                r0 = pl.multiple_of(r0, rows_b)

            def attend_block(i):
                gr = r0 + i * B_ROWS
                if not isinstance(gr, int):
                    gr = pl.multiple_of(gr, B_ROWS)
                masked = isinstance(gr, int) and gr < (WIN - 1) * DIL
                oB[attn_slot][i * B_ROWS:(i + 1) * B_ROWS, :] = b_attend(gr, masked)

            vpu = [functools.partial(attend_block, i) for i in range(rows_b // B_ROWS)]
        n = len(mxu)
        xs, xe = XLU_START * n // 20, XLU_END * n // 20
        vs, ve = vpu_range or (VPU_START, VPU_END)
        vs, ve = vs * n // 20, ve * n // 20
        for i in range(n):
            mxu[i]()
            if xs <= i < xe:
                k, c = i - xs, xe - xs
                for u in xlu[k * len(xlu) // c:(k + 1) * len(xlu) // c]:
                    u()
            if vs <= i < ve:
                k, c = i - vs, ve - vs
                for u in vpu[k * len(vpu) // c:(k + 1) * len(vpu) // c]:
                    u()

    def wait_pair(p):
        for cp in pair_copies(p):
            cp.wait()

    oB = (oB0, oB1)
    cp_xa0.wait()
    b_pack_x(0)
    for which in range(3):
        if which < 2:
            cp_wB[which + 1].wait()
            permute_wqkv(which + 1)
        for n in range(5 * which, 5 * which + 5):
            b_project_tile(0, n)
    cp_woB.wait()
    for c in range(5):
        w32[c, 3 * D:4 * D, :] = woB_raw[:, c * 128:(c + 1) * 128].astype(F32)
    gather_rows(3 * D, woB_v, 0)
    b_step(0, 0, None, 1, [], (0, 20))
    b_step(1, 1, 0, 2, [], (0, 20))
    cp_xa1.wait()

    def prologue_step(it, carry):
        for u in range(2):
            p = 2 * it + u
            wait_pair(p)
            b_step(p + LEAD, u, p + LEAD - 1, jnp.minimum(p + LEAD + 1, NPAIR - 1),
                   xlu_pieces(p))
        return carry

    lax.fori_loop(0, (NPAIR - LEAD) // 2, prologue_step, 0)
    wait_pair(NPAIR - 2)
    b_step(None, 0, NPAIR - 1, None, xlu_pieces(NPAIR - 2))
    last_copies, last_pieces = pair_copies(NPAIR - 1), xlu_pieces(NPAIR - 1)
    for cp in last_copies[:3]:
        cp.wait()
    for u in last_pieces[:9]:
        u()
    last_copies[3].wait()
    for u in last_pieces[9:]:
        u()

    cp_m0.wait()
    cp_gw.wait()
    mem_v[...] = mem0_v[...].astype(F32)

    scale_a = DH_A ** (-0.5)
    qi = lax.broadcasted_iota(jnp.int32, (L, 2 * L), 0)
    kl = lax.broadcasted_iota(jnp.int32, (L, 2 * L), 1)
    head_a = kl < L
    ki = jnp.where(head_a, kl, kl - L)
    mask = (qi < M_A) | (qi >= ki)
    lane = lax.broadcasted_iota(jnp.int32, (L, 128), 1)
    lo = lane < 64
    zblk = jnp.zeros((L, 128), F32)

    def softmax_pair(s):
        s = jnp.where(mask, s * scale_a, NEG)
        ma = jnp.max(jnp.where(head_a, s, -jnp.inf), axis=1, keepdims=True)
        mb = jnp.max(jnp.where(head_a, -jnp.inf, s), axis=1, keepdims=True)
        e = jnp.exp(s - jnp.where(head_a, ma, mb))
        da = jnp.sum(jnp.where(head_a, e, 0.0), axis=1, keepdims=True)
        db = jnp.sum(jnp.where(head_a, 0.0, e), axis=1, keepdims=True)
        return e * _recip(jnp.where(head_a, da, db))

    def segment(r0, mem):
        xs = xa_v[pl.ds(r0, SEG), :].astype(F32)
        h = [jnp.concatenate([mem[j], xs[:, j * 128:(j + 1) * 128]], axis=0) for j in range(5)]
        h_full = jnp.concatenate(h, axis=1)

        def qkv_proj(p):
            if p == 0:
                y = None
                for j in range(5):
                    t = _dot(h[j], _unpack(wqkv_v[p, j * 64:(j + 1) * 64, :]))
                    y = t if y is None else y + t
                return y
            return _dot(h_full, _unpack(wqkv_v[p]))

        def scores(y):
            q0, q1, q2 = (y[:, k * 128:(k + 1) * 128] for k in range(3))
            k0, k1, k2 = (y[:, (3 + k) * 128:(4 + k) * 128] for k in range(3))
            k2n = jnp.concatenate([jnp.where(lo, k2, 0.0), jnp.where(lo, 0.0, k2)], axis=0)
            sc = (_dot(q0, jnp.concatenate([k0, zblk], axis=0).astype(BF16), NT)
                  + _dot(q1, jnp.concatenate([zblk, k1], axis=0).astype(BF16), NT)
                  + _dot(q2, k2n.astype(BF16), NT))
            return softmax_pair(sc)

        def pv(p, y, pr):
            v0, v1, v2 = (y[:, (6 + k) * 128:(7 + k) * 128] for k in range(3))
            v2n = jnp.concatenate([jnp.where(lo, v2, 0.0), jnp.where(lo, 0.0, v2)], axis=0)
            o_v[:, p * PAIR:p * PAIR + 128] = _dot(
                pr, jnp.concatenate([v0, zblk], axis=0).astype(BF16))
            o_v[:, p * PAIR + 128:p * PAIR + 256] = _dot(
                pr, jnp.concatenate([zblk, v1], axis=0).astype(BF16))
            o_v[:, p * PAIR + 256:p * PAIR + 384] = _dot(pr, v2n.astype(BF16))

        def out_proj(p, acc):
            t = _dot(o_v[:, p * PAIR:(p + 1) * PAIR], _unpack(woA_v[p]))
            return t if acc is None else acc + t

        ys, probs = {}, {}
        acc = None
        wo_next = 0
        for i in range(NPAIR + 2):
            if i < NPAIR:
                ys[i] = qkv_proj(i)
            else:
                for _ in range(3):
                    acc = out_proj(wo_next, acc)
                    wo_next += 1
            if 1 <= i <= NPAIR:
                probs[i - 1] = scores(ys[i - 1])
            if i >= 2:
                pv(i - 2, ys.pop(i - 2), probs.pop(i - 2))
        n_tail = 2
        while wo_next < NPAIR - n_tail:
            acc = out_proj(wo_next, acc)
            wo_next += 1
        accs = []
        for j in range(5):
            t = acc[:, j * 128:(j + 1) * 128]
            for p in range(NPAIR - n_tail, NPAIR):
                t = t + _dot(o_v[:, p * PAIR:(p + 1) * PAIR],
                             _unpack(woA_v[p, :, j * 128:(j + 1) * 128]))
            accs.append(t)
        a = jnp.concatenate([t[M_A:] for t in accs], axis=1)
        gw = gw_v[...].astype(F32)
        gx = xs[:, 0:128] * gw[0:1, :]
        for j in range(1, 5):
            gx = gx + xs[:, j * 128:(j + 1) * 128] * gw[j:j + 1, :]
        g = jax.nn.sigmoid(jnp.sum(gx, axis=1, keepdims=True))
        res = g * a + (1.0 - g) * bmix[pl.ds(r0, SEG), :]
        out_v[pl.ds(r0, SEG), :] = res.astype(BF16)
        return [t[:M_A] for t in accs]

    def seg_step(it, carry):
        rows = UNROLL * SEG
        base = pl.multiple_of(it * rows, rows)
        mem = [mem_v[:, j * 128:(j + 1) * 128] for j in range(5)]
        for u in range(UNROLL):
            r0 = pl.multiple_of(base + u * SEG, SEG)
            mem = segment(r0, mem)
            pltpu.make_async_copy(out_v.at[pl.ds(r0, SEG), :], out_hbm.at[pl.ds(r0, SEG), :],
                                  out_sem).start()
        for j in range(5):
            mem_v[:, j * 128:(j + 1) * 128] = mem[j]
        return carry

    lax.fori_loop(0, NSTEPS // UNROLL, seg_step, 0)
    pltpu.make_async_copy(out_v.at[pl.ds(0, NSTEPS * SEG), :], out_hbm.at[pl.ds(0, NSTEPS * SEG), :],
                          out_sem).wait()


def pallas_gated_mix__memory_aug_recurrent_mem_tr__sliding_local_dilated__prompt_kernel(
    A_x, A_mem0, A_Wq, A_Wk, A_Wv, A_Wo, A_seg_len, B_x, B_wqkv, B_wo, gate_w,
):
    del B_x
    if isinstance(A_seg_len, int):
        assert A_seg_len == SEG
    hd = H_A * DH_A
    xa = A_x.reshape(S, D)
    mem0 = A_mem0.reshape(M_A, D)
    wqT = A_Wq.transpose(1, 2, 0).reshape(hd, D)
    wkT = A_Wk.transpose(1, 2, 0).reshape(hd, D)
    wvT = A_Wv.transpose(1, 2, 0).reshape(hd, D)
    woA = A_Wo.reshape(hd, D)
    gw = gate_w.reshape(5, 128)

    scratch = [
        pltpu.VMEM((S, D), BF16),
        pltpu.VMEM((M_A, D), BF16),
        pltpu.VMEM((4, hd, D), BF16),
        pltpu.VMEM((NPAIR, D // 2, 9 * 128), jnp.uint32),
        pltpu.VMEM((NPAIR, PAIR // 2, D), jnp.uint32),
        pltpu.VMEM((D, 3 * D), BF16),
        pltpu.VMEM((D, D), BF16),
        pltpu.VMEM((5, 4 * D + 32, 128), F32),
        pltpu.VMEM((3 * D // 2, D), jnp.uint32),
        pltpu.VMEM((D // 2, D), jnp.uint32),
        pltpu.VMEM((5, 128), BF16),
        pltpu.VMEM((S // NPAIR // 2, D), jnp.uint32),
        pltpu.VMEM((5, S, 128), F32),
        pltpu.VMEM((5, HALO + S, 128), F32),
        pltpu.VMEM((5, HALO + S, 128), F32),
        pltpu.VMEM((S // NPAIR, D), F32),
        pltpu.VMEM((S // NPAIR, D), F32),
        pltpu.VMEM((S, D), F32),
        pltpu.VMEM((M_A, D), F32),
        pltpu.VMEM((L, hd), F32),
        pltpu.VMEM((S, D), BF16),
        pltpu.SemaphoreType.DMA((9,)),
        pltpu.SemaphoreType.DMA((NPAIR,)),
        pltpu.SemaphoreType.DMA,
    ]
    out = pl.pallas_call(
        _kernel,
        out_shape=jax.ShapeDtypeStruct((S, D), BF16),
        in_specs=[pl.BlockSpec(memory_space=pl.ANY)] * 9,
        out_specs=pl.BlockSpec(memory_space=pl.ANY),
        scratch_shapes=scratch,
        compiler_params=pltpu.CompilerParams(vmem_limit_bytes=120 * 1024 * 1024,
                                             disable_bounds_checks=True),
    )(xa, mem0, wqT, wkT, wvT, woA, B_wqkv, B_wo, gw)
    return out.reshape(1, S, D)
```
